```python
import jax
import jax.numpy as jnp

def _softmax(x, axis=-1):
    return jax.nn.softmax(x, axis=axis)

def _gelu(x):
    return jax.nn.gelu(x, approximate=True)

def _silu(x):
    return jax.nn.silu(x)

def _sigmoid(x):
    return jax.nn.sigmoid(x)

def _layernorm(x, axis=-1, eps=1e-05):
    m = jnp.mean(x, axis=axis, keepdims=True)
    v = jnp.var(x, axis=axis, keepdims=True)
    return (x - m) / jnp.sqrt(v + eps)

def _scatter_add(tgt, idx, src, axis=0):
    return tgt.at[idx].add(src)

def _segment_sum(src, seg, n):
    return jax.ops.segment_sum(src, seg, n)

class _Rng:

    def __init__(self, key):
        self._k = key

    def _next(self):
        self._k, sub = jax.random.split(self._k)
        return sub

    def normal(self, shape):
        return jax.random.normal(self._next(), shape, dtype=jnp.bfloat16)

    def randint(self, lo, hi, shape):
        return jax.random.randint(self._next(), shape, lo, hi, dtype=jnp.int32)

    def uniform(self, shape, lo=0.0, hi=1.0):
        return jax.random.uniform(self._next(), shape, jnp.bfloat16, lo, hi)

    def permutation(self, n):
        return jax.random.permutation(self._next(), n)
kernel_name = 'interleave_layers__memory_aug_recurrent_mem_tr__glu_gated_glu__prompt'

def setup_inputs():
    _rng = _Rng(jax.random.key(int.from_bytes(__import__("os").urandom(4), "little")))
    _w = lambda a: (lambda t: t.astype(jnp.bfloat16) if jnp.issubdtype(t.dtype, jnp.floating) else t)(jnp.asarray(a))

    def _A_setup():
        B, S, Dm = (1, 2048, 1024)
        H, Dh = (32, 128)
        M, seg = (8, 32)
        seg = min(seg, S)
        S = S // seg * seg
        return {'x': _w((lambda *s: _rng.normal(s) * 0.05)(B, S, Dm)), 'mem0': _w((lambda *s: _rng.normal(s) * 0.05)(B, M, Dm)), 'Wq': _w((lambda *s: _rng.normal(s) * 0.05)(Dm, H, Dh) * Dm ** (-0.5)), 'Wk': _w((lambda *s: _rng.normal(s) * 0.05)(Dm, H, Dh) * Dm ** (-0.5)), 'Wv': _w((lambda *s: _rng.normal(s) * 0.05)(Dm, H, Dh) * Dm ** (-0.5)), 'Wo': _w((lambda *s: _rng.normal(s) * 0.05)(H, Dh, Dm) * (H * Dh) ** (-0.5)), 'seg_len': seg}
    _A_in = _A_setup()

    def _B_setup():
        B, S, D, F = (1, 2048, 1024, 3584)
        return {'x': _w((lambda *s: _rng.normal(s) * 0.05)(B, S, D)), 'w_gate': _w((lambda *s: _rng.normal(s) * 0.05)(D, F)), 'w_up': _w((lambda *s: _rng.normal(s) * 0.05)(D, F)), 'w_down': _w((lambda *s: _rng.normal(s) * 0.05)(F, D))}
    _B_in = _B_setup()
    return {'A_x': _A_in['x'], 'A_mem0': _A_in['mem0'], 'A_Wq': _A_in['Wq'], 'A_Wk': _A_in['Wk'], 'A_Wv': _A_in['Wv'], 'A_Wo': _A_in['Wo'], 'A_seg_len': _A_in['seg_len'], 'B_x': _B_in['x'], 'B_w_gate': _B_in['w_gate'], 'B_w_up': _B_in['w_up'], 'B_w_down': _B_in['w_down']}

def reference(A_x, A_mem0, A_Wq, A_Wk, A_Wv, A_Wo, A_seg_len, B_x, B_w_gate, B_w_up, B_w_down):

    def _A_ref(x, mem0, Wq, Wk, Wv, Wo, seg_len):
        B, S, Dm = x.shape
        H, Dh = (Wq.shape[1], Wq.shape[2])
        M = mem0.shape[1]
        scale = Dh ** (-0.5)
        n_seg = S // seg_len
        L = M + seg_len
        idx = jnp.arange(L)
        mask = (idx[:, None] < M) | (idx[:, None] >= idx[None, :])
        mem = mem0
        outs = []
        for s in range(n_seg):
            xs = x[:, s * seg_len:(s + 1) * seg_len, :].copy()
            h = jnp.concatenate([mem, xs], axis=1)
            q = jnp.einsum('btd,dhe->bhte', h, Wq)
            k = jnp.einsum('btd,dhe->bhte', h, Wk)
            v = jnp.einsum('btd,dhe->bhte', h, Wv)
            scores = jnp.einsum('bhqe,bhke->bhqk', q, k) * scale
            scores = jnp.where(mask[None, None], scores, -1000000000.0)
            p = _softmax(scores, axis=-1)
            o = jnp.einsum('bhqk,bhke->bhqe', p, v)
            o = jnp.einsum('bhte,hed->btd', o, Wo)
            mem = o[:, :M, :].copy()
            outs.append(o[:, M:, :])
        return jnp.concatenate(outs, axis=1)

    def _B_ref(x, w_gate, w_up, w_down):
        g = jnp.einsum('bsd,df->bsf', x, w_gate)
        u = jnp.einsum('bsd,df->bsf', x, w_up)
        h = _sigmoid(g) * u
        return jnp.einsum('bsf,fd->bsd', h, w_down)
    x = A_x
    x = x + _A_ref(_layernorm(x, axis=-1), A_mem0, A_Wq, A_Wk, A_Wv, A_Wo, A_seg_len)
    x = x + _B_ref(_layernorm(x, axis=-1), B_w_gate, B_w_up, B_w_down)
    x = x + _A_ref(_layernorm(x, axis=-1), A_mem0, A_Wq, A_Wk, A_Wv, A_Wo, A_seg_len)
    x = x + _B_ref(_layernorm(x, axis=-1), B_w_gate, B_w_up, B_w_down)
    return x
```

```python
import functools

import jax
import jax.numpy as jnp
import numpy as np
import jax.experimental.pallas as pl
import jax.experimental.pallas.tpu as pltpu

F32 = jnp.float32
BF16 = jnp.bfloat16
U32 = jnp.uint32
EPS = 1e-5
LOG2E = 1.4426950408889634

CFG = dict(G=2, WG=2, FC=512, NSTAGE=4, DC=128, LAG=3)


def _ln(x):
    m = jnp.mean(x, axis=-1, keepdims=True)
    c = x - m
    v = jnp.mean(c * c, axis=-1, keepdims=True)
    return c * jax.lax.rsqrt(v + EPS)


def _pack(x):
    return pltpu.bitcast(x.astype(BF16), U32)


def _unpack(x):
    return pltpu.bitcast(x, BF16)


def _dot(a, b):
    return jnp.dot(a, b, preferred_element_type=F32)


def _dot_nt(a, b):
    return jax.lax.dot_general(a, b, (((1,), (1,)), ((), ())), preferred_element_type=F32)


def _make_kernel(S, D, H, E, M, T, F, cfg):
    G, WG, FC, NSTAGE, DC, LAG = (cfg[k] for k in ("G", "WG", "FC", "NSTAGE", "DC", "LAG"))
    NSEG = S // T
    NG = H // G
    NDC = D // DC
    NFC = F // FC
    NWO = NG // WG
    KO = WG * G * E
    MM = 2 * M
    T2 = T // 2
    XHEAD = (LAG + 1) * T
    scale = float(E) ** -0.5

    def mask_tables(nl):
        R = MM + nl * T
        r = jax.lax.broadcasted_iota(jnp.int32, (R, R), 0)
        c = jax.lax.broadcasted_iota(jnp.int32, (R, R), 1)

        def layer(i):
            return jnp.where(i < M, 0, jnp.where(i < MM, 1, jnp.where(i < MM + T, 0, 1)))

        same = layer(r) == layer(c)
        vis = same & ((r < MM) | (c <= r))
        fill = jnp.where(same, -1e9 * LOG2E, -jnp.inf).astype(F32)
        return vis, fill

    def kernel(x_hbm, mem_ref, wq_hbm, wk_hbm, wv_hbm, wo_hbm, wg_hbm, wu_hbm, wd_hbm, out_hbm,
               x_v, out_v, wqkv, wo, wg, wu, wd, stage, h_s, hb_s, y_s, z_s,
               sem_x, sem_stage, sem_wo, sem_g, sem_u, sem_d, sem_out):
        srcs = (wq_hbm, wk_hbm, wv_hbm)

        def stage_copy(i):
            return pltpu.make_async_copy(srcs[i // NDC].at[i % NDC], stage.at[i % NSTAGE],
                                         sem_stage.at[i % NSTAGE])

        cx0 = pltpu.make_async_copy(x_hbm.at[0:XHEAD], x_v.at[0:XHEAD], sem_x.at[0])
        cx1 = pltpu.make_async_copy(x_hbm.at[XHEAD:S], x_v.at[XHEAD:S], sem_x.at[1])
        cwo = pltpu.make_async_copy(wo_hbm, wo, sem_wo)
        cwg = pltpu.make_async_copy(wg_hbm, wg, sem_g)
        cwu = pltpu.make_async_copy(wu_hbm, wu, sem_u)
        cwd = pltpu.make_async_copy(wd_hbm, wd, sem_d)
        cx0.start()
        for i in range(NSTAGE):
            stage_copy(i).start()
        for i in range(3 * NDC):
            stage_copy(i).wait()
            which, c = i // NDC, i % NDC
            s32 = stage.at[i % NSTAGE].bitcast(U32)
            for j in range(H // 2):
                a = s32[pl.ds(j, DC // 2, stride=H), :]
                b = s32[pl.ds(H // 2 + j, DC // 2, stride=H), :]
                lo = (a & np.uint32(0xFFFF)) | (b << 16)
                hi = (a >> 16) | (b & np.uint32(0xFFFF0000))
                for hh, val in ((2 * j, lo), (2 * j + 1, hi)):
                    col = (which * G + hh % G) * E
                    wqkv[hh // G, c * (DC // 2):(c + 1) * (DC // 2), col:col + E] = val
            if i + NSTAGE < 3 * NDC:
                stage_copy(i + NSTAGE).start()
            elif i + NSTAGE == 3 * NDC:
                cwo.start()

        def rows(seg, n=1):
            return pl.ds(pl.multiple_of(seg * T, T), n * T)

        def out_copy(seg):
            return pltpu.make_async_copy(out_v.at[rows(seg)], out_hbm.at[rows(seg)], sem_out)

        def x_seg(seg):
            return x_v[rows(seg), :].astype(F32)

        def attention_ops(nl, finish):
            R = MM + nl * T
            vis, fill = mask_tables(nl)

            def proj(g):
                return _dot(_unpack(h_s[0:R // 2, :]), _unpack(wqkv[g])).astype(BF16)

            def softmax(s):
                s = jnp.where(vis, s * (scale * LOG2E), fill)
                p = jnp.exp2(s - jnp.max(s, axis=-1, keepdims=True))
                return p.astype(BF16), 1.0 / jnp.sum(p, axis=-1, keepdims=True)

            def out_proj(acc, outs, c):
                d = _dot(jnp.concatenate(outs, axis=1), wo[c * KO:(c + 1) * KO, :])
                return d if acc is None else acc + d

            qkv = proj(0)
            acc, outs, pend = None, [], None
            for g in range(NG):
                tail = g + 1 == NG
                ss = [_dot_nt(qkv[:, i * E:(i + 1) * E], qkv[:, (G + i) * E:(G + i + 1) * E])
                      for i in range(G)]
                if pend is not None and (tail or g + 1 + cfg.get("HOLD", 1) < NG):
                    acc = out_proj(acc, *pend)
                    pend = None
                if tail:
                    yield
                else:
                    nxt = proj(g + 1)
                for i in range(G):
                    p, inv = softmax(ss[i])
                    o = _dot(p, qkv[:, (2 * G + i) * E:(2 * G + i + 1) * E]) * inv
                    outs.append(o.astype(BF16))
                if (g + 1) % WG == 0:
                    pend, outs = (outs, g // WG), []
                qkv = nxt
            yield
            finish(out_proj(acc, *pend))

        def glu_ops(load_h, finish, waits=False):
            def gate_up(c):
                cols = slice(c * FC, (c + 1) * FC)
                hb = load_h()
                return (jax.nn.sigmoid(_dot(hb, wg[:, cols])) * _dot(hb, wu[:, cols])).astype(BF16)

            if waits:
                cwg.wait()
                cwu.wait()
                acts = [gate_up(c) for c in range(NFC)]
                cwd.wait()
                finish(sum(_dot(acts[c], wd[c * FC:(c + 1) * FC, :]) for c in range(NFC)))
                return
            a = gate_up(0)
            yield
            acc = None
            for c in range(NFC):
                if c + 1 < NFC:
                    nxt = gate_up(c + 1)
                if c == 0:
                    yield
                d = _dot(a, wd[c * FC:(c + 1) * FC, :])
                acc = d if acc is None else acc + d
                a = nxt
            finish(acc)

        def run(*gens):
            gens = list(gens)
            while gens:
                for gen in list(gens):
                    if next(gen, "done") == "done":
                        gens.remove(gen)

        cx0.wait()
        mem0 = mem_ref[...].astype(F32)
        h_s[0:M, :] = _pack(jnp.concatenate([mem0, mem0], axis=0))
        h_s[M:M + T2, :] = _pack(_ln(x_seg(0)))
        cwo.wait()
        cwg.start()
        cwu.start()
        cwd.start()
        cx1.start()

        def head_step(t, carry):
            def finish(acc):
                y = x_seg(t) + acc[MM:]
                z_s[rows(t), :] = y
                h_s[0:M, :] = _pack(jnp.concatenate([acc[0:M], mem0], axis=0))
                h_s[M:M + T2, :] = _pack(_ln(x_seg(t + 1)))
            run(attention_ops(1, finish))
            return carry

        jax.lax.fori_loop(0, LAG, head_step, 0)
        nb = (LAG - 1) * T
        hb0 = _ln(z_s[0:nb, :]).astype(BF16)

        def head_glu_finish(d):
            z_s[0:nb, :] = z_s[0:nb, :] + d

        run(glu_ops(lambda: hb0, head_glu_finish, waits=True))
        y_last = z_s[nb:nb + T, :]
        h_last = _pack(_ln(y_last))
        for i in range(2):
            y_s[LAG % 2, i * T:(i + 1) * T, :] = y_last
            hb_s[LAG % 2, i * T2:(i + 1) * T2, :] = h_last
        h_s[M + T2:, :] = _pack(_ln(z_s[0:T, :]))
        cx1.wait()

        def step(t, carry):
            cur, prv = (t + 1) % 2, t % 2
            if LAG > 2:
                h_next = _pack(_ln(z_s[rows(t + 1 - LAG), :]))

            def att_finish(acc):
                y = jnp.concatenate([x_seg(t), z_s[rows(t - LAG), :]], axis=0) + acc[MM:]
                y_s[cur] = y
                hb_s[cur] = _pack(_ln(y))
                h_s[0:M, :] = _pack(acc[0:MM])
                h_s[M:M + T2, :] = _pack(_ln(x_seg(jnp.minimum(t + 1, NSEG - 1))))
                if LAG > 2:
                    h_s[M + T2:, :] = h_next

            def glu_finish(d):
                z = y_s[prv] + d
                z_s[rows(t - 1), :] = z[0:T]
                if LAG == 2:
                    h_s[M + T2:, :] = _pack(_ln(z[0:T]))
                out_v[rows(jnp.maximum(t - 1 - LAG, 0)), :] = z[T:].astype(BF16)

            @pl.when(t > LAG + 1)
            def _():
                out_copy(t - 2 - LAG).start()

            run(attention_ops(2, att_finish), glu_ops(lambda: _unpack(hb_s[prv]), glu_finish))
            return carry

        NS = cfg.get("NSTEP", NSEG)
        jax.lax.fori_loop(LAG, NS, step, 0)
        out_copy(NS - 2 - LAG).start()

        def mid_finish(d):
            z = y_s[NSEG % 2] + d
            z_s[(NSEG - 1) * T:, :] = z[0:T]
            out_v[rows(NSEG - 1 - LAG), :] = z[T:].astype(BF16)

        run(glu_ops(lambda: _unpack(hb_s[NSEG % 2]), mid_finish))
        out_copy(NSEG - 1 - LAG).start()
        mem2 = _unpack(h_s[0:M, :]).astype(F32)[M:MM]
        h_s[0:M, :] = _pack(jnp.concatenate([mem2, mem2], axis=0))
        h_s[M:M + T2, :] = h_s[M + T2:, :]

        def tail_step(t, carry):
            def finish(acc):
                h_next = _pack(_ln(z_s[rows(jnp.minimum(t + 1, NSEG - 1)), :]))
                z_s[rows(t), :] = z_s[rows(t), :] + acc[MM:]
                h_s[0:M, :] = _pack(acc[0:MM])
                h_s[M:M + T2, :] = h_next
            run(attention_ops(1, finish))
            return carry

        jax.lax.fori_loop(NSEG - LAG, NSEG, tail_step, 0)
        r0 = (NSEG - LAG) * T
        hb1 = _ln(z_s[r0:, :]).astype(BF16)

        def last_finish(d):
            out_v[r0:, :] = (z_s[r0:, :] + d).astype(BF16)

        run(glu_ops(lambda: hb1, last_finish))
        pltpu.make_async_copy(out_v.at[r0:S], out_hbm.at[r0:S], sem_out).start()
        n_out = NS * T
        pltpu.make_async_copy(out_v.at[0:n_out], out_hbm.at[0:n_out], sem_out).wait()

    dma = pltpu.SemaphoreType.DMA
    scratch = [
        pltpu.VMEM((S, D), BF16),
        pltpu.VMEM((S, D), BF16),
        pltpu.VMEM((NG, D // 2, 3 * G * E), U32),
        pltpu.VMEM((H * E, D), BF16),
        pltpu.VMEM((D, F), BF16),
        pltpu.VMEM((D, F), BF16),
        pltpu.VMEM((F, D), BF16),
        pltpu.VMEM((NSTAGE, DC * H, E), BF16),
        pltpu.VMEM((M + T, D), U32),
        pltpu.VMEM((2, T, D), U32),
        pltpu.VMEM((2, 2 * T, D), F32),
        pltpu.VMEM((S, D), F32),
        dma((2,)), dma((NSTAGE,)), dma, dma, dma, dma, dma,
    ]
    return kernel, scratch


def build(cfg):
    @functools.partial(jax.jit, static_argnames=("A_seg_len",))
    def fn(A_x, A_mem0, A_Wq, A_Wk, A_Wv, A_Wo, A_seg_len, B_x, B_w_gate, B_w_up, B_w_down):
        del B_x
        B, S, D = A_x.shape
        _, H, E = A_Wq.shape
        M = A_mem0.shape[1]
        F = B_w_gate.shape[1]
        T = int(A_seg_len)
        DC = cfg["DC"]
        kernel, scratch = _make_kernel(S, D, H, E, M, T, F, cfg)
        hbm = pl.BlockSpec(memory_space=pl.ANY)
        out = pl.pallas_call(
            kernel,
            out_shape=jax.ShapeDtypeStruct((S, D), A_x.dtype),
            in_specs=[hbm, pl.BlockSpec(memory_space=pltpu.VMEM)] + [hbm] * 7,
            out_specs=hbm,
            scratch_shapes=scratch,
            compiler_params=pltpu.CompilerParams(vmem_limit_bytes=110 * 1024 * 1024,
                                                 flags=cfg.get("flags")),
        )(A_x.reshape(S, D), A_mem0.reshape(M, D),
          A_Wq.reshape(D // DC, DC * H, E), A_Wk.reshape(D // DC, DC * H, E),
          A_Wv.reshape(D // DC, DC * H, E), A_Wo.reshape(H * E, D),
          B_w_gate, B_w_up, B_w_down)
        return out.reshape(B, S, D)

    return fn


pallas_interleave_layers__memory_aug_recurrent_mem_tr__glu_gated_glu__prompt_kernel = build(CFG)
```

```python
import functools

import jax
import jax.numpy as jnp
import numpy as np
import jax.experimental.pallas as pl
import jax.experimental.pallas.tpu as pltpu

F32 = jnp.float32
BF16 = jnp.bfloat16
U32 = jnp.uint32
EPS = 1e-5
LOG2E = 1.4426950408889634

CFG = dict(OSPLIT=12, DSPLIT=12, FW=256, NSTAGE=4, NSTRIP=8, DC=64, LAG=3, RING=8)


def _ln(x):
    m = jnp.mean(x, axis=-1, keepdims=True)
    c = x - m
    v = jnp.mean(c * c, axis=-1, keepdims=True)
    return c * jax.lax.rsqrt(v + EPS)


def _pack(x):
    return pltpu.bitcast(x.astype(BF16), U32)


def _unpack(x):
    return pltpu.bitcast(x, BF16)


def _dot(a, b):
    return jax.lax.dot_general(a, b, (((1,), (0,)), ((), ())), preferred_element_type=F32)


def _dot_nt(a, b):
    return jax.lax.dot_general(a, b, (((1,), (1,)), ((), ())), preferred_element_type=F32)


def _halves(x):
    n = x.shape[1] // 2
    return x[:, :n], x[:, n:]


def _left_terms(a11, a12, a21=None, a22=None):
    if a21 is None:
        return {0: a11, 2: a11, 4: a11 + a12, 6: a12}
    return {0: a11 + a22, 1: a21 + a22, 2: a11, 3: a22, 4: a11 + a12, 6: a12 - a22, 5: a21 - a11}


def _right_terms(b11, b12, b21, b22):
    f11, f12, f21, f22 = (b.astype(F32) for b in (b11, b12, b21, b22))
    return [_pack(b) for b in (f11 + f22, b11, f12 - f22, f21 - f11, b22, f11 + f12, f21 + f22)]


def _block_product(nl, product):
    if nl == 1:
        m4 = product(4)
        return [product(0) - m4 + product(6), product(2) + m4]
    m0 = product(0)
    m1 = product(1)
    c22 = m0 - m1
    m3 = product(3)
    c11, c21 = m0 + m3, m1 + m3
    m2 = product(2)
    c22 = c22 + m2
    m4 = product(4)
    c11, c12 = c11 - m4, m2 + m4
    return [c11 + product(6), c12, c21, c22 + product(5)]


def _long_product(nl, left, right, k0, k1, n0, n1, width, acc):
    out = []
    for n in range(n0, n1, width):
        def product(i):
            parts = [_dot(left(i, k, min(k + 512, k1)), right(i, k, min(k + 512, k1), n, n + width))
                     for k in range(k0, k1, 512)]
            return functools.reduce(lambda a, b: a + b, parts)
        blocks = _block_product(nl, product)
        out += [[b[:, j:j + 128] for b in blocks] for j in range(0, width, 128)]
    if acc is not None:
        out = [[a + b for a, b in zip(old, new)] for old, new in zip(acc, out)]
    return out


def _row_blocks(tiles):
    return [jnp.concatenate([t[j] for t in tiles] + [t[j + 1] for t in tiles], axis=1)
            for j in range(0, len(tiles[0]), 2)]


def _run(*gens):
    gens = list(gens)
    while gens:
        for gen in list(gens):
            if next(gen, "done") == "done":
                gens.remove(gen)


def _make_kernel(S, D, H, E, M, T, F, cfg):
    OSPLIT, DSPLIT, FW, NSTAGE, NSTRIP, DC, LAG, RING = (
        cfg[k] for k in ("OSPLIT", "DSPLIT", "FW", "NSTAGE", "NSTRIP", "DC", "LAG", "RING"))
    NSEG = S // T
    NG = H // 2
    DH = D // 2
    NDC = DH // DC
    NFC = F // (2 * FW)
    NFT = F // 256
    L = M + T
    scale = float(E) ** -0.5
    SUB = 64

    def mask_tables(nl):
        r = jax.lax.broadcasted_iota(jnp.int32, (nl * L, nl * L), 0)
        c = jax.lax.broadcasted_iota(jnp.int32, (nl * L, nl * L), 1)
        same = (r < L) == (c < L)
        vis = same & ((jnp.where(r < L, r, r - L) < M) | (c <= r))
        return vis, jnp.where(same, -1e9 * LOG2E, -jnp.inf).astype(F32)

    def kernel(x_hbm, mem_ref, wq_hbm, wk_hbm, wv_hbm, wo_hbm, wg_hbm, wu_hbm, wd_hbm, out_hbm,
               wqkv, wo, wgu, wd, st_qkv, st_row, st_col, x_v, out_v, last_v,
               h_s, o_s, hb_s, a_s, mem_s, ya_s, yb_s, z_s,
               sem_qkv, sem_row, sem_col, sem_x, sem_out, sem_last):
        def qkv_copy(i):
            src = (wq_hbm, wk_hbm, wv_hbm)[i // NDC]
            return pltpu.make_async_copy(src.at[:, i % NDC], st_qkv.at[i % NSTAGE],
                                         sem_qkv.at[i % NSTAGE])

        def wo_copy(i):
            return pltpu.make_async_copy(wo_hbm.at[i], st_row.at[i], sem_row.at[i])

        def wd_copy(i):
            return pltpu.make_async_copy(wd_hbm.at[i], st_row.at[i], sem_row.at[i])

        def gu_copy(i):
            cols = pl.ds((i // 2) * 2 * FW, 2 * FW)
            return pltpu.make_async_copy((wg_hbm, wu_hbm)[i % 2].at[:, cols],
                                         st_col.at[i % NSTRIP], sem_col.at[i % NSTRIP])

        def convert(n, load, store):
            def body(r, carry):
                src = pl.ds(pl.multiple_of(r * SUB, SUB), SUB)
                dst = pl.ds(pl.multiple_of(r * (SUB // 2), SUB // 2), SUB // 2)
                for i, w in enumerate(_right_terms(*load(src))):
                    store(i, dst, w)
                return carry
            jax.lax.fori_loop(0, n // SUB, body, 0)

        def convert_qkv(i):
            qkv_copy(i).wait()
            which, c = i // NDC, i % NDC
            words = [st_qkv.at[i % NSTAGE, half].bitcast(U32) for half in range(2)]
            for g in range(NG):
                blocks = []
                for w in words:
                    a = w[pl.ds(g, DC // 2, stride=H), :]
                    b = w[pl.ds(NG + g, DC // 2, stride=H), :]
                    blocks.append(_unpack((a & np.uint32(0xFFFF)) | (b << 16)))
                    blocks.append(_unpack((a >> 16) | (b & np.uint32(0xFFFF0000))))
                for k, w in enumerate(_right_terms(*blocks)):
                    wqkv[g, k, c * (DC // 2):(c + 1) * (DC // 2), which * E:(which + 1) * E] = w

        def convert_wo(c):
            wo_copy(c).wait()
            for r in range(0, 2 * FW, SUB):
                g, e = divmod(r, 2 * E)
                if e < E:
                    blocks = _halves(st_row[c, r:r + SUB, :]) + _halves(st_row[c, r + E:r + E + SUB, :])
                    dst = (c * FW + g * E + e) // 2
                    for i, w in enumerate(_right_terms(*blocks)):
                        wo[i, dst:dst + SUB // 2, :] = w
            if c < NFC:
                wd_copy(c).start()

        def convert_gu(i):
            gu_copy(i).wait()
            slot = i % NSTRIP

            def store(k, rows, w):
                wgu[i % 2, k, rows, (i // 2) * FW:(i // 2 + 1) * FW] = w
            convert(DH, lambda r: (_halves(st_col.at[slot, 0:DH][r, :])
                                   + _halves(st_col.at[slot, DH:D][r, :])), store)
            if i + NSTRIP < 2 * NFC:
                gu_copy(i + NSTRIP).start()

        def convert_wd(c):
            wd_copy(c).wait()

            def store(k, rows, w):
                wd.at[k, c * FW // 2:(c + 1) * FW // 2][rows, :] = w
            convert(FW, lambda r: (_halves(st_row.at[c, 0:FW][r, :])
                                   + _halves(st_row.at[c, FW:2 * FW][r, :])), store)

        def x_copy(seg):
            return pltpu.make_async_copy(x_hbm.at[seg], x_v.at[seg % RING], sem_x.at[seg % RING])

        def out_copy(seg):
            return pltpu.make_async_copy(out_v.at[seg % 2], out_hbm.at[seg], sem_out.at[seg % 2])

        def x_seg(seg):
            return x_v[seg % RING].astype(F32)

        def set_rows(*blocks):
            parts = ()
            for j, (mem, tok) in enumerate(blocks):
                mem_s[j] = mem
                parts += _halves(jnp.concatenate([mem, tok], axis=0))
            for i, a in _left_terms(*parts).items():
                h_s[i] = a

        def attention_ops(nl, finish):
            vis, fill = mask_tables(nl)

            def proj(g):
                res = []
                for j in (1, 0, 2):
                    c = _block_product(
                        nl, lambda i: _dot(h_s[i], _unpack(wqkv[g, i, :, j * E:(j + 1) * E])))
                    c = [jnp.concatenate(c[h::2], axis=0) for h in range(2)]
                    res.append([x.astype(BF16) for x in c])
                return res

            def attend(s, v):
                s = jnp.where(vis, s * (scale * LOG2E), fill)
                p = jnp.exp2(s - jnp.max(s, axis=-1, keepdims=True))
                inv = 1.0 / jnp.sum(p, axis=-1, keepdims=True)
                return _dot(p, v) * inv

            def out_proj(k0, k1, acc):
                return _long_product(
                    nl, lambda i, a, b: o_s[i, :, a:b],
                    lambda i, a, b, n0, n1: _unpack(wo[i, a // 2:b // 2, n0:n1]),
                    k0, k1, 0, DH, 128, acc)

            k, q, v = proj(0)
            for g in range(NG):
                ss = [_dot_nt(q[h], k[h]) for h in range(2)]
                if g + 1 < NG:
                    nxt = proj(g + 1)
                else:
                    acc = out_proj(0, OSPLIT * E, None)
                o = [attend(ss[h], v[h]) for h in range(2)]
                parts = [o[h][j * L:(j + 1) * L] for j in range(nl) for h in range(2)]
                for i, a in _left_terms(*parts).items():
                    o_s[i, :, g * E:(g + 1) * E] = a
                k, q, v = nxt
            yield
            finish(_row_blocks(out_proj(OSPLIT * E, NG * E, acc)))

        def set_glu_rows(top, bot):
            for i, a in _left_terms(*_halves(_ln(top)), *_halves(_ln(bot))).items():
                hb_s[i, 0:top.shape[0] // 2, :] = _pack(a)

        def glu_ops(n, finish, before_up=None, before_down=None):
            def gate_up(c):
                g, u = (_block_product(2, lambda i: _dot(
                    _unpack(hb_s[i, 0:n // 2, :]), _unpack(wgu[j, i, :, c * 128:(c + 1) * 128])))
                        for j in range(2))
                act = [jax.nn.sigmoid(x) * y for x, y in zip(g, u)]
                for i, a in _left_terms(*act).items():
                    a_s[i, 0:n // 2, c * 128:(c + 1) * 128] = _pack(a)

            def down(k0, k1, acc):
                return _long_product(
                    2, lambda i, a, b: _unpack(a_s[i, 0:n // 2, a:b]),
                    lambda i, a, b, n0, n1: _unpack(wd[i, a // 2:b // 2, n0:n1]),
                    k0, k1, 0, DH, 128 if (k1 - k0) % 512 == 0 else 256, acc)

            for c in range(NFT):
                if before_up is not None:
                    before_up(c)
                gate_up(c)
                if c == 0:
                    yield
            if before_down is not None:
                before_down()
            finish(_row_blocks(down(DSPLIT * 128, NFT * 128, down(0, DSPLIT * 128, None))))

        for i in range(NSTAGE):
            qkv_copy(i).start()
        for seg in range(LAG + 2):
            x_copy(seg).start()
        for i in range(3 * NDC):
            convert_qkv(i)
            if i + NSTAGE < 3 * NDC:
                qkv_copy(i + NSTAGE).start()
            elif i + NSTAGE == 3 * NDC:
                for j in range(H * E // (2 * FW)):
                    wo_copy(j).start()
                for j in range(NSTRIP):
                    gu_copy(j).start()
        for c in range(H * E // (2 * FW)):
            convert_wo(c)

        for seg in range(LAG + 1):
            x_copy(seg).wait()
        mem0 = mem_ref[...].astype(F32)
        set_rows((mem0, _ln(x_seg(0))))
        n_early = cfg.get("NEARLY", 2)

        def head_step(t, carry):
            def finish(acc):
                z_s[t] = x_seg(t) + acc[0][M:]
                set_rows((acc[0][:M], _ln(x_seg(t + 1))))
            _run(attention_ops(1, finish))
            for j in range(LAG):
                @pl.when(t == j)
                def _():
                    for i in range(2 * n_early * j, 2 * n_early * (j + 1)):
                        convert_gu(i)
            return carry

        jax.lax.fori_loop(0, LAG, head_step, 0)
        set_glu_rows(z_s[0], z_s[1])

        def head_up(tile):
            c, first = divmod(tile * 128, FW)
            if first == 0 and c >= n_early * LAG:
                convert_gu(2 * c)
                convert_gu(2 * c + 1)

        def head_down():
            for c in range(NFC):
                convert_wd(c)

        def head_finish(d):
            z_s[0] = z_s[0] + d[0]
            z_s[1] = z_s[1] + d[1]

        _run(glu_ops(T, head_finish, head_up, head_down))
        ya_s[0] = z_s[LAG - 1]
        ya_s[1] = z_s[LAG - 1]
        set_rows((mem_s[0], _ln(x_seg(LAG))), (mem0, _ln(z_s[0])))

        def take_rows():
            top, bot = ya_s[0], ya_s[1]
            yb_s[0] = top
            yb_s[1] = bot
            set_glu_rows(top, bot)

        def step(t, carry):
            @pl.when(t + 1 < NSEG)
            def _():
                x_copy(t + 1).wait()

            @pl.when(t + 2 < NSEG)
            def _():
                x_copy(t + 2).start()

            @pl.when(t > LAG + 2)
            def _():
                out_copy(t - 3 - LAG).wait()

            @pl.when(t > LAG + 1)
            def _():
                out_copy(t - 2 - LAG).start()

            take_rows()

            def att_finish(acc):
                ya_s[0] = x_seg(t) + acc[0][M:]
                ya_s[1] = z_s[(t - LAG) % RING] + acc[1][M:]
                set_rows((acc[0][:M], _ln(x_seg(jnp.minimum(t + 1, NSEG - 1)))),
                         (acc[1][:M], _ln(z_s[(t + 1 - LAG) % RING])))

            def glu_finish(d):
                z_s[(t - 1) % RING] = yb_s[0] + d[0]
                out_v[(t + 1 - LAG) % 2] = (yb_s[1] + d[1]).astype(BF16)

            _run(attention_ops(2, att_finish), glu_ops(T, glu_finish))
            return carry

        NS = cfg.get("NSTEP", NSEG)
        jax.lax.fori_loop(LAG, NS, step, 0)
        if NS < NSEG:
            x_copy(NS + 1).wait()
        out_copy(NS - 3 - LAG).wait()
        out_copy(NS - 2 - LAG).start()

        def mid_finish(d):
            z_s[(NSEG - 1) % RING] = yb_s[0] + d[0]
            out_v[(NS - 1 - LAG) % 2] = (yb_s[1] + d[1]).astype(BF16)

        set_rows((mem_s[1], _ln(z_s[(NSEG - LAG) % RING])))
        take_rows()
        _run(glu_ops(T, mid_finish))
        out_copy(NS - 1 - LAG).start()

        def tail_step(t, carry):
            def finish(acc):
                tok = _ln(z_s[jnp.minimum(t + 1, NSEG - 1) % RING])
                z_s[t % RING] = z_s[t % RING] + acc[0][M:]
                set_rows((acc[0][:M], tok))
            _run(attention_ops(1, finish))
            return carry

        jax.lax.fori_loop(NSEG - LAG, NSEG, tail_step, 0)

        def last_rows():
            y = jnp.concatenate([z_s[t % RING] for t in range(NSEG - LAG, NSEG)], axis=0)
            return y[:LAG * T // 2], y[LAG * T // 2:]

        set_glu_rows(*last_rows())

        def last_finish(d):
            z = jnp.concatenate([y + x for y, x in zip(last_rows(), d)], axis=0).astype(BF16)
            for j in range(LAG):
                last_v[j] = z[j * T:(j + 1) * T]

        _run(glu_ops(LAG * T // 2, last_finish))
        last = pltpu.make_async_copy(last_v, out_hbm.at[NSEG - LAG:NSEG], sem_last)
        last.start()
        out_copy(NS - 2 - LAG).wait()
        out_copy(NS - 1 - LAG).wait()
        last.wait()

    dma = pltpu.SemaphoreType.DMA
    n_row = H * E // (2 * FW)
    scratch = [
        pltpu.VMEM((NG, 7, DH // 2, 3 * E), U32),
        pltpu.VMEM((7, H * E // 4, DH), U32),
        pltpu.VMEM((2, 7, DH // 2, F // 2), U32),
        pltpu.VMEM((7, F // 4, DH), U32),
        pltpu.VMEM((NSTAGE, 2, DC * H, E), BF16),
        pltpu.VMEM((n_row, 2 * FW, D), BF16),
        pltpu.VMEM((NSTRIP, D, 2 * FW), BF16),
        pltpu.VMEM((RING, T, D), BF16),
        pltpu.VMEM((2, T, D), BF16),
        pltpu.VMEM((LAG, T, D), BF16),
        pltpu.VMEM((7, L, DH), F32),
        pltpu.VMEM((7, L, H * E // 2), F32),
        pltpu.VMEM((7, LAG * T // 4, DH), U32),
        pltpu.VMEM((7, LAG * T // 4, F // 2), U32),
        pltpu.VMEM((2, M, D), F32),
        pltpu.VMEM((2, T, D), F32),
        pltpu.VMEM((2, T, D), F32),
        pltpu.VMEM((RING, T, D), F32),
        dma((NSTAGE,)), dma((n_row,)), dma((NSTRIP,)), dma((RING,)), dma((2,)), dma,
    ]
    return kernel, scratch


def build(cfg):
    @functools.partial(jax.jit, static_argnames=("A_seg_len",))
    def fn(A_x, A_mem0, A_Wq, A_Wk, A_Wv, A_Wo, A_seg_len, B_x, B_w_gate, B_w_up, B_w_down):
        del B_x
        B, S, D = A_x.shape
        _, H, E = A_Wq.shape
        M = A_mem0.shape[1]
        F = B_w_gate.shape[1]
        T = int(A_seg_len)
        DC, FC = cfg["DC"], 2 * cfg["FW"]
        kernel, scratch = _make_kernel(S, D, H, E, M, T, F, cfg)
        hbm = pl.BlockSpec(memory_space=pl.ANY)
        qkv_shape = (2, D // (2 * DC), DC * H, E)
        out = pl.pallas_call(
            kernel,
            out_shape=jax.ShapeDtypeStruct((S // T, T, D), A_x.dtype),
            in_specs=[hbm, pl.BlockSpec(memory_space=pltpu.VMEM)] + [hbm] * 7,
            out_specs=hbm,
            scratch_shapes=scratch,
            compiler_params=pltpu.CompilerParams(vmem_limit_bytes=124 * 1024 * 1024,
                                                 flags=cfg.get("flags")),
        )(A_x.reshape(S // T, T, D), A_mem0.reshape(M, D),
          A_Wq.reshape(qkv_shape), A_Wk.reshape(qkv_shape), A_Wv.reshape(qkv_shape),
          A_Wo.reshape(H * E // FC, FC, D), B_w_gate, B_w_up, B_w_down.reshape(F // FC, FC, D))
        return out.reshape(B, S, D)

    return fn


pallas_interleave_layers__memory_aug_recurrent_mem_tr__glu_gated_glu__prompt_kernel = build(CFG)
```

```python
import contextlib
import functools

import jax
import jax.numpy as jnp
import numpy as np
import jax.experimental.pallas as pl
import jax.experimental.pallas.tpu as pltpu

F32 = jnp.float32
BF16 = jnp.bfloat16
U32 = jnp.uint32
EPS = 1e-5
LOG2E = 1.4426950408889634
NB = 4
LANES = 128

CFG = dict(OSPLIT=((2, 2), (4, 4), (7, 6)), DSPLIT=((2, 2), (4, 4), (6, 6)), NSTAGE=4, NSTRIP=6,
           LAG=3, RING=4, T=(0.4, -0.4, 1.2, -1.2))

TERMS = [term for i in range(NB) for term in (
    [("a", i, i)] + [("q", i, j) for j in range(NB) if j != i]
    + [("r", i, j) for j in range(i + 1, NB)] + [("b", i, i)])]


def _ln(x, gain=1.0):
    m = jnp.mean(x, axis=-1, keepdims=True)
    c = x - m
    v = jnp.mean(c * c, axis=-1, keepdims=True)
    return c * (jax.lax.rsqrt(v + EPS) * gain)


def _pack(x):
    return pltpu.bitcast(x.astype(BF16), U32)


def _unpack(x):
    return pltpu.bitcast(x, BF16)


def _dot(a, b):
    return jax.lax.dot_general(a, b, (((1,), (0,)), ((), ())), preferred_element_type=F32)


def _dot_nt(a, b):
    return jax.lax.dot_general(a, b, (((1,), (1,)), ((), ())), preferred_element_type=F32)


def _blocks(x):
    n = x.shape[1] // NB
    return [x[:, i * n:(i + 1) * n] for i in range(NB)]


def _right_terms(w):
    f = [[b.astype(F32) for b in row] for row in w]
    out = []
    for kind, i, j in TERMS:
        if kind == "q":
            val = w[i][j]
        elif kind == "r":
            val = f[i][j] + f[j][i]
        else:
            val = f[i][i]
            for k in range(NB):
                if k != i:
                    val = val - f[i][k] if kind == "a" else val + f[k][i]
        out.append(_pack(val))
    return out


def _run(*gens):
    gens = list(gens)
    while gens:
        for gen in list(gens):
            if next(gen, "done") == "done":
                gens.remove(gen)


def _make_kernel(S, D, H, E, M, T, F, cfg):
    OSPLIT, DSPLIT, NSTAGE, NSTRIP, LAG, RING, nodes = (
        cfg[k] for k in ("OSPLIT", "DSPLIT", "NSTAGE", "NSTRIP", "LAG", "RING", "T"))
    NSEG = S // T
    NG = H // NB
    DB = D // NB
    DC = 32
    NDC = DB // DC
    FC = NB * LANES
    NFC = F // FC
    SUB = 32
    L = M + T
    scale = float(E) ** -0.5

    def left_terms(s, d=None):
        if d is None:
            return {n: s[i] for n, (kind, i, _) in enumerate(TERMS) if kind == "a"}
        e = [[nodes[k] * s[i] + d[i] for i in range(NB)] for k in range(NB)]
        out = {}
        for n, (kind, i, j) in enumerate(TERMS):
            if kind == "a":
                out[n] = s[i]
            elif kind == "b":
                out[n] = e[i][i]
            elif kind == "q":
                out[n] = (e[j][i] - e[j][j]) * (1.0 / (nodes[j] - nodes[i]))
            else:
                out[n] = (e[i][i] - e[j][j]) * (1.0 / (nodes[i] - nodes[j]))
        return out

    def block_product(nl, left, right, acc=None):
        acc = [[None] * NB for _ in range(nl)] if acc is None else [list(row) for row in acc]

        def add(row, j, x):
            acc[row][j] = x if acc[row][j] is None else acc[row][j] + x

        for n, (kind, i, j) in enumerate(TERMS):
            if nl == 1:
                if kind in "aq":
                    p = _dot(left(TERMS.index(("a", i, i))), right(n))
                    add(0, i, p)
                    if kind == "q":
                        add(0, j, p)
                continue
            p = _dot(left(n), right(n))
            if kind == "a":
                u = p
            elif kind == "b":
                add(0, i, u)
                add(1, i, p - nodes[i] * u)
            else:
                u = u + p
                add(0, j, p)
                add(1, j, -nodes[i if kind == "q" else j] * p)
        return acc

    def long_product(nl, left, right, k0, k1, acc):
        width = cfg.get("W1", DB) if k1 - k0 == LANES else LANES
        tiles = range(DB // LANES)
        step = width // LANES
        out = []
        for c in tiles[::step]:
            old = None if acc is None else [
                [jnp.concatenate([acc[c + x][r][j] for x in range(step)], axis=1)
                 for j in range(NB)] for r in range(nl)]
            new = block_product(
                nl, lambda n: left(n, k0, k1),
                lambda n: _unpack(right[n, k0 // 2:k1 // 2, c * LANES:c * LANES + width]), old)
            out += [[[b[:, x * LANES:(x + 1) * LANES] for b in row] for row in new]
                    for x in range(step)]
        return out

    def row_blocks(tiles):
        return [jnp.concatenate([t[r][j] for j in range(NB) for t in tiles], axis=1)
                for r in range(len(tiles[0]))]

    def scope(name):
        return jax.named_scope("S_" + name) if cfg.get("SCOPES") else contextlib.nullcontext()

    def mask_tables(nl):
        r = jax.lax.broadcasted_iota(jnp.int32, (nl * L, nl * L), 0)
        c = jax.lax.broadcasted_iota(jnp.int32, (nl * L, nl * L), 1)
        same = (r < L) == (c < L)
        vis = same & ((jnp.where(r < L, r, r - L) < M) | (c <= r))
        return vis, jnp.where(same, -1e9 * LOG2E, -jnp.inf).astype(F32)

    def kernel(x_hbm, mem_ref, wq_hbm, wk_hbm, wv_hbm, wo_hbm, wg_hbm, wu_hbm, wd_hbm, out_hbm,
               wqkv, wo, wgu, wd, st_qkv, st_row, st_col, x_v,
               h_s, o_s, hb_s, a_s, mem_s, ya_s, yb_s, z_s,
               sem_qkv, sem_row, sem_col, sem_x, sem_out):
        def qkv_copy(which, i):
            return pltpu.make_async_copy((wq_hbm, wk_hbm, wv_hbm)[which].at[:, i % NDC],
                                         st_qkv.at[i % NSTAGE], sem_qkv.at[i % NSTAGE])

        def qkv_start(i):
            for which in range(3):
                pl.when(i // NDC == which)(qkv_copy(which, i).start)

        def row_copy(src, i):
            return pltpu.make_async_copy(src.at[i], st_row.at[i], sem_row.at[i])

        def gu_copy(which, c):
            slot = (2 * c + which) % NSTRIP
            cols = pl.ds(pl.multiple_of(c * FC, FC), FC)
            return pltpu.make_async_copy((wg_hbm, wu_hbm)[which].at[:, cols],
                                         st_col.at[slot], sem_col.at[slot])

        def convert(src, dst, row0):
            n = src.shape[0] // NB

            def body(r, carry):
                w = [_blocks(src[pl.ds(pl.multiple_of(i * n + r * SUB, SUB), SUB), :])
                     for i in range(NB)]
                rows = pl.ds(pl.multiple_of((row0 + r * SUB) // 2, SUB // 2), SUB // 2)
                for k, val in enumerate(_right_terms(w)):
                    dst[k, rows, :] = val
                return carry
            jax.lax.fori_loop(0, n // SUB, body, 0)

        def convert_qkv(i):
            qkv_copy(0, i).wait()
            words = [st_qkv.at[i % NSTAGE, b].bitcast(U32) for b in range(NB)]
            rows = pl.ds(pl.multiple_of((i % NDC) * (DC // 2), DC // 2), DC // 2)
            for g in range(NG):
                w = []
                for src in words:
                    w.append([])
                    for pair in range(g * NB // 2, (g + 1) * NB // 2):
                        a = src[pl.ds(pair, DC // 2, stride=H), :]
                        b = src[pl.ds(H // 2 + pair, DC // 2, stride=H), :]
                        w[-1].append(_unpack((a & np.uint32(0xFFFF)) | (b << 16)))
                        w[-1].append(_unpack((a >> 16) | (b & np.uint32(0xFFFF0000))))
                for k, val in enumerate(_right_terms(w)):
                    wqkv[i // NDC, g, k, rows, :] = val

        def convert_gu(c):
            for which in range(2):
                gu_copy(which, c).wait()
                convert(st_col.at[(2 * c + which) % NSTRIP], wgu.at[which, c], 0)
            pending = c + NSTRIP // 2

            @pl.when(pending < NFC)
            def _():
                for which in range(2):
                    gu_copy(which, pending).start()

            for j in range(2):
                piece = 2 * (pending - NFC) + j
                pl.when((piece >= 0) & (piece < NFC))(
                    row_copy(wd_hbm, jnp.clip(piece, 0, NFC - 1)).start)

        x_head = pltpu.make_async_copy(x_hbm.at[0:LAG + 2], x_v.at[0:LAG + 2], sem_x.at[0])
        x_rest = pltpu.make_async_copy(x_hbm.at[LAG + 2:NSEG], x_v.at[LAG + 2:NSEG], sem_x.at[1])

        def out_copy(i, lo, hi):
            return pltpu.make_async_copy(x_v.at[lo:hi], out_hbm.at[lo:hi], sem_out.at[i])

        def x_seg(seg):
            return x_v[seg].astype(F32)

        def set_rows(*blocks):
            for j, (mem, _) in enumerate(blocks):
                mem_s[j] = mem
            parts = [_blocks(jnp.concatenate(blk, axis=0)) for blk in blocks]
            for n, a in left_terms(*parts).items():
                h_s[n] = a

        def attention_ops(nl, finish):
            vis, fill = mask_tables(nl)

            def proj(g):
                res = []
                for j in (1, 0, 2):
                    c = block_product(nl, h_s.__getitem__, lambda n: _unpack(wqkv[j, g, n]))
                    res.append([jnp.concatenate([row[h] for row in c], axis=0).astype(BF16)
                                for h in range(NB)])
                return res

            def attend(s, v):
                s = jnp.where(vis, s * (scale * LOG2E), fill)
                p = jnp.exp2(s - jnp.max(s, axis=-1, keepdims=True))
                tot = jnp.sum(p, axis=-1, keepdims=True)
                inv = pl.reciprocal(tot, approx=True)
                inv = inv * (2.0 - tot * inv)
                return _dot(p, v) * inv

            def out_proj(g0, g1, acc):
                return long_product(nl, lambda n, a, b: o_s[n, :, a:b], wo, g0 * E, g1 * E, acc)

            k, q, v = proj(0)
            acc, done = None, 0
            for g in range(NG):
                ss = [_dot_nt(q[h], k[h]) for h in range(NB)]
                for at, upto in OSPLIT:
                    if at == g:
                        acc, done = out_proj(done, upto, acc), upto
                if g + 1 < NG:
                    nxt = proj(g + 1)
                o = [attend(ss[h], v[h]) for h in range(NB)]
                parts = [[x[j * L:(j + 1) * L] for x in o] for j in range(nl)]
                for n, a in left_terms(*parts).items():
                    o_s[n, :, g * E:(g + 1) * E] = a
                k, q, v = nxt
            yield
            finish(row_blocks(out_proj(done, NG, acc)))

        def set_glu_rows(top, bot):
            for n, a in left_terms(_blocks(_ln(top, 0.5)), _blocks(_ln(bot, 0.5))).items():
                hb_s[n, 0:top.shape[0] // 2, :] = _pack(a)

        def glu_ops(rows, finish, before_down=None):
            def gate_up(c):
                g, u = (block_product(2, lambda n: _unpack(hb_s[n, 0:rows // 2, :]),
                                      lambda n: _unpack(wgu[j, c, n])) for j in range(2))
                act = [[jnp.tanh(x) * y + y for x, y in zip(gr, ur)] for gr, ur in zip(g, u)]
                for n, a in left_terms(*act).items():
                    a_s[n, 0:rows // 2, c * LANES:(c + 1) * LANES] = _pack(a)

            def down(c0, c1, acc):
                return long_product(2, lambda n, a, b: _unpack(a_s[n, 0:rows // 2, a:b]), wd,
                                    c0 * LANES, c1 * LANES, acc)

            acc, done = None, 0
            for c in range(NFC):
                gate_up(c)
                if c == 0:
                    yield
                if before_down is not None and c + 1 == NFC:
                    before_down()
                for at, upto in (DSPLIT if before_down is None else DSPLIT[-1:]):
                    if at == c:
                        acc, done = down(done, upto, acc), upto
            finish(row_blocks(down(done, NFC, acc)))

        x_head.start()
        for i in range(NSTAGE):
            qkv_copy(0, i).start()

        @pl.loop(0, 3 * NDC)
        def _(i):
            with scope("q"):
                convert_qkv(i)
            qkv_start(i + NSTAGE)
            piece = i + NSTAGE - 3 * NDC
            pl.when(piece >= 0)(row_copy(wo_hbm, jnp.maximum(piece, 0)).start)

        @pl.loop(0, NG)
        def _(g):
            with scope("o"):
                row_copy(wo_hbm, g).wait()
                convert(st_row.at[g], wo, g * E)
            pl.when(g + NSTAGE < NG)(row_copy(wo_hbm, jnp.minimum(g + NSTAGE, NG - 1)).start)
            strip = g + NSTAGE - NG
            for which in range(2):
                pl.when((strip >= 0) & (strip % 2 == which))(
                    gu_copy(which, jnp.maximum(strip, 0) // 2).start)

        for strip in range(NSTAGE, NSTRIP):
            gu_copy(strip % 2, strip // 2).start()

        x_head.wait()
        mem0 = mem_ref[...].astype(F32)
        set_rows((mem0, _ln(x_seg(0))))
        per_step = cfg.get("NEARLY", 2)

        @pl.loop(0, LAG)
        def _(t):
            def finish(acc):
                z_s[t] = x_seg(t) + acc[0][M:]
                set_rows((acc[0][:M], _ln(x_seg(t + 1))))

            with scope("head"):
                _run(attention_ops(1, finish))
            with scope("g"):
                pl.loop(t * per_step, jnp.where(t + 1 < LAG, (t + 1) * per_step, NFC))(convert_gu)

        set_glu_rows(z_s[0], z_s[1])

        def head_down():
            for piece in range(NSTRIP, NFC):
                row_copy(wd_hbm, piece).start()

            @pl.loop(0, NFC)
            def _(c):
                with scope("d"):
                    row_copy(wd_hbm, c).wait()
                    convert(st_row.at[c], wd, c * LANES)
            x_rest.start()

        def head_glu_finish(d):
            z_s[0] = z_s[0] + d[0]
            z_s[1] = z_s[1] + d[1]

        _run(glu_ops(T, head_glu_finish, head_down))
        ya_s[0] = z_s[LAG - 1]
        ya_s[1] = z_s[LAG - 1]
        set_rows((mem_s[0], _ln(x_seg(LAG))), (mem0, _ln(z_s[0])))

        def take_rows():
            top, bot = ya_s[0], ya_s[1]
            yb_s[0] = top
            yb_s[1] = bot
            set_glu_rows(top, bot)

        def step(t):
            pl.when(t == LAG + 1)(x_rest.wait)
            take_rows()

            def att_finish(acc):
                ya_s[0] = x_seg(t) + acc[0][M:]
                ya_s[1] = z_s[(t - LAG) % RING] + acc[1][M:]
                set_rows((acc[0][:M], _ln(x_seg(jnp.minimum(t + 1, NSEG - 1)))),
                         (acc[1][:M], _ln(z_s[(t + 1 - LAG) % RING])))

            def glu_finish(d):
                z_s[(t - 1) % RING] = yb_s[0] + d[0]
                x_v[jnp.maximum(t - 1 - LAG, 0)] = (yb_s[1] + d[1]).astype(BF16)

            _run(attention_ops(2, att_finish), glu_ops(T, glu_finish))

        with scope("main"):
            pl.loop(LAG, cfg.get("NSTEP", NSEG))(step)
        out_copy(0, 0, NSEG - 1 - LAG).start()

        def mid_finish(d):
            z_s[(NSEG - 1) % RING] = yb_s[0] + d[0]
            x_v[NSEG - 1 - LAG] = (yb_s[1] + d[1]).astype(BF16)

        take_rows()
        set_rows((mem_s[1], _ln(z_s[(NSEG - LAG) % RING])))
        _run(glu_ops(T, mid_finish))

        @pl.loop(NSEG - LAG, NSEG)
        def _(t):
            def finish(acc):
                tok = _ln(z_s[jnp.minimum(t + 1, NSEG - 1) % RING])
                z_s[t % RING] = z_s[t % RING] + acc[0][M:]
                set_rows((acc[0][:M], tok))

            with scope("tail"):
                _run(attention_ops(1, finish))

        def last_rows():
            y = jnp.concatenate([z_s[t % RING] for t in range(NSEG - LAG, NSEG)], axis=0)
            return y[:LAG * T // 2], y[LAG * T // 2:]

        def last_finish(d):
            z = jnp.concatenate([y + x for y, x in zip(last_rows(), d)], axis=0).astype(BF16)
            for j in range(LAG):
                x_v[NSEG - LAG + j] = z[j * T:(j + 1) * T]

        set_glu_rows(*last_rows())
        with scope("lglu"):
            _run(glu_ops(LAG * T // 2, last_finish))
        out_copy(1, NSEG - 1 - LAG, NSEG).start()
        out_copy(0, 0, NSEG - 1 - LAG).wait()
        out_copy(1, NSEG - 1 - LAG, NSEG).wait()

    dma = pltpu.SemaphoreType.DMA
    nt = len(TERMS)
    scratch = [
        pltpu.VMEM((3, NG, nt, DB // 2, E), U32),
        pltpu.VMEM((nt, NG * E // 2, DB), U32),
        pltpu.VMEM((2, NFC, nt, DB // 2, LANES), U32),
        pltpu.VMEM((nt, NFC * LANES // 2, DB), U32),
        pltpu.VMEM((NSTAGE, NB, DC * H, E), BF16),
        pltpu.VMEM((NG, FC, D), BF16),
        pltpu.VMEM((NSTRIP, D, FC), BF16),
        pltpu.VMEM((NSEG, T, D), BF16),
        pltpu.VMEM((nt, L, DB), F32),
        pltpu.VMEM((nt, L, NG * E), F32),
        pltpu.VMEM((nt, LAG * T // 4, DB), U32),
        pltpu.VMEM((nt, LAG * T // 4, NFC * LANES), U32),
        pltpu.VMEM((2, M, D), F32),
        pltpu.VMEM((2, T, D), F32),
        pltpu.VMEM((2, T, D), F32),
        pltpu.VMEM((RING, T, D), F32),
        dma((NSTAGE,)), dma((NG,)), dma((NSTRIP,)), dma((2,)), dma((2,)),
    ]
    return kernel, scratch, (NB, NDC, DC * H, E)


def build(cfg):
    @functools.partial(jax.jit, static_argnames=("A_seg_len",))
    def fn(A_x, A_mem0, A_Wq, A_Wk, A_Wv, A_Wo, A_seg_len, B_x, B_w_gate, B_w_up, B_w_down):
        del B_x
        B, S, D = A_x.shape
        _, H, E = A_Wq.shape
        M = A_mem0.shape[1]
        F = B_w_gate.shape[1]
        T = int(A_seg_len)
        FC = NB * LANES
        kernel, scratch, qkv_shape = _make_kernel(S, D, H, E, M, T, F, cfg)
        hbm = pl.BlockSpec(memory_space=pl.ANY)
        out = pl.pallas_call(
            kernel,
            out_shape=jax.ShapeDtypeStruct((S // T, T, D), A_x.dtype),
            in_specs=[hbm, pl.BlockSpec(memory_space=pltpu.VMEM)] + [hbm] * 7,
            out_specs=hbm,
            scratch_shapes=scratch,
            compiler_params=pltpu.CompilerParams(vmem_limit_bytes=126 * 1024 * 1024,
                                                 flags=cfg.get("flags")),
        )(A_x.reshape(S // T, T, D), A_mem0.reshape(M, D),
          A_Wq.reshape(qkv_shape), A_Wk.reshape(qkv_shape), A_Wv.reshape(qkv_shape),
          A_Wo.reshape(H * E // FC, FC, D), B_w_gate, B_w_up, B_w_down.reshape(F // FC, FC, D))
        return out.reshape(B, S, D)

    return fn


pallas_interleave_layers__memory_aug_recurrent_mem_tr__glu_gated_glu__prompt_kernel = build(CFG)
```

```python
import contextlib
import functools

import jax
import jax.numpy as jnp
import numpy as np
import jax.experimental.pallas as pl
import jax.experimental.pallas.tpu as pltpu

F32 = jnp.float32
BF16 = jnp.bfloat16
U32 = jnp.uint32
EPS = 1e-5
LOG2E = 1.4426950408889634
NB = 4
LANES = 128

CFG = dict(OSPLIT=((3, 2), (5, 4), (7, 6)), DSPLIT=((2, 1), (4, 3), (6, 5)), NSTAGE=4, NSTRIP=4,
           LAG=3, RING=4, ORDER="0000000010100", UNROLL=1)

NODES = (0.5, -0.5, 1.5, -1.5)
TERMS = [term for i in range(NB) for term in (
    [("a", i, i)] + [("q", i, j) for j in range(NB) if j != i]
    + [("r", i, j) for j in range(i + 1, NB)] + [("b", i, i)])]


def _q_gains(i, j):
    gain = 1.0 / (NODES[j] - NODES[i])
    return (1.0, gain) if np.frexp(abs(gain))[0] == 0.5 else (gain, 1.0)


def _scaled(x, gain):
    return x if gain == 1.0 else x * gain


def _ln(x, gain=1.0):
    m = jnp.mean(x, axis=-1, keepdims=True)
    c = x - m
    v = jnp.mean(c * c, axis=-1, keepdims=True)
    return c * (jax.lax.rsqrt(v + EPS) * gain)


def _interleave(even, odd):
    return pltpu.bitcast(pltpu.pack_elementwise([even, odd], packed_dtype=BF16), U32)


def _low(words):
    return pltpu.bitcast(words << 16, F32)


def _high(words):
    return pltpu.bitcast(words & np.uint32(0xFFFF0000), F32)


def _unpack(x):
    return pltpu.bitcast(x, BF16)


def _dot(a, b):
    return jax.lax.dot_general(a, b, (((1,), (0,)), ((), ())), preferred_element_type=F32)


def _dot_nt(a, b):
    return jax.lax.dot_general(a, b, (((1,), (1,)), ((), ())), preferred_element_type=F32)


def _blocks(x):
    n = x.shape[1] // NB
    return [x[:, i * n:(i + 1) * n] for i in range(NB)]


def _right_terms(even, odd):
    def term(w, kind, i, j):
        if kind == "q":
            return _scaled(w[i][j], _q_gains(i, j)[1])
        if kind == "r":
            return _scaled(w[i][j] + w[j][i], 1.0 / (NODES[i] - NODES[j]))
        val = w[i][i]
        for k in range(NB):
            if k != i:
                val = val - w[i][k] if kind == "a" else val + w[k][i]
        return val
    return [_interleave(term(even, *t), term(odd, *t)) for t in TERMS]


def _run(*gens, order=""):
    for which in order:
        next(gens[int(which)], None)
    for gen in gens:
        for _ in gen:
            pass


def _make_kernel(S, D, H, E, M, T, F, cfg):
    OSPLIT, DSPLIT, NSTAGE, NSTRIP, LAG, RING = (
        cfg[k] for k in ("OSPLIT", "DSPLIT", "NSTAGE", "NSTRIP", "LAG", "RING"))
    nodes = NODES
    NSEG = S // T
    NG = H // NB
    DB = D // NB
    DC = 32
    NDC = DB // DC
    FC = NB * LANES
    NFC = F // FC
    SUB = 128
    L = M + T
    scale = float(E) ** -0.5

    def left_terms(s, d=None):
        if d is None:
            return {n: s[i] for n, (kind, i, _) in enumerate(TERMS) if kind == "a"}
        ts = {t: [t * x for x in s] for t in nodes if t > 0}
        e = [[d[i] + ts[t][i] if t > 0 else d[i] - ts[-t][i] for i in range(NB)] for t in nodes]
        out = {}
        for n, (kind, i, j) in enumerate(TERMS):
            if kind == "a":
                out[n] = s[i]
            elif kind == "b":
                out[n] = e[i][i]
            elif kind == "q":
                out[n] = _scaled(e[j][i] - e[j][j], _q_gains(i, j)[0])
            else:
                out[n] = e[i][i] - e[j][j]
        return out

    def block_product(nl, left, right, acc=None):
        acc = [[None] * NB for _ in range(nl)] if acc is None else [list(row) for row in acc]

        def add(row, j, x):
            acc[row][j] = x if acc[row][j] is None else acc[row][j] + x

        for n, (kind, i, j) in enumerate(TERMS):
            if nl == 1:
                if kind in "aq":
                    p = _dot(left(TERMS.index(("a", i, i))), right(n))
                    if kind == "q":
                        p = _scaled(p, 1.0 / _q_gains(i, j)[1])
                    add(0, i, p)
                    if kind == "q":
                        add(0, j, p)
                continue
            p = _dot(left(n), right(n))
            if kind == "a":
                u = p
            elif kind == "b":
                add(0, i, u)
                add(1, i, p - nodes[i] * u)
            else:
                u = u + p
                add(0, j, p)
                add(1, j, -nodes[i if kind == "q" else j] * p)
        return acc

    def long_product(nl, left, right, k0, k1, acc):
        width = cfg.get("W1", DB) if k1 - k0 == LANES else LANES
        tiles = range(DB // LANES)
        step = width // LANES
        out = []
        for c in tiles[::step]:
            old = None if acc is None else [
                [jnp.concatenate([acc[c + x][r][j] for x in range(step)], axis=1)
                 for j in range(NB)] for r in range(nl)]
            new = block_product(
                nl, lambda n: left(n, k0, k1),
                lambda n: _unpack(right[n, k0 // 2:k1 // 2, c * LANES:c * LANES + width]), old)
            out += [[[b[:, x * LANES:(x + 1) * LANES] for b in row] for row in new]
                    for x in range(step)]
        return out

    def row_blocks(tiles):
        return [jnp.concatenate([t[r][j] for j in range(NB) for t in tiles], axis=1)
                for r in range(len(tiles[0]))]

    def scope(name):
        return jax.named_scope("S_" + name) if cfg.get("SCOPES") and name in cfg.get("WHICH", [name]) else contextlib.nullcontext()

    def mask_tables(nl):
        r = jax.lax.broadcasted_iota(jnp.int32, (nl * L, nl * L), 0)
        c = jax.lax.broadcasted_iota(jnp.int32, (nl * L, nl * L), 1)
        same = (r < L) == (c < L)
        vis = same & ((jnp.where(r < L, r, r - L) < M) | (c <= r))
        return vis, jnp.where(same, -1e9 * LOG2E, -jnp.inf).astype(F32)

    def kernel(x_hbm, mem_ref, wq_hbm, wk_hbm, wv_hbm, wo_hbm, wg_hbm, wu_hbm, wd_hbm, out_hbm,
               wqkv, wo, wgu, wd, st_qkv, st_row, st_col, x_v,
               h_s, o_s, hb_s, a_s, mem_s, ya_s, yb_s, z_s,
               sem_qkv, sem_row, sem_col, sem_x, sem_out):
        def qkv_copy(which, i):
            return pltpu.make_async_copy((wq_hbm, wk_hbm, wv_hbm)[which].at[:, i % NDC],
                                         st_qkv.at[i % NSTAGE], sem_qkv.at[i % NSTAGE])

        def qkv_start(i):
            for which in range(3):
                pl.when(i // NDC == which)(qkv_copy(which, i).start)

        def row_copy(src, i):
            return pltpu.make_async_copy(src.at[i], st_row.at[i], sem_row.at[i])

        def gu_copy(which, c):
            slot = (2 * c + which) % NSTRIP
            cols = pl.ds(pl.multiple_of(c * FC, FC), FC)
            return pltpu.make_async_copy((wg_hbm, wu_hbm)[which].at[:, cols],
                                         st_col.at[slot], sem_col.at[slot])

        def convert(src, dst, row0):
            n = src.shape[0] // NB
            sub = SUB * LANES * NB // src.shape[1]

            @pl.loop(0, n // sub)
            def _(r):
                w = [pltpu.bitcast(src[pl.ds(pl.multiple_of(i * n + r * sub, sub), sub), :], U32)
                     for i in range(NB)]
                rows = pl.ds(pl.multiple_of((row0 + r * sub) // 2, sub // 2), sub // 2)
                for k, val in enumerate(_right_terms([_blocks(_low(x)) for x in w],
                                                     [_blocks(_high(x)) for x in w])):
                    dst[k, rows, :] = val

        def convert_qkv(i):
            qkv_copy(0, i).wait()
            words = [st_qkv.at[i % NSTAGE, b].bitcast(U32) for b in range(NB)]
            rows = pl.ds(pl.multiple_of((i % NDC) * (DC // 2), DC // 2), DC // 2)
            span = (DC - 1) * H // 2 + NB

            @pl.loop(0, NG // 2)
            def _(gg):
                views = [w.at[pl.ds(pl.multiple_of(gg * NB, NB), span)] for w in words]
                for g in range(2):
                    def heads(src, parity):
                        pairs = [src[pl.ds(parity * H // 2 + p, DC // 2, stride=H), :]
                                 for p in range(g * NB // 2, (g + 1) * NB // 2)]
                        return [half(x) for x in pairs for half in (_low, _high)]
                    for k, val in enumerate(_right_terms(
                            *([heads(src, parity) for src in views] for parity in range(2)))):
                        wqkv[i // NDC, 2 * gg + g, k, rows, :] = val

        def convert_gu(c):
            for which in range(2):
                gu_copy(which, c).wait()
                convert(st_col.at[(2 * c + which) % NSTRIP], wgu.at[which, c], 0)
            pending = c + NSTRIP // 2

            @pl.when(pending < NFC)
            def _():
                for which in range(2):
                    gu_copy(which, pending).start()

            for j in range(2):
                piece = 2 * (pending - NFC) + j
                pl.when((piece >= 0) & (piece < NFC))(
                    row_copy(wd_hbm, jnp.clip(piece, 0, NFC - 1)).start)

        x_head = pltpu.make_async_copy(x_hbm.at[0:LAG + 2], x_v.at[0:LAG + 2], sem_x.at[0])
        x_rest = pltpu.make_async_copy(x_hbm.at[LAG + 2:NSEG], x_v.at[LAG + 2:NSEG], sem_x.at[1])

        def out_copy(i, lo, hi):
            return pltpu.make_async_copy(x_v.at[lo:hi], out_hbm.at[lo:hi], sem_out.at[i])

        def x_seg(seg):
            return x_v[seg].astype(F32)

        def set_rows(*blocks):
            for j, (mem, _) in enumerate(blocks):
                mem_s[j] = mem
            parts = [_blocks(jnp.concatenate(blk, axis=0)) for blk in blocks]
            for n, a in left_terms(*parts).items():
                h_s[n] = a

        def attention_ops(nl, finish):
            vis, fill = mask_tables(nl)

            def proj(g):
                res = []
                for j in (1, 0, 2):
                    c = block_product(nl, h_s.__getitem__, lambda n: _unpack(wqkv[j, g, n]))
                    res.append([jnp.concatenate([row[h] for row in c], axis=0).astype(BF16)
                                for h in range(NB)])
                return res

            def attend(s, v):
                s = jnp.where(vis, s * (scale * LOG2E), fill)
                p = jnp.exp2(s - jnp.max(s, axis=-1, keepdims=True))
                tot = jnp.sum(p, axis=-1, keepdims=True)
                inv = pl.reciprocal(tot, approx=True)
                inv = inv * (2.0 - tot * inv)
                return _dot(p, v) * inv

            def out_proj(g0, g1, acc):
                return long_product(nl, lambda n, a, b: o_s[n, :, a:b], wo, g0 * E, g1 * E, acc)

            k, q, v = proj(0)
            acc, done = None, 0
            for g in range(NG):
                ss = [_dot_nt(q[h], k[h]) for h in range(NB)]
                for at, upto in OSPLIT:
                    if at == g:
                        acc, done = out_proj(done, upto, acc), upto
                if g + 1 < NG:
                    nxt = proj(g + 1)
                else:
                    yield
                o = [attend(ss[h], v[h]) for h in range(NB)]
                parts = [[x[j * L:(j + 1) * L] for x in o] for j in range(nl)]
                for n, a in left_terms(*parts).items():
                    o_s[n, :, g * E:(g + 1) * E] = a
                k, q, v = nxt
                yield
            finish(row_blocks(out_proj(done, NG, acc)))

        def set_glu_rows(top, bot):
            for n, a in left_terms(_blocks(_ln(top, 0.5)), _blocks(_ln(bot, 0.5))).items():
                hb_s[n, 0:top.shape[0], :] = a

        def glu_ops(rows, finish, before_down=None):
            def gate_up(c):
                g, u = (block_product(2, lambda n: hb_s[n, 0:rows, :],
                                      lambda n: _unpack(wgu[j, c, n])) for j in range(2))
                act = [[jnp.tanh(x) * y + y for x, y in zip(gr, ur)] for gr, ur in zip(g, u)]
                for n, a in left_terms(*act).items():
                    a_s[n, 0:rows, c * LANES:(c + 1) * LANES] = a

            def down(c0, c1, acc):
                return long_product(2, lambda n, a, b: a_s[n, 0:rows, a:b], wd,
                                    c0 * LANES, c1 * LANES, acc)

            acc, done = None, 0
            for c in range(NFC):
                gate_up(c)
                if before_down is not None and c + 1 == NFC:
                    before_down()
                for at, upto in (DSPLIT if before_down is None else DSPLIT[-1:]):
                    if at == c:
                        acc, done = down(done, upto, acc), upto
                yield
            finish(row_blocks(down(done, NFC, acc)))

        x_head.start()
        for i in range(NSTAGE):
            qkv_copy(0, i).start()

        @pl.loop(0, 3 * NDC)
        def _(i):
            with scope("q"):
                convert_qkv(i)
            qkv_start(i + NSTAGE)
            piece = i + NSTAGE - 3 * NDC
            pl.when(piece >= 0)(row_copy(wo_hbm, jnp.maximum(piece, 0)).start)

        @pl.loop(0, NG)
        def _(g):
            with scope("o"):
                row_copy(wo_hbm, g).wait()
                convert(st_row.at[g], wo, g * E)
            pl.when(g + NSTAGE < NG)(row_copy(wo_hbm, jnp.minimum(g + NSTAGE, NG - 1)).start)
            strip = g + NSTAGE - NG
            for which in range(2):
                pl.when((strip >= 0) & (strip % 2 == which))(
                    gu_copy(which, jnp.maximum(strip, 0) // 2).start)

        for strip in range(NSTAGE, NSTRIP):
            gu_copy(strip % 2, strip // 2).start()

        x_head.wait()
        mem0 = mem_ref[...].astype(F32)
        set_rows((mem0, _ln(x_seg(0))))
        per_step = cfg.get("NEARLY", 2)

        @pl.loop(0, LAG)
        def _(t):
            def finish(acc):
                z_s[t] = x_seg(t) + acc[0][M:]
                set_rows((acc[0][:M], _ln(x_seg(t + 1))))

            with scope("head"):
                _run(attention_ops(1, finish))
            with scope("g"):
                pl.loop(t * per_step, jnp.where(t + 1 < LAG, (t + 1) * per_step, NFC))(convert_gu)

        set_glu_rows(z_s[0], z_s[1])

        def head_down():
            for piece in range(NSTRIP, NFC):
                row_copy(wd_hbm, piece).start()

            @pl.loop(0, NFC)
            def _(c):
                with scope("d"):
                    row_copy(wd_hbm, c).wait()
                    convert(st_row.at[c], wd, c * LANES)
            x_rest.start()

        def head_glu_finish(d):
            z_s[0] = z_s[0] + d[0]
            z_s[1] = z_s[1] + d[1]

        _run(glu_ops(T, head_glu_finish, head_down))
        ya_s[0] = z_s[LAG - 1]
        ya_s[1] = z_s[LAG - 1]
        set_rows((mem_s[0], _ln(x_seg(LAG))), (mem0, _ln(z_s[0])))

        def take_rows():
            top, bot = ya_s[0], ya_s[1]
            yb_s[0] = top
            yb_s[1] = bot
            set_glu_rows(top, bot)

        def step(t):
            take_rows()

            def att_finish(acc):
                ya_s[0] = x_seg(t) + acc[0][M:]
                ya_s[1] = z_s[(t - LAG) % RING] + acc[1][M:]
                set_rows((acc[0][:M], _ln(x_seg(jnp.minimum(t + 1, NSEG - 1)))),
                         (acc[1][:M], _ln(z_s[(t + 1 - LAG) % RING])))

            def glu_finish(d):
                z_s[(t - 1) % RING] = yb_s[0] + d[0]
                x_v[jnp.maximum(t - 1 - LAG, 0)] = (yb_s[1] + d[1]).astype(BF16)

            _run(attention_ops(2, att_finish), glu_ops(T, glu_finish), order=cfg["ORDER"])

        with scope("main"):
            @pl.loop(0, (cfg.get("NSTEP", NSEG) - LAG) // cfg["UNROLL"])
            def _(i):
                pl.when(i == (cfg["UNROLL"] == 1))(x_rest.wait)
                for j in range(cfg["UNROLL"]):
                    step(LAG + i * cfg["UNROLL"] + j)
        out_copy(0, 0, NSEG - 1 - LAG).start()

        def mid_finish(d):
            z_s[(NSEG - 1) % RING] = yb_s[0] + d[0]
            x_v[NSEG - 1 - LAG] = (yb_s[1] + d[1]).astype(BF16)

        take_rows()
        set_rows((mem_s[1], _ln(z_s[(NSEG - LAG) % RING])))
        _run(glu_ops(T, mid_finish))

        @pl.loop(NSEG - LAG, NSEG)
        def _(t):
            def finish(acc):
                tok = _ln(z_s[jnp.minimum(t + 1, NSEG - 1) % RING])
                z_s[t % RING] = z_s[t % RING] + acc[0][M:]
                set_rows((acc[0][:M], tok))

            with scope("tail"):
                _run(attention_ops(1, finish))

        def last_rows():
            y = jnp.concatenate([z_s[t % RING] for t in range(NSEG - LAG, NSEG)], axis=0)
            return y[:LAG * T // 2], y[LAG * T // 2:]

        def last_finish(d):
            z = jnp.concatenate([y + x for y, x in zip(last_rows(), d)], axis=0).astype(BF16)
            for j in range(LAG):
                x_v[NSEG - LAG + j] = z[j * T:(j + 1) * T]

        set_glu_rows(*last_rows())
        with scope("lglu"):
            _run(glu_ops(LAG * T // 2, last_finish))
        out_copy(1, NSEG - 1 - LAG, NSEG).start()
        out_copy(0, 0, NSEG - 1 - LAG).wait()
        out_copy(1, NSEG - 1 - LAG, NSEG).wait()

    dma = pltpu.SemaphoreType.DMA
    nt = len(TERMS)
    scratch = [
        pltpu.VMEM((3, NG, nt, DB // 2, E), U32),
        pltpu.VMEM((nt, NG * E // 2, DB), U32),
        pltpu.VMEM((2, NFC, nt, DB // 2, LANES), U32),
        pltpu.VMEM((nt, NFC * LANES // 2, DB), U32),
        pltpu.VMEM((NSTAGE, NB, DC * H, E), BF16),
        pltpu.VMEM((NG, FC, D), BF16),
        pltpu.VMEM((NSTRIP, D, FC), BF16),
        pltpu.VMEM((NSEG, T, D), BF16),
        pltpu.VMEM((nt, L, DB), F32),
        pltpu.VMEM((nt, L, NG * E), F32),
        pltpu.VMEM((nt, LAG * T // 2, DB), F32),
        pltpu.VMEM((nt, LAG * T // 2, NFC * LANES), F32),
        pltpu.VMEM((2, M, D), F32),
        pltpu.VMEM((2, T, D), F32),
        pltpu.VMEM((2, T, D), F32),
        pltpu.VMEM((RING, T, D), F32),
        dma((NSTAGE,)), dma((NG,)), dma((NSTRIP,)), dma((2,)), dma((2,)),
    ]
    return kernel, scratch, (NB, NDC, DC * H, E)


def build(cfg):
    @functools.partial(jax.jit, static_argnames=("A_seg_len",))
    def fn(A_x, A_mem0, A_Wq, A_Wk, A_Wv, A_Wo, A_seg_len, B_x, B_w_gate, B_w_up, B_w_down):
        del B_x
        B, S, D = A_x.shape
        _, H, E = A_Wq.shape
        M = A_mem0.shape[1]
        F = B_w_gate.shape[1]
        T = int(A_seg_len)
        FC = NB * LANES
        kernel, scratch, qkv_shape = _make_kernel(S, D, H, E, M, T, F, cfg)
        hbm = pl.BlockSpec(memory_space=pl.ANY)
        out = pl.pallas_call(
            kernel,
            out_shape=jax.ShapeDtypeStruct((S // T, T, D), A_x.dtype),
            in_specs=[hbm, pl.BlockSpec(memory_space=pltpu.VMEM)] + [hbm] * 7,
            out_specs=hbm,
            scratch_shapes=scratch,
            compiler_params=pltpu.CompilerParams(vmem_limit_bytes=126 * 1024 * 1024,
                                                 flags=cfg.get("flags")),
        )(A_x.reshape(S // T, T, D), A_mem0.reshape(M, D),
          A_Wq.reshape(qkv_shape), A_Wk.reshape(qkv_shape), A_Wv.reshape(qkv_shape),
          A_Wo.reshape(H * E // FC, FC, D), B_w_gate, B_w_up, B_w_down.reshape(F // FC, FC, D))
        return out.reshape(B, S, D)

    return fn


pallas_interleave_layers__memory_aug_recurrent_mem_tr__glu_gated_glu__prompt_kernel = build(CFG)
```

```python
import contextlib
import functools

import jax
import jax.numpy as jnp
import numpy as np
import jax.experimental.pallas as pl
import jax.experimental.pallas.tpu as pltpu

F32 = jnp.float32
BF16 = jnp.bfloat16
U32 = jnp.uint32
EPS = 1e-5
LOG2E = 1.4426950408889634
NB = 4
LANES = 128

CFG = dict(OSPLIT=((3, 2), (5, 4), (7, 6)), DSPLIT=((2, 1), (4, 3), (6, 5)), NSTAGE=4, NSTRIP=6,
           LAG=3, RING=4, ORDER="11111111010111", CUT=7, DCUT={"0": 3, "3": 7})

NODES = (0.5, -0.5, 1.5, -1.5)
TERMS = [term for i in range(NB) for term in (
    [("a", i, i)] + [("q", i, j) for j in range(NB) if j != i]
    + [("r", i, j) for j in range(i + 1, NB)] + [("b", i, i)])]


def _gains(kind, i, j):
    gain = 1.0 / (NODES[j] - NODES[i]) if kind == "q" else 1.0 / (NODES[i] - NODES[j])
    right = abs(gain) if kind == "r" or np.frexp(abs(gain))[0] == 0.5 else 1.0
    return gain / right, right


def _difference(x, y, gain):
    return _scaled(x - y if gain > 0 else y - x, abs(gain))


def _scaled(x, gain):
    return x if gain == 1.0 else x * gain


def _ln(x, gain=1.0):
    m = jnp.mean(x, axis=-1, keepdims=True)
    c = x - m
    v = jnp.mean(c * c, axis=-1, keepdims=True)
    return c * (jax.lax.rsqrt(v + EPS) * gain)


def _interleave(even, odd):
    return pltpu.bitcast(pltpu.pack_elementwise([even, odd], packed_dtype=BF16), U32)


def _low(words):
    return pltpu.bitcast(words << 16, F32)


def _high(words):
    return pltpu.bitcast(words & np.uint32(0xFFFF0000), F32)


def _unpack(x):
    return pltpu.bitcast(x, BF16)


def _dot(a, b):
    return jax.lax.dot_general(a, b, (((1,), (0,)), ((), ())), preferred_element_type=F32)


def _dot_nt(a, b):
    return jax.lax.dot_general(a, b, (((1,), (1,)), ((), ())), preferred_element_type=F32)


def _blocks(x):
    n = x.shape[1] // NB
    return [x[:, i * n:(i + 1) * n] for i in range(NB)]


def _right_terms(even, odd, words=None):
    def term(w, kind, i, j):
        if kind == "q":
            return _scaled(w[i][j], _gains(kind, i, j)[1])
        if kind == "r":
            return _scaled(w[i][j] + w[j][i], _gains(kind, i, j)[1])
        val = w[i][i]
        for k in range(NB):
            if k != i:
                val = val - w[i][k] if kind == "a" else val + w[k][i]
        return val
    return [words[t[1]][t[2]] if words is not None and t[0] == "q" and _gains(*t)[1] == 1.0
            else _interleave(term(even, *t), term(odd, *t)) for t in TERMS]


def _run(*gens, order=""):
    for which in order:
        next(gens[int(which)], None)
    for gen in gens:
        for _ in gen:
            pass


def _make_kernel(S, D, H, E, M, T, F, cfg):
    OSPLIT, DSPLIT, NSTAGE, NSTRIP, LAG, RING = (
        cfg[k] for k in ("OSPLIT", "DSPLIT", "NSTAGE", "NSTRIP", "LAG", "RING"))
    nodes = NODES
    NSEG = S // T
    NG = H // NB
    DB = D // NB
    DC = 32
    NDC = DB // DC
    FC = NB * LANES
    NFC = F // FC
    SUB = cfg.get('SUB', 64)
    L = M + T
    CUT = cfg['CUT']
    ARING = cfg.get("ARING", 7)
    scale = float(E) ** -0.5

    def left_terms(s, d=None):
        if d is None:
            return {n: s[i] for n, (kind, i, _) in enumerate(TERMS) if kind == "a"}
        ts = {t: [t * x for x in s] for t in nodes if t > 0}
        e = [[d[i] + ts[t][i] if t > 0 else d[i] - ts[-t][i] for i in range(NB)] for t in nodes]
        out = {}
        for n, (kind, i, j) in enumerate(TERMS):
            if kind == "a":
                out[n] = s[i]
            elif kind == "b":
                out[n] = e[i][i]
            elif kind == "q":
                out[n] = _difference(e[j][i], e[j][j], _gains(kind, i, j)[0])
            else:
                out[n] = _difference(e[i][i], e[j][j], _gains(kind, i, j)[0])
        return out

    def block_product(nl, left, right, acc=None):
        acc = [[None] * NB for _ in range(nl)] if acc is None else [list(row) for row in acc]

        def add(row, j, x):
            acc[row][j] = x if acc[row][j] is None else acc[row][j] + x

        for n, (kind, i, j) in enumerate(TERMS):
            if nl == 1:
                if kind in "aq":
                    p = _dot(left(TERMS.index(("a", i, i))), right(n))
                    if kind == "q":
                        p = _scaled(p, 1.0 / _gains(kind, i, j)[1])
                    add(0, i, p)
                    if kind == "q":
                        add(0, j, p)
                continue
            p = _dot(left(n), right(n))
            if kind == "a":
                u = p
            elif kind == "b":
                add(0, i, u)
                add(1, i, p - nodes[i] * u)
            else:
                u = u + p
                add(0, j, p)
                add(1, j, -nodes[i if kind == "q" else j] * p)
        return acc

    def long_product(nl, left, right, k0, k1, acc):
        width = cfg.get("W1", DB) if k1 - k0 == LANES else LANES
        tiles = range(DB // LANES)
        step = width // LANES
        out = []
        for c in tiles[::step]:
            old = None if acc is None else [
                [jnp.concatenate([acc[c + x][r][j] for x in range(step)], axis=1)
                 for j in range(NB)] for r in range(nl)]
            new = block_product(
                nl, lambda n: left(n, k0, k1),
                lambda n: _unpack(right[n, k0 // 2:k1 // 2, c * LANES:c * LANES + width]), old)
            out += [[[b[:, x * LANES:(x + 1) * LANES] for b in row] for row in new]
                    for x in range(step)]
        return out

    def ring(ref, n, rows, k0, k1):
        return jnp.concatenate([ref[n, k % ref.shape[1], 0:rows, :]
                                for k in range(k0 // LANES, k1 // LANES)], axis=1)

    def column_tiles(blocks):
        return [[[b[:, j * DB + c:j * DB + c + LANES] for j in range(NB)] for b in blocks]
                for c in range(0, DB, LANES)]

    def row_blocks(tiles):
        return [jnp.concatenate([t[r][j] for j in range(NB) for t in tiles], axis=1)
                for r in range(len(tiles[0]))]

    def scope(name):
        return jax.named_scope("S_" + name) if cfg.get("SCOPES") and name in cfg.get("WHICH", [name]) else contextlib.nullcontext()

    def mask_tables(nl):
        r = jax.lax.broadcasted_iota(jnp.int32, (nl * L, nl * L), 0)
        c = jax.lax.broadcasted_iota(jnp.int32, (nl * L, nl * L), 1)
        same = (r < L) == (c < L)
        vis = same & ((jnp.where(r < L, r, r - L) < M) | (c <= r))
        return vis, jnp.where(same, -1e9 * LOG2E, -jnp.inf).astype(F32)

    def kernel(x_hbm, mem_ref, wq_hbm, wk_hbm, wv_hbm, wo_hbm, wg_hbm, wu_hbm, wd_hbm, out_hbm,
               wqkv, wo, wgu, wd, st_qkv, st_row, st_col, x_v,
               h_s, o_s, hb_s, a_s, y_s, d_s, z_s,
               sem_qkv, sem_row, sem_col, sem_x, sem_out):
        def qkv_copy(which, i):
            return pltpu.make_async_copy((wq_hbm, wk_hbm, wv_hbm)[which].at[:, i % NDC],
                                         st_qkv.at[i % NSTAGE], sem_qkv.at[i % NSTAGE])

        def qkv_start(i):
            for which in range(3):
                pl.when(i // NDC == which)(qkv_copy(which, i).start)

        def row_copy(src, i):
            return pltpu.make_async_copy(src.at[i], st_row.at[i], sem_row.at[i])

        def gu_copy(which, c):
            slot = (2 * c + which) % NSTRIP
            cols = pl.ds(pl.multiple_of(c * FC, FC), FC)
            return pltpu.make_async_copy((wg_hbm, wu_hbm)[which].at[:, cols],
                                         st_col.at[slot], sem_col.at[slot])

        def convert(src, dst, row0):
            n = src.shape[0] // NB
            sub = SUB * LANES * NB // src.shape[1]

            @pl.loop(0, n // sub)
            def _(r):
                w = [pltpu.bitcast(src[pl.ds(pl.multiple_of(i * n + r * sub, sub), sub), :], U32)
                     for i in range(NB)]
                rows = pl.ds(pl.multiple_of((row0 + r * sub) // 2, sub // 2), sub // 2)
                for k, val in enumerate(_right_terms([_blocks(_low(x)) for x in w],
                                                     [_blocks(_high(x)) for x in w],
                                                     [_blocks(x) for x in w])):
                    dst[k, rows, :] = val

        def convert_qkv(i):
            qkv_copy(0, i).wait()
            words = [st_qkv.at[i % NSTAGE, b].bitcast(U32) for b in range(NB)]
            rows = pl.ds(pl.multiple_of((i % NDC) * (DC // 2), DC // 2), DC // 2)
            span = (DC - 1) * H // 2 + NB

            @pl.loop(0, NG // 2)
            def _(gg):
                views = [w.at[pl.ds(pl.multiple_of(gg * NB, NB), span)] for w in words]
                for g in range(2):
                    def heads(src, parity):
                        pairs = [src[pl.ds(parity * H // 2 + p, DC // 2, stride=H), :]
                                 for p in range(g * NB // 2, (g + 1) * NB // 2)]
                        return [half(x) for x in pairs for half in (_low, _high)]
                    for k, val in enumerate(_right_terms(
                            *([heads(src, parity) for src in views] for parity in range(2)))):
                        wqkv[i // NDC, 2 * gg + g, k, rows, :] = val

        def convert_gu(c):
            for which in range(2):
                gu_copy(which, c).wait()
                convert(st_col.at[(2 * c + which) % NSTRIP], wgu.at[which, c], 0)
            pending = c + NSTRIP // 2

            @pl.when(pending < NFC)
            def _():
                for which in range(2):
                    gu_copy(which, pending).start()

            for j in range(2):
                piece = 2 * (pending - NFC) + j
                pl.when((piece >= 0) & (piece < NFC))(
                    row_copy(wd_hbm, jnp.clip(piece, 0, NFC - 1)).start)

        x_head = pltpu.make_async_copy(x_hbm.at[0:LAG + 2], x_v.at[0:LAG + 2], sem_x.at[0])
        x_rest = pltpu.make_async_copy(x_hbm.at[LAG + 2:NSEG], x_v.at[LAG + 2:NSEG], sem_x.at[1])

        def out_copy(i, lo, hi):
            return pltpu.make_async_copy(x_v.at[lo:hi], out_hbm.at[lo:hi], sem_out.at[i])

        def x_seg(seg):
            return x_v[seg].astype(F32)

        def set_rows(*blocks):
            parts = [_blocks(jnp.concatenate(blk, axis=0)) for blk in blocks]
            for n, a in left_terms(*parts).items():
                h_s[n] = a

        def attention_ops(nl, residual, before_out=None):
            vis, fill = mask_tables(nl)

            def proj(g):
                res = []
                for j in (1, 0, 2):
                    c = block_product(nl, h_s.__getitem__, lambda n: _unpack(wqkv[j, g, n]))
                    res.append([jnp.concatenate([row[h] for row in c], axis=0).astype(BF16)
                                for h in range(NB)])
                return res

            def attend(s, v):
                s = jnp.where(vis, s * (scale * LOG2E), fill)
                p = jnp.exp2(s - jnp.max(s, axis=-1, keepdims=True))
                tot = jnp.sum(p, axis=-1, keepdims=True)
                inv = pl.reciprocal(tot, approx=True)
                inv = inv * (2.0 - tot * inv)
                return _dot(p, v) * inv

            def out_proj(g0, g1, acc):
                if g0 == 0:
                    acc = column_tiles([jnp.concatenate([jnp.zeros((M, D), F32), x], axis=0)
                                        for x in residual()])
                return long_product(nl, lambda n, a, b: ring(o_s, n, L, a, b), wo, g0 * E, g1 * E, acc)

            k, q, v = proj(0)
            acc, done = None, 0
            for g in range(NG):
                ss = [_dot_nt(q[h], k[h]) for h in range(NB)]
                for at, upto in (OSPLIT if before_out is None else ()):
                    if at == g:
                        acc, done = out_proj(done, upto, acc), upto
                if g + 1 < NG:
                    nxt = proj(g + 1)
                else:
                    yield
                o = [attend(ss[h], v[h]) for h in range(NB)]
                parts = [[x[j * L:(j + 1) * L] for x in o] for j in range(nl)]
                for n, a in left_terms(*parts).items():
                    o_s[n, g] = a
                k, q, v = nxt
                yield
            if before_out is not None:
                before_out()
                for g in range(0, NG - 2, 2):
                    acc, done = out_proj(g, g + 2, acc), g + 2
            acc = out_proj(done, NG, acc)
            yield
            for j, y in enumerate(row_blocks(acc)):
                y_s[j] = y

        def set_glu_rows(top, bot):
            for n, a in left_terms(_blocks(_ln(top, 0.5)), _blocks(_ln(bot, 0.5))).items():
                hb_s[n, 0:top.shape[0], :] = a

        def glu_ops(rows, start, finish, c0=0, c1=NFC, need=lambda c0, c1: None):
            def gate_up(c):
                g, u = (block_product(2, lambda n: hb_s[n, 0:rows, :],
                                      lambda n: _unpack(wgu[j, c, n])) for j in range(2))
                act = [[jnp.tanh(x) * y + y for x, y in zip(gr, ur)] for gr, ur in zip(g, u)]
                for n, a in left_terms(*act).items():
                    a_s[n, c % ARING, 0:rows, :] = a

            def down(c0, c1, acc):
                need(c0, c1)
                acc = column_tiles(start()) if acc is None else acc
                return long_product(2, lambda n, a, b: ring(a_s, n, rows, a, b), wd,
                                    c0 * LANES, c1 * LANES, acc)

            acc, done = None, c0
            for c in range(c0, c1):
                gate_up(c)
                for at, upto in DSPLIT:
                    if at == c and upto > done:
                        acc, done = down(done, upto, acc), upto
                yield
            finish(row_blocks(down(done, c1, acc)))

        x_head.start()
        for i in range(NSTAGE):
            qkv_copy(0, i).start()

        @pl.loop(0, 3 * NDC)
        def _(i):
            with scope("q"):
                convert_qkv(i)
            qkv_start(i + NSTAGE)
            piece = i + NSTAGE - 3 * NDC
            pl.when(piece >= 0)(row_copy(wo_hbm, jnp.maximum(piece, 0)).start)

        for g in range(NSTAGE, NG):
            row_copy(wo_hbm, g).start()

        def convert_wo(g):
            for which in range(2):
                pl.when((g < NSTRIP) & (g % 2 == which))(gu_copy(which, g // 2).start)
            row_copy(wo_hbm, g).wait()
            convert(st_row.at[g], wo, g * E)

        x_head.wait()
        mem0 = mem_ref[...].astype(F32)
        set_rows((mem0, _ln(x_seg(0))))
        per_step = cfg.get("NEARLY", 3)

        @pl.loop(0, LAG)
        def _(t):
            def convert_arrived():
                with scope("g"):
                    pl.loop(0, jnp.where(t == 0, NG, 0))(convert_wo)
                    pl.loop(jnp.maximum(t - 1, 0) * per_step,
                            jnp.where(t + 1 < LAG, t * per_step, NFC))(convert_gu)

            with scope("head"):
                _run(attention_ops(1, lambda: [x_seg(t)], convert_arrived))
                z_s[t] = y_s[0, M:, :]
                set_rows((y_s[0, :M, :], _ln(x_seg(t + 1))))

        set_glu_rows(z_s[1], z_s[0])

        for piece in range(NSTRIP, NFC):
            row_copy(wd_hbm, piece).start()

        def head_down(c0, c1):
            cuts = cfg.get("DCUT")
            if cuts is not None:
                if str(c0) not in cuts:
                    return
                c1 = cuts[str(c0)]

            @pl.loop(c0, c1)
            def _(c):
                with scope("d"):
                    row_copy(wd_hbm, c).wait()
                    convert(st_row.at[c], wd, c * LANES)

        def partial_sums():
            return [d_s[0], d_s[1]]

        def keep_partial_sums(d):
            d_s[0], d_s[1] = d

        def head_glu_finish(d):
            z_s[1], z_s[0] = d

        def tokens():
            return [y_s[0, M:, :], y_s[1, M:, :]]

        def step_rows(t):
            set_rows((y_s[0, :M, :], _ln(x_seg(jnp.minimum(t, NSEG - 1)))),
                     (y_s[1, :M, :], _ln(z_s[(t - LAG) % RING])))

        def glu_finish(t):
            def finish(d):
                z_s[t % RING] = d[0]
                x_v[jnp.maximum(t - LAG, 0)] = d[1].astype(BF16)
            return finish

        if CUT < NFC:
            _run(glu_ops(T, lambda: [z_s[1], z_s[0]], keep_partial_sums, 0, CUT, head_down))
            _run(glu_ops(T, partial_sums, head_glu_finish, CUT, NFC, head_down))
        else:
            _run(glu_ops(T, lambda: [z_s[1], z_s[0]], head_glu_finish, 0, NFC, head_down))
        x_rest.start()
        y_s[1] = jnp.concatenate([mem0, y_s[0, M:, :]], axis=0)
        if CUT == NFC:
            step_rows(LAG)

        with scope("main"):
            @pl.loop(LAG, cfg.get("NSTEP", NSEG))
            def _(t):
                pl.when(t == LAG + 1)(x_rest.wait)
                attention = attention_ops(2, lambda: [x_seg(t), z_s[(t - LAG) % RING]])
                if CUT < NFC:
                    step_rows(t)
                    _run(glu_ops(T, partial_sums, glu_finish(t - 2), CUT, NFC))
                    set_glu_rows(*tokens())
                    _run(glu_ops(T, tokens, keep_partial_sums, 0, CUT), attention, order=cfg["ORDER"])
                else:
                    set_glu_rows(*tokens())
                    keep_partial_sums(tokens())

                    def both():
                        yield from attention
                        step_rows(t + 1)
                    _run(glu_ops(T, partial_sums, glu_finish(t - 1)), both(), order=cfg["ORDER"])

        done = NSEG - 2 - LAG
        out_copy(0, 0, done).start()
        if CUT < NFC:
            _run(glu_ops(T, partial_sums, glu_finish(NSEG - 2), CUT, NFC))
        set_glu_rows(*tokens())
        set_rows((y_s[1, :M, :], _ln(z_s[(NSEG - LAG) % RING])))
        _run(glu_ops(T, tokens, glu_finish(NSEG - 1)))

        @pl.loop(NSEG - LAG, NSEG)
        def _(t):
            with scope("tail"):
                _run(attention_ops(1, lambda: [z_s[t % RING]]))
                set_rows((y_s[0, :M, :], _ln(z_s[jnp.minimum(t + 1, NSEG - 1) % RING])))
                z_s[t % RING] = y_s[0, M:, :]

        def last_rows():
            y = jnp.concatenate([z_s[t % RING] for t in range(NSEG - LAG, NSEG)], axis=0)
            return y[:LAG * T // 2], y[LAG * T // 2:]

        def last_finish(d):
            z = jnp.concatenate(d, axis=0).astype(BF16)
            for j in range(LAG):
                x_v[NSEG - LAG + j] = z[j * T:(j + 1) * T]

        set_glu_rows(*last_rows())
        with scope("lglu"):
            _run(glu_ops(LAG * T // 2, last_rows, last_finish))
        out_copy(1, done, NSEG).start()
        out_copy(0, 0, done).wait()
        out_copy(1, done, NSEG).wait()

    dma = pltpu.SemaphoreType.DMA
    nt = len(TERMS)
    scratch = [
        pltpu.VMEM((3, NG, nt, DB // 2, E), U32),
        pltpu.VMEM((nt, NG * E // 2, DB), U32),
        pltpu.VMEM((2, NFC, nt, DB // 2, LANES), U32),
        pltpu.VMEM((nt, NFC * LANES // 2, DB), U32),
        pltpu.VMEM((NSTAGE, NB, DC * H, E), BF16),
        pltpu.VMEM((NG, FC, D), BF16),
        pltpu.VMEM((NSTRIP, D, FC), BF16),
        pltpu.VMEM((NSEG, T, D), BF16),
        pltpu.VMEM((nt, L, DB), F32),
        pltpu.VMEM((nt, NG, L, E), F32),
        pltpu.VMEM((nt, LAG * T // 2, DB), F32),
        pltpu.VMEM((nt, ARING, LAG * T // 2, LANES), F32),
        pltpu.VMEM((2, L, D), F32),
        pltpu.VMEM((2, T, D), F32),
        pltpu.VMEM((RING, T, D), F32),
        dma((NSTAGE,)), dma((NG,)), dma((NSTRIP,)), dma((2,)), dma((2,)),
    ]
    return kernel, scratch, (NB, NDC, DC * H, E)


def build(cfg):
    @functools.partial(jax.jit, static_argnames=("A_seg_len",))
    def fn(A_x, A_mem0, A_Wq, A_Wk, A_Wv, A_Wo, A_seg_len, B_x, B_w_gate, B_w_up, B_w_down):
        del B_x
        B, S, D = A_x.shape
        _, H, E = A_Wq.shape
        M = A_mem0.shape[1]
        F = B_w_gate.shape[1]
        T = int(A_seg_len)
        FC = NB * LANES
        kernel, scratch, qkv_shape = _make_kernel(S, D, H, E, M, T, F, cfg)
        hbm = pl.BlockSpec(memory_space=pl.ANY)
        out = pl.pallas_call(
            kernel,
            out_shape=jax.ShapeDtypeStruct((S // T, T, D), A_x.dtype),
            in_specs=[hbm, pl.BlockSpec(memory_space=pltpu.VMEM)] + [hbm] * 7,
            out_specs=hbm,
            scratch_shapes=scratch,
            compiler_params=pltpu.CompilerParams(vmem_limit_bytes=127 * 1024 * 1024,
                                                 flags=cfg.get("flags")),
        )(A_x.reshape(S // T, T, D), A_mem0.reshape(M, D),
          A_Wq.reshape(qkv_shape), A_Wk.reshape(qkv_shape), A_Wv.reshape(qkv_shape),
          A_Wo.reshape(H * E // FC, FC, D), B_w_gate, B_w_up, B_w_down.reshape(F // FC, FC, D))
        return out.reshape(B, S, D)

    return fn


pallas_interleave_layers__memory_aug_recurrent_mem_tr__glu_gated_glu__prompt_kernel = build(CFG)
```

```python
import functools

import jax
import jax.numpy as jnp
import numpy as np
import jax.experimental.pallas as pl
import jax.experimental.pallas.tpu as pltpu

F32 = jnp.float32
BF16 = jnp.bfloat16
U32 = jnp.uint32
EPS = 1e-5
LOG2E = 1.4426950408889634
LANES = 128
NB = 4
LAG = 3
RING = 4
DC = 32
NSTAGE = 4
NSTRIP = 6
OUT_SPLIT = ((3, 2), (5, 4), (7, 6))
DOWN_SPLIT = ((2, 1), (4, 3), (6, 5))

NODES = (0.5, -0.5, 1.5, -1.5)
TERMS = [term for i in range(NB) for term in (
    [("a", i, i)] + [("q", i, j) for j in range(NB) if j != i]
    + [("r", i, j) for j in range(i + 1, NB)] + [("b", i, i)])]


def _gains(kind, i, j):
    gain = 1.0 / (NODES[j] - NODES[i]) if kind == "q" else 1.0 / (NODES[i] - NODES[j])
    right = abs(gain) if kind == "r" or np.frexp(abs(gain))[0] == 0.5 else 1.0
    return gain / right, right


def _scaled(x, gain):
    return x if gain == 1.0 else x * gain


def _ln(x, gain=1.0):
    m = jnp.mean(x, axis=-1, keepdims=True)
    c = x - m
    v = jnp.mean(c * c, axis=-1, keepdims=True)
    return c * (jax.lax.rsqrt(v + EPS) * gain)


def _rows(words):
    return pltpu.bitcast(words, BF16)


def _store_rows(words_ref, col, rows):
    words_ref.bitcast(BF16)[:, col:col + rows.shape[1]] = rows


def _dot(a, b):
    return jax.lax.dot_general(a, b, (((1,), (0,)), ((), ())), preferred_element_type=F32)


def _dot_nt(a, b):
    return jax.lax.dot_general(a, b, (((1,), (1,)), ((), ())), preferred_element_type=F32)


def _blocks(x):
    n = x.shape[1] // NB
    return [x[:, i * n:(i + 1) * n] for i in range(NB)]


def _left_terms(s, d=None):
    if d is None:
        return {n: s[i] for n, (kind, i, _) in enumerate(TERMS) if kind == "a"}
    ts = {t: [t * x for x in s] for t in NODES if t > 0}
    e = [[d[i] + ts[t][i] if t > 0 else d[i] - ts[-t][i] for i in range(NB)] for t in NODES]
    out = {}
    for n, (kind, i, j) in enumerate(TERMS):
        if kind == "a":
            out[n] = s[i]
        elif kind == "b":
            out[n] = e[i][i]
        else:
            x, y = e[j if kind == "q" else i][i], e[j][j]
            gain = _gains(kind, i, j)[0]
            out[n] = _scaled(x - y if gain > 0 else y - x, abs(gain))
    return out


def _right_terms(w):
    f = [[b.astype(F32) for b in row] for row in w]
    out = []
    for kind, i, j in TERMS:
        if kind in "qr":
            gain = _gains(kind, i, j)[1]
            if kind == "q" and gain == 1.0:
                val = w[i][j]
            else:
                val = _scaled(f[i][j] if kind == "q" else f[i][j] + f[j][i], gain)
        else:
            val = f[i][i]
            for k in range(NB):
                if k != i:
                    val = val - f[i][k] if kind == "a" else val + f[k][i]
        out.append(val.astype(BF16))
    return out


def _block_product(nl, left, right, acc=None):
    acc = [[None] * NB for _ in range(nl)] if acc is None else [list(row) for row in acc]

    def add(row, j, x):
        acc[row][j] = x if acc[row][j] is None else acc[row][j] + x

    for n, (kind, i, j) in enumerate(TERMS):
        if nl == 1:
            if kind in "aq":
                p = _dot(left(TERMS.index(("a", i, i))), right(n))
                if kind == "q":
                    p = _scaled(p, 1.0 / _gains(kind, i, j)[1])
                    add(0, j, p)
                add(0, i, p)
            continue
        p = _dot(left(n), right(n))
        if kind == "a":
            u = p
        elif kind == "b":
            add(0, i, u)
            add(1, i, p - NODES[i] * u)
        else:
            u = u + p
            add(0, j, p)
            add(1, j, -NODES[i if kind == "q" else j] * p)
    return acc


def _long_product(left_ref, rows, right_ref, k0, k1, acc):
    def left(n):
        return jnp.concatenate([left_ref[n, k, 0:rows, :] for k in range(k0, k1)], axis=1)

    def right(c, n):
        return _rows(right_ref[n, k0 * LANES // 2:k1 * LANES // 2, c * LANES:(c + 1) * LANES])

    return [_block_product(len(old), left, functools.partial(right, c), old)
            for c, old in enumerate(acc)]


def _column_tiles(row_blocks):
    width = row_blocks[0].shape[1] // NB
    return [[[b[:, j * width + c:j * width + c + LANES] for j in range(NB)] for b in row_blocks]
            for c in range(0, width, LANES)]


def _row_blocks(tiles):
    return [jnp.concatenate([t[r][j] for j in range(NB) for t in tiles], axis=1)
            for r in range(len(tiles[0]))]


def _run(*gens, order=()):
    for which in order:
        next(gens[which], None)
    for gen in gens:
        for _ in gen:
            pass


def _make_kernel(S, D, H, E, M, T, F):
    NSEG = S // T
    NG = H // NB
    DB = D // NB
    NDC = DB // DC
    PITCH = DC + 1
    FC = NB * LANES
    NFC = F // FC
    EARLY = NFC // 2
    L = M + T
    scale = float(E) ** -0.5

    def mask_tables(nl):
        r = jax.lax.broadcasted_iota(jnp.int32, (nl * L, nl * L), 0)
        c = jax.lax.broadcasted_iota(jnp.int32, (nl * L, nl * L), 1)
        same = (r < L) == (c < L)
        vis = same & ((jnp.where(r < L, r, r - L) < M) | (c <= r))
        return vis, jnp.where(same, -1e9 * LOG2E, -jnp.inf).astype(F32)

    def kernel(x_hbm, mem_ref, wq_hbm, wk_hbm, wv_hbm, wo_hbm, wg_hbm, wu_hbm, wd_hbm, out_hbm,
               wqkv, wo, wgu, wd, st_qkv, st_word, st_row, st_col, x_v,
               h_s, o_s, hb_s, a_s, y_s, d_s, z_s,
               sem_qkv, sem_row, sem_col, sem_x, sem_out):
        def qkv_copy(which, i):
            return pltpu.make_async_copy((wq_hbm, wk_hbm, wv_hbm)[which].at[:, i % NDC],
                                         st_qkv.at[i % NSTAGE], sem_qkv.at[i % NSTAGE])

        def row_copy(src, i):
            return pltpu.make_async_copy(src.at[i], st_row.at[i], sem_row.at[i])

        def gu_copy(which, c):
            slot = (2 * c + which) % NSTRIP
            cols = pl.ds(pl.multiple_of(c * FC, FC), FC)
            return pltpu.make_async_copy((wg_hbm, wu_hbm)[which].at[:, cols],
                                         st_col.at[slot], sem_col.at[slot])

        def convert(src, dst, row0=0, col0=0):
            n = src.shape[0] // NB
            sub = 64 * FC // src.shape[1]

            @pl.loop(0, n // sub)
            def _(r):
                w = [_blocks(src[pl.ds(pl.multiple_of(i * n + r * sub, sub), sub), :])
                     for i in range(NB)]
                rows = pl.ds(pl.multiple_of((row0 + r * sub) // 2, sub // 2), sub // 2)
                for k, val in enumerate(_right_terms(w)):
                    _store_rows(dst.at[k, rows], col0, val)

        def convert_qkv(i):
            for b in range(NB):
                for d in range(DC):
                    st_word[b, pl.ds(d // 2 + d % 2 * DC // 2, H // 2, stride=PITCH), :] = (
                        pltpu.bitcast(st_qkv[i % NSTAGE, b, d * H:(d + 1) * H, :], U32))
            rows = pl.ds(pl.multiple_of((i % NDC) * (DC // 2), DC // 2), DC // 2)
            for g in range(NG):
                w = []
                for b in range(NB):
                    w.append([])
                    for pair in range(g * NB // 2, (g + 1) * NB // 2):
                        x = st_word[b, pl.ds(pair * PITCH, DC // 2), :]
                        y = st_word[b, pl.ds(pair * PITCH + DC // 2, DC // 2), :]
                        w[-1].append(_rows((x & np.uint32(0xFFFF)) | (y << 16)))
                        w[-1].append(_rows((x >> 16) | (y & np.uint32(0xFFFF0000))))
                for k, val in enumerate(_right_terms(w)):
                    _store_rows(wqkv.at[i // NDC, g // 2, k, rows], g % 2 * E, val)

        def convert_wo(g):
            for which in range(2):
                pl.when((g < NSTRIP) & (g % 2 == which))(gu_copy(which, g // 2).start)
            row_copy(wo_hbm, g).wait()
            convert(st_row.at[g], wo, g * E)

        def convert_gu(c):
            for which in range(2):
                gu_copy(which, c).wait()
                convert(st_col.at[(2 * c + which) % NSTRIP], wgu.at[c], 0, which * LANES)
            pending = c + NSTRIP // 2

            @pl.when(pending < NFC)
            def _():
                for which in range(2):
                    gu_copy(which, pending).start()

            for j in range(2):
                piece = 2 * (pending - NFC) + j
                pl.when((piece >= 0) & (piece < NFC))(
                    row_copy(wd_hbm, jnp.clip(piece, 0, NFC - 1)).start)

        def convert_wd(c):
            row_copy(wd_hbm, c).wait()
            convert(st_row.at[c], wd, c * LANES)

        x_head = pltpu.make_async_copy(x_hbm.at[0:LAG + 2], x_v.at[0:LAG + 2], sem_x.at[0])
        x_rest = pltpu.make_async_copy(x_hbm.at[LAG + 2:NSEG], x_v.at[LAG + 2:NSEG], sem_x.at[1])

        def out_copy(i, lo, hi):
            return pltpu.make_async_copy(x_v.at[lo:hi], out_hbm.at[lo:hi], sem_out.at[i])

        def x_seg(seg):
            return x_v[seg].astype(F32)

        def set_rows(*blocks):
            parts = [_blocks(jnp.concatenate(blk, axis=0)) for blk in blocks]
            for n, a in _left_terms(*parts).items():
                h_s[n] = a

        def attention(nl, residual, before_out=None):
            vis, fill = mask_tables(nl)

            def proj(j, g):
                cols = slice(g % 2 * E, (g % 2 + 1) * E)
                c = _block_product(nl, h_s.__getitem__,
                                   lambda n: _rows(wqkv[j, g // 2, n, :, cols]))
                heads = [jnp.concatenate([row[h] for row in c], axis=0) for h in range(NB)]
                return heads if j == 0 else [x.astype(BF16) for x in heads]

            def proj_all(g):
                k = proj(1, g)
                return proj(0, g), k, proj(2, g)

            def attend(s, v):
                s = jnp.where(vis, s * (scale * LOG2E), fill)
                p = jnp.exp2(s - jnp.max(s, axis=-1, keepdims=True))
                tot = jnp.sum(p, axis=-1, keepdims=True)
                inv = pl.reciprocal(tot, approx=True)
                inv = inv * (2.0 - tot * inv)
                return _dot(p, v) * inv

            def out_proj(g0, g1, acc):
                if acc is None:
                    acc = _column_tiles([jnp.concatenate([jnp.zeros((M, D), F32), x], axis=0)
                                         for x in residual()])
                return _long_product(o_s, L, wo, g0, g1, acc)

            q, k, v = proj_all(0)
            acc, done = None, 0
            for g in range(NG):
                scores = [_dot_nt(q[h], k[h]) for h in range(NB)]
                for at, upto in (OUT_SPLIT if before_out is None else ()):
                    if at == g:
                        acc, done = out_proj(done, upto, acc), upto
                if g + 1 < NG:
                    nxt = proj_all(g + 1)
                else:
                    yield
                o = [attend(scores[h], v[h]) for h in range(NB)]
                parts = [[x[j * L:(j + 1) * L] for x in o] for j in range(nl)]
                for n, a in _left_terms(*parts).items():
                    o_s[n, g] = a
                q, k, v = nxt
                yield
            if before_out is not None:
                before_out()
                for _, upto in OUT_SPLIT:
                    acc, done = out_proj(done, upto, acc), upto
            acc = out_proj(done, NG, acc)
            yield
            for j, y in enumerate(_row_blocks(acc)):
                y_s[j] = y

        def set_glu_rows(top, bot):
            for n, a in _left_terms(_blocks(_ln(top, 0.5)), _blocks(_ln(bot, 0.5))).items():
                hb_s[n, 0:top.shape[0], :] = a

        def glu(rows, residual, finish, before_down=lambda c: None):
            def gate_up(c):
                g, u = (_block_product(2, lambda n: hb_s[n, 0:rows, :],
                                       lambda n: _rows(wgu[c, n, :, j * LANES:(j + 1) * LANES]))
                        for j in range(2))
                act = [[jnp.tanh(x) * y + y for x, y in zip(gr, ur)] for gr, ur in zip(g, u)]
                for n, a in _left_terms(*act).items():
                    a_s[n, c, 0:rows, :] = a

            def down(c0, c1, acc):
                before_down(c0)
                acc = _column_tiles(residual()) if acc is None else acc
                return _long_product(a_s, rows, wd, c0, c1, acc)

            acc, done = None, 0
            for c in range(NFC):
                gate_up(c)
                for at, upto in DOWN_SPLIT:
                    if at == c:
                        acc, done = down(done, upto, acc), upto
                yield
            finish(_row_blocks(down(done, NFC, acc)))

        x_head.start()
        for i in range(NSTAGE):
            qkv_copy(0, i).start()

        @pl.loop(0, 3 * NDC)
        def _(i):
            for which in range(3):
                pl.when(i // NDC == which)(qkv_copy(which, i).wait)
            convert_qkv(i)
            for which in range(3):
                pl.when((i + NSTAGE) // NDC == which)(qkv_copy(which, i + NSTAGE).start)
            piece = i + NSTAGE - 3 * NDC
            pl.when(piece >= 0)(row_copy(wo_hbm, jnp.maximum(piece, 0)).start)

        for g in range(NSTAGE, NG):
            row_copy(wo_hbm, g).start()
        x_head.wait()
        mem0 = mem_ref[...].astype(F32)
        set_rows((mem0, _ln(x_seg(0))))

        @pl.loop(0, LAG)
        def _(t):
            def convert_arrived():
                pl.loop(0, jnp.where(t == 0, NG, 0))(convert_wo)
                pl.loop(jnp.maximum(t - 1, 0) * EARLY,
                        jnp.where(t + 1 < LAG, t * EARLY, NFC))(convert_gu)

            _run(attention(1, lambda: [x_seg(t)], convert_arrived))
            z_s[t] = y_s[0, M:, :]
            set_rows((y_s[0, :M, :], _ln(x_seg(t + 1))))

        set_glu_rows(z_s[0], z_s[1])
        for piece in range(NSTRIP, NFC):
            row_copy(wd_hbm, piece).start()

        def head_down(c):
            cut = DOWN_SPLIT[1][1]
            if c in (0, cut):
                pl.loop(c, NFC if c else cut)(convert_wd)

        def head_finish(z):
            z_s[0], z_s[1] = z

        _run(glu(T, lambda: [z_s[0], z_s[1]], head_finish, head_down))
        x_rest.start()

        def tokens():
            return [y_s[0, M:, :], y_s[1, M:, :]]

        def step_rows(t):
            set_rows((y_s[0, :M, :], _ln(x_seg(jnp.minimum(t, NSEG - 1)))),
                     (y_s[1, :M, :], _ln(z_s[(t - LAG) % RING])))

        def glu_finish(t):
            def finish(z):
                z_s[t % RING] = z[0]
                x_v[jnp.maximum(t - LAG, 0)] = z[1].astype(x_v.dtype)
            return finish

        y_s[1] = jnp.concatenate([mem0, y_s[0, M:, :]], axis=0)
        step_rows(LAG)

        @pl.loop(LAG, NSEG)
        def _(t):
            pl.when(t == LAG + 1)(x_rest.wait)
            set_glu_rows(*tokens())
            d_s[0], d_s[1] = tokens()

            def attention_then_next_rows():
                yield from attention(2, lambda: [x_seg(t), z_s[(t - LAG) % RING]])
                step_rows(t + 1)

            _run(glu(T, lambda: [d_s[0], d_s[1]], glu_finish(t - 1)), attention_then_next_rows(),
                 order=(1,) * NG + (0, 1, 0, 1, 1))

        ready = NSEG - 1 - LAG
        out_copy(0, 0, ready).start()
        set_glu_rows(*tokens())
        set_rows((y_s[1, :M, :], _ln(z_s[(NSEG - LAG) % RING])))
        _run(glu(T, tokens, glu_finish(NSEG - 1)))

        @pl.loop(NSEG - LAG, NSEG)
        def _(t):
            _run(attention(1, lambda: [z_s[t % RING]]))
            set_rows((y_s[0, :M, :], _ln(z_s[jnp.minimum(t + 1, NSEG - 1) % RING])))
            z_s[t % RING] = y_s[0, M:, :]

        def last_rows():
            y = jnp.concatenate([z_s[t % RING] for t in range(NSEG - LAG, NSEG)], axis=0)
            return y[:LAG * T // 2], y[LAG * T // 2:]

        def last_finish(z):
            z = jnp.concatenate(z, axis=0).astype(x_v.dtype)
            for j in range(LAG):
                x_v[NSEG - LAG + j] = z[j * T:(j + 1) * T]

        set_glu_rows(*last_rows())
        _run(glu(LAG * T // 2, last_rows, last_finish))
        out_copy(1, ready, NSEG).start()
        out_copy(0, 0, ready).wait()
        out_copy(1, ready, NSEG).wait()

    dma = pltpu.SemaphoreType.DMA
    nt = len(TERMS)
    scratch = [
        pltpu.VMEM((3, NG // 2, nt, DB // 2, 2 * E), U32),
        pltpu.VMEM((nt, NG * E // 2, DB), U32),
        pltpu.VMEM((NFC, nt, DB // 2, 2 * LANES), U32),
        pltpu.VMEM((nt, NFC * LANES // 2, DB), U32),
        pltpu.VMEM((NSTAGE, NB, DC * H, E), BF16),
        pltpu.VMEM((NB, (PITCH + 7) * H // 2, E), U32),
        pltpu.VMEM((NG, FC, D), BF16),
        pltpu.VMEM((NSTRIP, D, FC), BF16),
        pltpu.VMEM((NSEG, T, D), BF16),
        pltpu.VMEM((nt, L, DB), F32),
        pltpu.VMEM((nt, NG, L, E), F32),
        pltpu.VMEM((nt, LAG * T // 2, DB), F32),
        pltpu.VMEM((nt, NFC, LAG * T // 2, LANES), F32),
        pltpu.VMEM((2, L, D), F32),
        pltpu.VMEM((2, T, D), F32),
        pltpu.VMEM((RING, T, D), F32),
        dma((NSTAGE,)), dma((NG,)), dma((NSTRIP,)), dma((2,)), dma((2,)),
    ]
    return kernel, scratch


@functools.partial(jax.jit, static_argnames=("A_seg_len",))
def pallas_interleave_layers__memory_aug_recurrent_mem_tr__glu_gated_glu__prompt_kernel(
    A_x: jax.Array,
    A_mem0: jax.Array,
    A_Wq: jax.Array,
    A_Wk: jax.Array,
    A_Wv: jax.Array,
    A_Wo: jax.Array,
    A_seg_len: int,
    B_x: jax.Array,
    B_w_gate: jax.Array,
    B_w_up: jax.Array,
    B_w_down: jax.Array,
):
    del B_x
    B, S, D = A_x.shape
    _, H, E = A_Wq.shape
    M = A_mem0.shape[1]
    F = B_w_gate.shape[1]
    T = int(A_seg_len)
    FC = NB * LANES
    assert (B, D, H, E, M, T, F) == (1, 1024, 32, LANES, 8, 32, 3584) and S % T == 0
    kernel, scratch = _make_kernel(S, D, H, E, M, T, F)
    qkv_shape = (NB, D // (NB * DC), DC * H, E)
    hbm = pl.BlockSpec(memory_space=pl.ANY)
    out = pl.pallas_call(
        kernel,
        out_shape=jax.ShapeDtypeStruct((S // T, T, D), A_x.dtype),
        in_specs=[hbm, pl.BlockSpec(memory_space=pltpu.VMEM)] + [hbm] * 7,
        out_specs=hbm,
        scratch_shapes=scratch,
        compiler_params=pltpu.CompilerParams(
            vmem_limit_bytes=127 * 1024 * 1024,
            flags={"XLA_TPU_EVENLY_DISTRIBUTE_CRITICAL_NODES": True}),
    )(A_x.reshape(S // T, T, D), A_mem0.reshape(M, D),
      A_Wq.reshape(qkv_shape), A_Wk.reshape(qkv_shape), A_Wv.reshape(qkv_shape),
      A_Wo.reshape(H * E // FC, FC, D), B_w_gate, B_w_up, B_w_down.reshape(F // FC, FC, D))
    return out.reshape(B, S, D)
```

```python
import functools

import jax
import jax.numpy as jnp
import numpy as np
import jax.experimental.pallas as pl
import jax.experimental.pallas.tpu as pltpu

F32 = jnp.float32
BF16 = jnp.bfloat16
U32 = jnp.uint32
EPS = 1e-5
LOG2E = 1.4426950408889634
LANES = 128
NB = 4
LAG = 3
RING = 4
DC = 32
NSTAGE = 4
NSTRIP = 8
OUT_SPLIT = ((3, 2), (5, 4), (7, 6))
DOWN_SPLIT = ((2, 1), (4, 3), (6, 5))

NODES = (0.5, -0.5, 1.5, -1.5)
TERMS = [term for i in range(NB) for term in (
    [("a", i, i)] + [("q", i, j) for j in range(NB) if j != i]
    + [("r", i, j) for j in range(i + 1, NB)] + [("b", i, i)])]


def _gains(kind, i, j):
    gain = 1.0 / (NODES[j] - NODES[i]) if kind == "q" else 1.0 / (NODES[i] - NODES[j])
    right = abs(gain) if kind == "r" or np.frexp(abs(gain))[0] == 0.5 else 1.0
    return gain / right, right


def _scaled(x, gain):
    return x if gain == 1.0 else x * gain


def _ln(x, gain=1.0):
    m = jnp.mean(x, axis=-1, keepdims=True)
    c = x - m
    v = jnp.mean(c * c, axis=-1, keepdims=True)
    return c * (jax.lax.rsqrt(v + EPS) * gain)


def _rows(words):
    return pltpu.bitcast(words, BF16)


def _store_rows(words_ref, col, rows):
    words_ref.bitcast(BF16)[:, col:col + rows.shape[1]] = rows


def _dot(a, b):
    return jax.lax.dot_general(a, b, (((1,), (0,)), ((), ())), preferred_element_type=F32)


def _dot_nt(a, b):
    return jax.lax.dot_general(a, b, (((1,), (1,)), ((), ())), preferred_element_type=F32)


def _blocks(x):
    n = x.shape[1] // NB
    return [x[:, i * n:(i + 1) * n] for i in range(NB)]


def _left_terms(s, d=None):
    if d is None:
        return {n: s[i] for n, (kind, i, _) in enumerate(TERMS) if kind == "a"}
    ts = {t: [t * x for x in s] for t in NODES if t > 0}
    e = [[d[i] + ts[t][i] if t > 0 else d[i] - ts[-t][i] for i in range(NB)] for t in NODES]
    out = {}
    for n, (kind, i, j) in enumerate(TERMS):
        if kind == "a":
            out[n] = s[i]
        elif kind == "b":
            out[n] = e[i][i]
        else:
            x, y = e[j if kind == "q" else i][i], e[j][j]
            gain = _gains(kind, i, j)[0]
            out[n] = _scaled(x - y if gain > 0 else y - x, abs(gain))
    return out


def _right_terms(w):
    f = [[b.astype(F32) for b in row] for row in w]
    out = []
    for kind, i, j in TERMS:
        if kind in "qr":
            gain = _gains(kind, i, j)[1]
            if kind == "q" and gain == 1.0:
                val = w[i][j]
            else:
                val = _scaled(f[i][j] if kind == "q" else f[i][j] + f[j][i], gain)
        else:
            val = f[i][i]
            for k in range(NB):
                if k != i:
                    val = val - f[i][k] if kind == "a" else val + f[k][i]
        out.append(val.astype(BF16))
    return out


def _block_product(nl, left, right, acc=None):
    acc = [[None] * NB for _ in range(nl)] if acc is None else [list(row) for row in acc]

    def add(row, j, x):
        acc[row][j] = x if acc[row][j] is None else acc[row][j] + x

    for n, (kind, i, j) in enumerate(TERMS):
        if nl == 1:
            if kind in "aq":
                p = _dot(left(TERMS.index(("a", i, i))), right(n))
                if kind == "q":
                    p = _scaled(p, 1.0 / _gains(kind, i, j)[1])
                    add(0, j, p)
                add(0, i, p)
            continue
        p = _dot(left(n), right(n))
        if kind == "a":
            u = p
        elif kind == "b":
            add(0, i, u)
            add(1, i, p - NODES[i] * u)
        else:
            u = u + p
            add(0, j, p)
            add(1, j, -NODES[i if kind == "q" else j] * p)
    return acc


def _long_product(left, right_ref, k0, k1, acc):
    def right(c, n):
        return _rows(right_ref[n, k0 * LANES // 2:k1 * LANES // 2, c * LANES:(c + 1) * LANES])

    return [_block_product(len(old), left, functools.partial(right, c), old)
            for c, old in enumerate(acc)]


def _column_tiles(row_blocks):
    width = row_blocks[0].shape[1] // NB
    return [[[b[:, j * width + c:j * width + c + LANES] for j in range(NB)] for b in row_blocks]
            for c in range(0, width, LANES)]


def _row_blocks(tiles):
    return [jnp.concatenate([t[r][j] for j in range(NB) for t in tiles], axis=1)
            for r in range(len(tiles[0]))]


def _run(*gens, order=()):
    for which in order:
        next(gens[which], None)
    for gen in gens:
        for _ in gen:
            pass


def _make_kernel(S, D, H, E, M, T, F):
    NSEG = S // T
    NG = H // NB
    DB = D // NB
    NDC = DB // DC
    PITCH = DC + 1
    FC = NB * LANES
    NFC = F // FC
    EARLY = NSTRIP // 2
    L = M + T
    scale = float(E) ** -0.5
    assert NSTRIP == NG >= NFC and NSEG > LAG + 2

    def mask_tables(nl):
        r = jax.lax.broadcasted_iota(jnp.int32, (nl * L, nl * L), 0)
        c = jax.lax.broadcasted_iota(jnp.int32, (nl * L, nl * L), 1)
        same = (r < L) == (c < L)
        vis = same & ((jnp.where(r < L, r, r - L) < M) | (c <= r))
        return vis, jnp.where(same, -1e9 * LOG2E, -jnp.inf).astype(F32)

    def kernel(x_hbm, mem_ref, wq_hbm, wk_hbm, wv_hbm, wo_hbm, wg_hbm, wu_hbm, wd_hbm, out_hbm,
               wqkv, wo, wgu, wd, st_qkv, st_word, st_row, st_col, x_v,
               h_s, o_s, hb_s, a_s, y_s, d_s, z_s,
               sem_qkv, sem_row, sem_col, sem_x, sem_out):
        def qkv_copy(which, i):
            return pltpu.make_async_copy((wq_hbm, wk_hbm, wv_hbm)[which].at[:, i % NDC],
                                         st_qkv.at[i % NSTAGE], sem_qkv.at[i % NSTAGE])

        def row_copy(src, i):
            return pltpu.make_async_copy(src.at[i], st_row.at[i], sem_row.at[i])

        def gu_copy(which, c):
            slot = (2 * c + which) % NSTRIP
            cols = pl.ds(pl.multiple_of(c * FC, FC), FC)
            return pltpu.make_async_copy((wg_hbm, wu_hbm)[which].at[:, cols],
                                         st_col.at[slot], sem_col.at[slot])

        def convert(src, dst, row0=0, col0=0):
            n = src.shape[0] // NB
            sub = 32 * FC // src.shape[1]

            @pl.loop(0, n // sub)
            def _(r):
                w = [_blocks(src[pl.ds(pl.multiple_of(i * n + r * sub, sub), sub), :])
                     for i in range(NB)]
                rows = pl.ds(pl.multiple_of((row0 + r * sub) // 2, sub // 2), sub // 2)
                for k, val in enumerate(_right_terms(w)):
                    _store_rows(dst.at[k, rows], col0, val)

        def convert_qkv(i):
            for b in range(NB):
                for d in range(DC):
                    st_word[b, pl.ds(d // 2 + d % 2 * DC // 2, H // 2, stride=PITCH), :] = (
                        pltpu.bitcast(st_qkv[i % NSTAGE, b, d * H:(d + 1) * H, :], U32))
            rows = pl.ds(pl.multiple_of((i % NDC) * (DC // 2), DC // 2), DC // 2)
            for g in range(NG):
                w = []
                for b in range(NB):
                    w.append([])
                    for pair in range(g * NB // 2, (g + 1) * NB // 2):
                        x = st_word[b, pl.ds(pair * PITCH, DC // 2), :]
                        y = st_word[b, pl.ds(pair * PITCH + DC // 2, DC // 2), :]
                        w[-1].append(_rows((x & np.uint32(0xFFFF)) | (y << 16)))
                        w[-1].append(_rows((x >> 16) | (y & np.uint32(0xFFFF0000))))
                for k, val in enumerate(_right_terms(w)):
                    _store_rows(wqkv.at[i // NDC, g // 2, k, rows], g % 2 * E, val)

        def convert_wo(g):
            for which in range(2):
                pl.when(g % 2 == which)(gu_copy(which, g // 2).start)
            row_copy(wo_hbm, g).wait()
            convert(st_row.at[g], wo, g * E)

        def convert_gu(c):
            for which in range(2):
                gu_copy(which, c).wait()
                convert(st_col.at[(2 * c + which) % NSTRIP], wgu.at[c], 0, which * LANES)
            pending = c + NSTRIP // 2

            @pl.when(pending < NFC)
            def _():
                for which in range(2):
                    gu_copy(which, pending).start()

            for j in range(2):
                piece = 2 * (pending - NFC) + j
                pl.when((piece >= 0) & (piece < NFC))(
                    row_copy(wd_hbm, jnp.clip(piece, 0, NFC - 1)).start)

        def convert_wd(c):
            row_copy(wd_hbm, c).wait()
            convert(st_row.at[c], wd, c * LANES)

        x_head = pltpu.make_async_copy(x_hbm.at[0:LAG + 2], x_v.at[0:LAG + 2], sem_x.at[0])
        x_rest = pltpu.make_async_copy(x_hbm.at[LAG + 2:NSEG], x_v.at[LAG + 2:NSEG], sem_x.at[1])

        def out_copy(i, lo, hi):
            return pltpu.make_async_copy(x_v.at[lo:hi], out_hbm.at[lo:hi], sem_out.at[i])

        def x_seg(seg):
            return x_v[seg].astype(F32)

        def set_rows(*blocks):
            parts = [_blocks(jnp.concatenate(blk, axis=0)) for blk in blocks]
            for n, a in _left_terms(*parts).items():
                h_s[n] = a

        def attention(nl, residual, before_out=None):
            vis, fill = mask_tables(nl)

            def proj(j, g):
                cols = slice(g % 2 * E, (g % 2 + 1) * E)
                c = _block_product(nl, h_s.__getitem__,
                                   lambda n: _rows(wqkv[j, g // 2, n, :, cols]))
                heads = [jnp.concatenate([row[h] for row in c], axis=0) for h in range(NB)]
                return heads if j == 0 else [x.astype(BF16) for x in heads]

            def proj_all(g):
                k = proj(1, g)
                return proj(0, g), k, proj(2, g)

            def attend(s, v):
                s = jnp.where(vis, s * (scale * LOG2E), fill)
                p = jnp.exp2(s - jnp.max(s, axis=-1, keepdims=True))
                tot = jnp.sum(p, axis=-1, keepdims=True)
                inv = pl.reciprocal(tot, approx=True)
                inv = inv * (2.0 - tot * inv)
                return _dot(p.astype(BF16), v) * inv

            def out_proj(g0, g1, acc):
                if acc is None:
                    acc = _column_tiles([jnp.concatenate([jnp.zeros((M, D), F32), x], axis=0)
                                         for x in residual()])
                return _long_product(
                    lambda n: jnp.concatenate([o_s[n, g] for g in range(g0, g1)], axis=1),
                    wo, g0, g1, acc)

            q, k, v = proj_all(0)
            acc, done = None, 0
            for g in range(NG):
                scores = [_dot_nt(q[h], k[h]) for h in range(NB)]
                for at, upto in (OUT_SPLIT if before_out is None else ()):
                    if at == g:
                        acc, done = out_proj(done, upto, acc), upto
                if g + 1 < NG:
                    nxt = proj_all(g + 1)
                else:
                    yield
                o = [attend(scores[h], v[h]) for h in range(NB)]
                parts = [[x[j * L:(j + 1) * L] for x in o] for j in range(nl)]
                for n, a in _left_terms(*parts).items():
                    o_s[n, g] = a
                q, k, v = nxt
                yield
            if before_out is not None:
                before_out()
                for _, upto in OUT_SPLIT:
                    acc, done = out_proj(done, upto, acc), upto
            acc = out_proj(done, NG, acc)
            yield
            for j, y in enumerate(_row_blocks(acc)):
                y_s[j] = y

        def set_glu_rows(*blocks):
            for n, a in _left_terms(*[_blocks(_ln(b, 0.5)) for b in blocks]).items():
                _store_rows(hb_s.at[n, 0:a.shape[0] // 2], 0, a.astype(BF16))

        def glu(nl, rows, residual, finish, before_down=lambda c: None):
            def gate_up(c):
                g, u = (_block_product(nl, lambda n: _rows(hb_s[n, 0:rows // 2, :]),
                                       lambda n: _rows(wgu[c, n, :, j * LANES:(j + 1) * LANES]))
                        for j in range(2))
                act = [[jnp.tanh(x) * y + y for x, y in zip(gr, ur)] for gr, ur in zip(g, u)]
                for n, a in _left_terms(*act).items():
                    _store_rows(a_s.at[n, 0:rows // 2], c * LANES, a.astype(BF16))

            def down(c0, c1, acc):
                before_down(c0)
                acc = _column_tiles(residual()) if acc is None else acc
                return _long_product(
                    lambda n: _rows(a_s[n, 0:rows // 2, c0 * LANES:c1 * LANES]), wd, c0, c1, acc)

            acc, done = None, 0
            for c in range(NFC):
                gate_up(c)
                for at, upto in DOWN_SPLIT:
                    if at == c:
                        acc, done = down(done, upto, acc), upto
                yield
            finish(_row_blocks(down(done, NFC, acc)))

        x_head.start()
        for i in range(NSTAGE):
            qkv_copy(0, i).start()

        @pl.loop(0, 3 * NDC)
        def _(i):
            for which in range(3):
                pl.when(i // NDC == which)(qkv_copy(which, i).wait)
            convert_qkv(i)
            for which in range(3):
                pl.when((i + NSTAGE) // NDC == which)(qkv_copy(which, i + NSTAGE).start)
            piece = i + NSTAGE - 3 * NDC
            pl.when(piece >= 0)(row_copy(wo_hbm, jnp.maximum(piece, 0)).start)

        for g in range(NSTAGE, NG):
            row_copy(wo_hbm, g).start()
        x_head.wait()
        mem0 = mem_ref[...].astype(F32)
        set_rows((mem0, _ln(x_seg(0))))

        @pl.loop(0, LAG)
        def _(t):
            def convert_arrived():
                pl.loop(0, jnp.where(t == 0, NG, 0))(convert_wo)
                pl.loop(jnp.maximum(t - 1, 0) * EARLY,
                        jnp.where(t + 1 < LAG, t * EARLY, NFC))(convert_gu)

            _run(attention(1, lambda: [x_seg(t)], convert_arrived))
            z_s[t] = y_s[0, M:, :]
            set_rows((y_s[0, :M, :], _ln(x_seg(t + 1))))

        set_glu_rows(z_s[0])

        def head_down(c):
            cut = DOWN_SPLIT[1][1]
            if c in (0, cut):
                pl.loop(c, NFC if c else cut)(convert_wd)

        def head_finish(z):
            z_s[0], = z

        _run(glu(1, T, lambda: [z_s[0]], head_finish, head_down))
        x_rest.start()

        def tokens():
            return [y_s[0, M:, :], y_s[1, M:, :]]

        def step_rows(t):
            set_rows((y_s[0, :M, :], _ln(x_seg(jnp.minimum(t, NSEG - 1)))),
                     (y_s[1, :M, :], _ln(z_s[(t - LAG) % RING])))

        def glu_finish(t):
            def finish(z):
                z_s[t % RING] = z[0]
                x_v[jnp.maximum(t - LAG, 0)] = z[1].astype(x_v.dtype)
            return finish

        y_s[1] = jnp.concatenate([mem0, z_s[1]], axis=0)
        step_rows(LAG)

        def second_step():
            x_rest.wait()
            z_s[1] = x_seg(0)
            step_rows(LAG + 1)

        @pl.loop(LAG, NSEG)
        def _(t):
            pl.when(t == LAG + 1)(second_step)
            set_glu_rows(*tokens())
            d_s[0], d_s[1] = tokens()

            def attention_then_next_rows():
                yield from attention(2, lambda: [x_seg(t), z_s[(t - LAG) % RING]])
                step_rows(t + 1)

            _run(glu(2, T, lambda: [d_s[0], d_s[1]], glu_finish(t - 1)), attention_then_next_rows(),
                 order=(1,) * NG + (0, 1, 0, 0, 1, 1))

        ready = NSEG - 1 - LAG
        out_copy(0, 0, ready).start()
        set_glu_rows(*tokens())
        set_rows((y_s[1, :M, :], _ln(z_s[(NSEG - LAG) % RING])))
        _run(glu(2, T, tokens, glu_finish(NSEG - 1)))

        @pl.loop(NSEG - LAG, NSEG)
        def _(t):
            _run(attention(1, lambda: [z_s[t % RING]]))
            set_rows((y_s[0, :M, :], _ln(z_s[jnp.minimum(t + 1, NSEG - 1) % RING])))
            z_s[t % RING] = y_s[0, M:, :]

        def last_rows():
            y = jnp.concatenate([z_s[t % RING] for t in range(NSEG - LAG, NSEG)], axis=0)
            return y[:LAG * T // 2], y[LAG * T // 2:]

        def last_finish(z):
            z = jnp.concatenate(z, axis=0).astype(x_v.dtype)
            for j in range(LAG):
                x_v[NSEG - LAG + j] = z[j * T:(j + 1) * T]

        set_glu_rows(*last_rows())
        _run(glu(2, LAG * T // 2, last_rows, last_finish))
        out_copy(1, ready, NSEG).start()
        out_copy(0, 0, ready).wait()
        out_copy(1, ready, NSEG).wait()

    dma = pltpu.SemaphoreType.DMA
    nt = len(TERMS)
    scratch = [
        pltpu.VMEM((3, NG // 2, nt, DB // 2, 2 * E), U32),
        pltpu.VMEM((nt, NG * E // 2, DB), U32),
        pltpu.VMEM((NFC, nt, DB // 2, 2 * LANES), U32),
        pltpu.VMEM((nt, NFC * LANES // 2, DB), U32),
        pltpu.VMEM((NSTAGE, NB, DC * H, E), BF16),
        pltpu.VMEM((NB, (PITCH + 7) * H // 2, E), U32),
        pltpu.VMEM((NG, FC, D), BF16),
        pltpu.VMEM((NSTRIP, D, FC), BF16),
        pltpu.VMEM((NSEG, T, D), BF16),
        pltpu.VMEM((nt, L, DB), F32),
        pltpu.VMEM((nt, NG, L, E), F32),
        pltpu.VMEM((nt, LAG * T // 4, DB), U32),
        pltpu.VMEM((nt, LAG * T // 4, NFC * LANES), U32),
        pltpu.VMEM((2, L, D), F32),
        pltpu.VMEM((2, T, D), F32),
        pltpu.VMEM((RING, T, D), F32),
        dma((NSTAGE,)), dma((NG,)), dma((NSTRIP,)), dma((2,)), dma((2,)),
    ]
    return kernel, scratch


@functools.partial(jax.jit, static_argnames=("A_seg_len",))
def pallas_interleave_layers__memory_aug_recurrent_mem_tr__glu_gated_glu__prompt_kernel(
    A_x: jax.Array,
    A_mem0: jax.Array,
    A_Wq: jax.Array,
    A_Wk: jax.Array,
    A_Wv: jax.Array,
    A_Wo: jax.Array,
    A_seg_len: int,
    B_x: jax.Array,
    B_w_gate: jax.Array,
    B_w_up: jax.Array,
    B_w_down: jax.Array,
):
    del B_x
    B, S, D = A_x.shape
    _, H, E = A_Wq.shape
    M = A_mem0.shape[1]
    F = B_w_gate.shape[1]
    T = int(A_seg_len)
    FC = NB * LANES
    assert (B, D, H, E, M, T, F) == (1, 1024, 32, LANES, 8, 32, 3584) and S % T == 0
    kernel, scratch = _make_kernel(S, D, H, E, M, T, F)
    qkv_shape = (NB, D // (NB * DC), DC * H, E)
    hbm = pl.BlockSpec(memory_space=pl.ANY)
    out = pl.pallas_call(
        kernel,
        out_shape=jax.ShapeDtypeStruct((S // T, T, D), A_x.dtype),
        in_specs=[hbm, pl.BlockSpec(memory_space=pltpu.VMEM)] + [hbm] * 7,
        out_specs=hbm,
        scratch_shapes=scratch,
        compiler_params=pltpu.CompilerParams(
            vmem_limit_bytes=127 * 1024 * 1024,
            flags={"XLA_TPU_EVENLY_DISTRIBUTE_CRITICAL_NODES": True}),
    )(A_x.reshape(S // T, T, D), A_mem0.reshape(M, D),
      A_Wq.reshape(qkv_shape), A_Wk.reshape(qkv_shape), A_Wv.reshape(qkv_shape),
      A_Wo.reshape(H * E // FC, FC, D), B_w_gate, B_w_up, B_w_down.reshape(F // FC, FC, D))
    return out.reshape(B, S, D)
```

```python
import functools

import jax
import jax.numpy as jnp
import numpy as np
import jax.experimental.pallas as pl
import jax.experimental.pallas.tpu as pltpu

F32 = jnp.float32
BF16 = jnp.bfloat16
U32 = jnp.uint32
EPS = 1e-5
LOG2E = 1.4426950408889634
LANES = 128
NB = 4
LAG = 3
RING = 4
DC = 32
NSTAGE = 4
NSTRIP = 8
OUT_SPLIT = ((3, 2), (5, 4), (7, 6))
DOWN_SPLIT = ((2, 1), (4, 3), (6, 5))

NODES = (0.5, -0.5, 1.5, -1.5)
TERMS = [term for i in range(NB) for term in (
    [("a", i, i)] + [("q", i, j) for j in range(NB) if j != i]
    + [("r", i, j) for j in range(i + 1, NB)] + [("b", i, i)])]


def _gains(kind, i, j):
    gain = 1.0 / (NODES[j] - NODES[i]) if kind == "q" else 1.0 / (NODES[i] - NODES[j])
    right = abs(gain) if kind == "r" or np.frexp(abs(gain))[0] == 0.5 else 1.0
    return gain / right, right


def _scaled(x, gain):
    return x if gain == 1.0 else x * gain


def _ln(x, gain=1.0):
    m = jnp.mean(x, axis=-1, keepdims=True)
    c = x - m
    v = jnp.mean(c * c, axis=-1, keepdims=True)
    return c * (jax.lax.rsqrt(v + EPS) * gain)


def _rows(words):
    return pltpu.bitcast(words, BF16)


def _store_rows(words_ref, col, rows):
    words_ref.bitcast(BF16)[:, col:col + rows.shape[1]] = rows


def _dot(a, b):
    return jax.lax.dot_general(a, b, (((1,), (0,)), ((), ())), preferred_element_type=F32)


def _dot_nt(a, b):
    return jax.lax.dot_general(a, b, (((1,), (1,)), ((), ())), preferred_element_type=F32)


def _blocks(x):
    n = x.shape[1] // NB
    return [x[:, i * n:(i + 1) * n] for i in range(NB)]


def _left_terms(s, d=None):
    if d is None:
        return {n: s[i] for n, (kind, i, _) in enumerate(TERMS) if kind == "a"}
    ts = {t: [t * x for x in s] for t in NODES if t > 0}
    e = [[d[i] + ts[t][i] if t > 0 else d[i] - ts[-t][i] for i in range(NB)] for t in NODES]
    out = {}
    for n, (kind, i, j) in enumerate(TERMS):
        if kind == "a":
            out[n] = s[i]
        elif kind == "b":
            out[n] = e[i][i]
        else:
            x, y = e[j if kind == "q" else i][i], e[j][j]
            gain = _gains(kind, i, j)[0]
            out[n] = _scaled(x - y if gain > 0 else y - x, abs(gain))
    return out


def _right_terms(w):
    f = [[b.astype(F32) for b in row] for row in w]
    out = []
    for kind, i, j in TERMS:
        if kind in "qr":
            gain = _gains(kind, i, j)[1]
            if kind == "q" and gain == 1.0:
                val = w[i][j]
            else:
                val = _scaled(f[i][j] if kind == "q" else f[i][j] + f[j][i], gain)
        else:
            val = f[i][i]
            for k in range(NB):
                if k != i:
                    val = val - f[i][k] if kind == "a" else val + f[k][i]
        out.append(val.astype(BF16))
    return out


def _block_product(nl, left, right, acc=None):
    acc = [[None] * NB for _ in range(nl)] if acc is None else [list(row) for row in acc]

    def add(row, j, x):
        acc[row][j] = x if acc[row][j] is None else acc[row][j] + x

    for n, (kind, i, j) in enumerate(TERMS):
        if nl == 1:
            if kind in "aq":
                p = _dot(left(TERMS.index(("a", i, i))), right(n))
                if kind == "q":
                    p = _scaled(p, 1.0 / _gains(kind, i, j)[1])
                    add(0, j, p)
                add(0, i, p)
            continue
        p = _dot(left(n), right(n))
        if kind == "a":
            u = p
        elif kind == "b":
            add(0, i, u)
            add(1, i, p - NODES[i] * u)
        else:
            u = u + p
            add(0, j, p)
            add(1, j, -NODES[i if kind == "q" else j] * p)
    return acc


def _long_product(left, right_ref, k0, k1, acc):
    def right(c, n):
        return _rows(right_ref[n, k0 * LANES // 2:k1 * LANES // 2, c * LANES:(c + 1) * LANES])

    return [_block_product(len(old), left, functools.partial(right, c), old)
            for c, old in enumerate(acc)]


def _column_tiles(row_blocks):
    width = row_blocks[0].shape[1] // NB
    return [[[b[:, j * width + c:j * width + c + LANES] for j in range(NB)] for b in row_blocks]
            for c in range(0, width, LANES)]


def _row_blocks(tiles):
    return [jnp.concatenate([t[r][j] for j in range(NB) for t in tiles], axis=1)
            for r in range(len(tiles[0]))]


def _run(*gens, order=()):
    for which in order:
        next(gens[which], None)
    for gen in gens:
        for _ in gen:
            pass


def _make_kernel(S, D, H, E, M, T, F):
    NSEG = S // T
    NG = H // NB
    DB = D // NB
    NDC = DB // DC
    PITCH = DC + 1
    FC = NB * LANES
    NFC = F // FC
    EARLY = NSTRIP // 2
    L = M + T
    scale = float(E) ** -0.5
    assert NSTRIP == NG >= NFC and NSEG > LAG + 2

    def mask_tables(nl):
        r = jax.lax.broadcasted_iota(jnp.int32, (nl * L, nl * L), 0)
        c = jax.lax.broadcasted_iota(jnp.int32, (nl * L, nl * L), 1)
        same = (r < L) == (c < L)
        vis = same & ((jnp.where(r < L, r, r - L) < M) | (c <= r))
        return vis, jnp.where(same, -1e9 * LOG2E, -jnp.inf).astype(F32)

    def kernel(x_hbm, mem_ref, wq_hbm, wk_hbm, wv_hbm, wo_hbm, wg_hbm, wu_hbm, wd_hbm, out_hbm,
               wqkv, wo, wgu, wd, st_qkv, st_word, st_row, st_col, x_v,
               h_s, o_s, hb_s, y_s, d_s, z_s,
               sem_qkv, sem_row, sem_col, sem_x, sem_out):
        def qkv_copy(which, i):
            return pltpu.make_async_copy((wq_hbm, wk_hbm, wv_hbm)[which].at[:, i % NDC],
                                         st_qkv.at[i % NSTAGE], sem_qkv.at[i % NSTAGE])

        def row_copy(src, i):
            return pltpu.make_async_copy(src.at[i], st_row.at[i], sem_row.at[i])

        def gu_copy(which, c):
            slot = (2 * c + which) % NSTRIP
            cols = pl.ds(pl.multiple_of(c * FC, FC), FC)
            return pltpu.make_async_copy((wg_hbm, wu_hbm)[which].at[:, cols],
                                         st_col.at[slot], sem_col.at[slot])

        def convert(src, dst, row0=0, col0=0):
            n = src.shape[0] // NB
            sub = 32 * FC // src.shape[1]

            @pl.loop(0, n // sub)
            def _(r):
                w = [_blocks(src[pl.ds(pl.multiple_of(i * n + r * sub, sub), sub), :])
                     for i in range(NB)]
                rows = pl.ds(pl.multiple_of((row0 + r * sub) // 2, sub // 2), sub // 2)
                for k, val in enumerate(_right_terms(w)):
                    _store_rows(dst.at[k, rows], col0, val)

        def convert_qkv(i):
            for b in range(NB):
                for d in range(DC):
                    st_word[b, pl.ds(d // 2 + d % 2 * DC // 2, H // 2, stride=PITCH), :] = (
                        pltpu.bitcast(st_qkv[i % NSTAGE, b, d * H:(d + 1) * H, :], U32))
            rows = pl.ds(pl.multiple_of((i % NDC) * (DC // 2), DC // 2), DC // 2)
            for g in range(NG):
                w = []
                for b in range(NB):
                    w.append([])
                    for pair in range(g * NB // 2, (g + 1) * NB // 2):
                        x = st_word[b, pl.ds(pair * PITCH, DC // 2), :]
                        y = st_word[b, pl.ds(pair * PITCH + DC // 2, DC // 2), :]
                        w[-1].append(_rows((x & np.uint32(0xFFFF)) | (y << 16)))
                        w[-1].append(_rows((x >> 16) | (y & np.uint32(0xFFFF0000))))
                for k, val in enumerate(_right_terms(w)):
                    _store_rows(wqkv.at[i // NDC, g // 2, k, rows], g % 2 * E, val)

        def convert_wo(g):
            for which in range(2):
                pl.when(g % 2 == which)(gu_copy(which, g // 2).start)
            row_copy(wo_hbm, g).wait()
            convert(st_row.at[g], wo, g * E)

        def convert_gu(c):
            for which in range(2):
                gu_copy(which, c).wait()
                convert(st_col.at[(2 * c + which) % NSTRIP], wgu.at[c], 0, which * LANES)
            pending = c + NSTRIP // 2

            @pl.when(pending < NFC)
            def _():
                for which in range(2):
                    gu_copy(which, pending).start()

            for j in range(2):
                piece = 2 * (pending - NFC) + j
                pl.when((piece >= 0) & (piece < NFC))(
                    row_copy(wd_hbm, jnp.clip(piece, 0, NFC - 1)).start)

        def convert_wd(c):
            row_copy(wd_hbm, c).wait()
            convert(st_row.at[c], wd, c * LANES)

        x_head = pltpu.make_async_copy(x_hbm.at[0:LAG + 2], x_v.at[0:LAG + 2], sem_x.at[0])
        x_rest = pltpu.make_async_copy(x_hbm.at[LAG + 2:NSEG], x_v.at[LAG + 2:NSEG], sem_x.at[1])

        def out_copy(i, lo, hi):
            return pltpu.make_async_copy(x_v.at[lo:hi], out_hbm.at[lo:hi], sem_out.at[i])

        def x_seg(seg):
            return x_v[seg].astype(F32)

        def set_rows(*blocks):
            for j, (mem, tok) in enumerate(blocks):
                h_s[j, :M, :] = mem
                h_s[j, M:, :] = tok

        def attention(nl, residual, before_out=None):
            vis, fill = mask_tables(nl)
            h = _left_terms(*[_blocks(h_s[j]) for j in range(nl)])

            def proj(j, g):
                cols = slice(g % 2 * E, (g % 2 + 1) * E)
                c = _block_product(nl, h.__getitem__,
                                   lambda n: _rows(wqkv[j, g // 2, n, :, cols]))
                heads = [jnp.concatenate([row[h] for row in c], axis=0) for h in range(NB)]
                return heads if j == 0 else [x.astype(BF16) for x in heads]

            def proj_all(g):
                k = proj(1, g)
                return proj(0, g), k, proj(2, g)

            def attend(s, v):
                s = jnp.where(vis, s * (scale * LOG2E), fill)
                p = jnp.exp2(s - jnp.max(s, axis=-1, keepdims=True))
                tot = jnp.sum(p, axis=-1, keepdims=True)
                inv = pl.reciprocal(tot, approx=True)
                inv = inv * (2.0 - tot * inv)
                return _dot(p, v) * inv

            def out_proj(g0, g1, acc):
                if acc is None:
                    acc = _column_tiles([jnp.concatenate([jnp.zeros((M, D), F32), x], axis=0)
                                         for x in residual()])
                return _long_product(
                    lambda n: jnp.concatenate([o_s[n, g] for g in range(g0, g1)], axis=1),
                    wo, g0, g1, acc)

            q, k, v = proj_all(0)
            acc, done = None, 0
            for g in range(NG):
                scores = [_dot_nt(q[h], k[h]) for h in range(NB)]
                for at, upto in (OUT_SPLIT if before_out is None else ()):
                    if at == g:
                        acc, done = out_proj(done, upto, acc), upto
                if g + 1 < NG:
                    nxt = proj_all(g + 1)
                else:
                    yield
                o = [attend(scores[h], v[h]) for h in range(NB)]
                parts = [[x[j * L:(j + 1) * L] for x in o] for j in range(nl)]
                for n, a in _left_terms(*parts).items():
                    o_s[n, g] = a
                q, k, v = nxt
                yield
            if before_out is not None:
                before_out()
                for _, upto in OUT_SPLIT:
                    acc, done = out_proj(done, upto, acc), upto
            acc = out_proj(done, NG, acc)
            yield
            for j, y in enumerate(_row_blocks(acc)):
                y_s[j] = y

        def set_glu_rows(*blocks):
            for j, b in enumerate(blocks):
                hb_s[j, 0:b.shape[0], :] = _ln(b, 0.5)

        def glu(nl, rows, residual, finish, before_down=lambda c: None):
            hb = _left_terms(*[_blocks(hb_s[j, 0:rows, :]) for j in range(nl)])
            hb = {n: a.astype(BF16) for n, a in hb.items()}

            acts = []

            def gate_up(c):
                g, u = (_block_product(nl, hb.__getitem__,
                                       lambda n: _rows(wgu[c, n, :, j * LANES:(j + 1) * LANES]))
                        for j in range(2))
                act = [[jnp.tanh(x) * y + y for x, y in zip(gr, ur)] for gr, ur in zip(g, u)]
                acts.append(_left_terms(*act))

            def down(c0, c1, acc):
                before_down(c0)
                acc = _column_tiles(residual()) if acc is None else acc
                return _long_product(
                    lambda n: jnp.concatenate([acts[c][n] for c in range(c0, c1)], axis=1),
                    wd, c0, c1, acc)

            acc, done = None, 0
            for c in range(NFC):
                gate_up(c)
                for at, upto in DOWN_SPLIT:
                    if at == c:
                        acc, done = down(done, upto, acc), upto
                yield
            finish(_row_blocks(down(done, NFC, acc)))

        x_head.start()
        for i in range(NSTAGE):
            qkv_copy(0, i).start()

        @pl.loop(0, 3 * NDC)
        def _(i):
            for which in range(3):
                pl.when(i // NDC == which)(qkv_copy(which, i).wait)
            convert_qkv(i)
            for which in range(3):
                pl.when((i + NSTAGE) // NDC == which)(qkv_copy(which, i + NSTAGE).start)
            piece = i + NSTAGE - 3 * NDC
            pl.when(piece >= 0)(row_copy(wo_hbm, jnp.maximum(piece, 0)).start)

        for g in range(NSTAGE, NG):
            row_copy(wo_hbm, g).start()
        x_head.wait()
        mem0 = mem_ref[...].astype(F32)
        set_rows((mem0, _ln(x_seg(0))))

        @pl.loop(0, LAG)
        def _(t):
            def convert_arrived():
                pl.loop(0, jnp.where(t == 0, NG, 0))(convert_wo)
                pl.loop(jnp.maximum(t - 1, 0) * EARLY,
                        jnp.where(t + 1 < LAG, t * EARLY, NFC))(convert_gu)

            _run(attention(1, lambda: [x_seg(t)], convert_arrived))
            z_s[t] = y_s[0, M:, :]
            set_rows((y_s[0, :M, :], _ln(x_seg(t + 1))))

        set_glu_rows(z_s[0])

        def head_down(c):
            cut = DOWN_SPLIT[1][1]
            if c in (0, cut):
                pl.loop(c, NFC if c else cut)(convert_wd)

        def head_finish(z):
            z_s[0], = z

        _run(glu(1, T, lambda: [z_s[0]], head_finish, head_down))
        x_rest.start()

        def tokens():
            return [y_s[0, M:, :], y_s[1, M:, :]]

        def step_rows(t):
            set_rows((y_s[0, :M, :], _ln(x_seg(jnp.minimum(t, NSEG - 1)))),
                     (y_s[1, :M, :], _ln(z_s[(t - LAG) % RING])))

        def glu_finish(t):
            def finish(z):
                z_s[t % RING] = z[0]
                x_v[jnp.maximum(t - LAG, 0)] = z[1].astype(x_v.dtype)
            return finish

        y_s[1] = jnp.concatenate([mem0, z_s[1]], axis=0)
        step_rows(LAG)
        set_glu_rows(*tokens())

        def second_step():
            x_rest.wait()
            z_s[1] = x_seg(0)
            step_rows(LAG + 1)

        @pl.loop(LAG, NSEG)
        def _(t):
            pl.when(t == LAG + 1)(second_step)
            d_s[0], d_s[1] = tokens()

            def attention_then_next_rows():
                yield from attention(2, lambda: [x_seg(t), z_s[(t - LAG) % RING]])
                step_rows(t + 1)
                set_glu_rows(*tokens())

            _run(glu(2, T, lambda: [d_s[0], d_s[1]], glu_finish(t - 1)), attention_then_next_rows(),
                 order=(1,) * NG + (0, 1, 0, 0, 1, 1))

        ready = NSEG - 1 - LAG
        out_copy(0, 0, ready).start()
        set_rows((y_s[1, :M, :], _ln(z_s[(NSEG - LAG) % RING])))
        _run(glu(2, T, tokens, glu_finish(NSEG - 1)))

        @pl.loop(NSEG - LAG, NSEG)
        def _(t):
            _run(attention(1, lambda: [z_s[t % RING]]))
            set_rows((y_s[0, :M, :], _ln(z_s[jnp.minimum(t + 1, NSEG - 1) % RING])))
            z_s[t % RING] = y_s[0, M:, :]

        def last_rows():
            y = jnp.concatenate([z_s[t % RING] for t in range(NSEG - LAG, NSEG)], axis=0)
            return y[:LAG * T // 2], y[LAG * T // 2:]

        def last_finish(z):
            z = jnp.concatenate(z, axis=0).astype(x_v.dtype)
            for j in range(LAG):
                x_v[NSEG - LAG + j] = z[j * T:(j + 1) * T]

        set_glu_rows(*last_rows())
        _run(glu(2, LAG * T // 2, last_rows, last_finish))
        out_copy(1, ready, NSEG).start()
        out_copy(0, 0, ready).wait()
        out_copy(1, ready, NSEG).wait()

    dma = pltpu.SemaphoreType.DMA
    nt = len(TERMS)
    scratch = [
        pltpu.VMEM((3, NG // 2, nt, DB // 2, 2 * E), U32),
        pltpu.VMEM((nt, NG * E // 2, DB), U32),
        pltpu.VMEM((NFC, nt, DB // 2, 2 * LANES), U32),
        pltpu.VMEM((nt, NFC * LANES // 2, DB), U32),
        pltpu.VMEM((NSTAGE, NB, DC * H, E), BF16),
        pltpu.VMEM((NB, (PITCH + 7) * H // 2, E), U32),
        pltpu.VMEM((NG, FC, D), BF16),
        pltpu.VMEM((NSTRIP, D, FC), BF16),
        pltpu.VMEM((NSEG, T, D), BF16),
        pltpu.VMEM((2, L, D), F32),
        pltpu.VMEM((nt, NG, L, E), F32),
        pltpu.VMEM((2, LAG * T // 2, D), F32),
        pltpu.VMEM((2, L, D), F32),
        pltpu.VMEM((2, T, D), F32),
        pltpu.VMEM((RING, T, D), F32),
        dma((NSTAGE,)), dma((NG,)), dma((NSTRIP,)), dma((2,)), dma((2,)),
    ]
    return kernel, scratch


@functools.partial(jax.jit, static_argnames=("A_seg_len",))
def pallas_interleave_layers__memory_aug_recurrent_mem_tr__glu_gated_glu__prompt_kernel(
    A_x: jax.Array,
    A_mem0: jax.Array,
    A_Wq: jax.Array,
    A_Wk: jax.Array,
    A_Wv: jax.Array,
    A_Wo: jax.Array,
    A_seg_len: int,
    B_x: jax.Array,
    B_w_gate: jax.Array,
    B_w_up: jax.Array,
    B_w_down: jax.Array,
):
    del B_x
    B, S, D = A_x.shape
    _, H, E = A_Wq.shape
    M = A_mem0.shape[1]
    F = B_w_gate.shape[1]
    T = int(A_seg_len)
    FC = NB * LANES
    assert (B, D, H, E, M, T, F) == (1, 1024, 32, LANES, 8, 32, 3584) and S % T == 0
    kernel, scratch = _make_kernel(S, D, H, E, M, T, F)
    qkv_shape = (NB, D // (NB * DC), DC * H, E)
    hbm = pl.BlockSpec(memory_space=pl.ANY)
    out = pl.pallas_call(
        kernel,
        out_shape=jax.ShapeDtypeStruct((S // T, T, D), A_x.dtype),
        in_specs=[hbm, pl.BlockSpec(memory_space=pltpu.VMEM)] + [hbm] * 7,
        out_specs=hbm,
        scratch_shapes=scratch,
        compiler_params=pltpu.CompilerParams(
            vmem_limit_bytes=127 * 1024 * 1024),
    )(A_x.reshape(S // T, T, D), A_mem0.reshape(M, D),
      A_Wq.reshape(qkv_shape), A_Wk.reshape(qkv_shape), A_Wv.reshape(qkv_shape),
      A_Wo.reshape(H * E // FC, FC, D), B_w_gate, B_w_up, B_w_down.reshape(F // FC, FC, D))
    return out.reshape(B, S, D)
```

```python
import functools

import jax
import jax.numpy as jnp
import numpy as np
import jax.experimental.pallas as pl
import jax.experimental.pallas.tpu as pltpu

F32 = jnp.float32
BF16 = jnp.bfloat16
U32 = jnp.uint32
EPS = 1e-5
LOG2E = 1.4426950408889634
LANES = 128
NB = 4
LAG = 3
RING = 4
DC = 32
NSTAGE = 4
NSTRIP = 8
OUT_SPLIT = ((3, 2), (5, 4), (7, 6))
DOWN_SPLIT = ((2, 1), (4, 3), (6, 5))

NODES = (0.5, -0.5, 1.5, -1.5)
TERMS = [term for i in range(NB) for term in (
    [("a", i, i)] + [("q", i, j) for j in range(NB) if j != i]
    + [("r", i, j) for j in range(i + 1, NB)] + [("b", i, i)])]


def _gains(kind, i, j):
    gain = 1.0 / (NODES[j] - NODES[i]) if kind == "q" else 1.0 / (NODES[i] - NODES[j])
    right = abs(gain) if kind == "r" or np.frexp(abs(gain))[0] == 0.5 else 1.0
    return gain / right, right


def _scaled(x, gain):
    return x if gain == 1.0 else x * gain


def _ln(x, gain=1.0):
    m = jnp.mean(x, axis=-1, keepdims=True)
    c = x - m
    v = jnp.mean(c * c, axis=-1, keepdims=True)
    return c * (jax.lax.rsqrt(v + EPS) * gain)


def _rows(words):
    return pltpu.bitcast(words, BF16)


def _store_rows(words_ref, col, rows):
    words_ref.bitcast(BF16)[:, col:col + rows.shape[1]] = rows


def _dot(a, b):
    return jax.lax.dot_general(a, b, (((1,), (0,)), ((), ())), preferred_element_type=F32)


def _dot_nt(a, b):
    return jax.lax.dot_general(a, b, (((1,), (1,)), ((), ())), preferred_element_type=F32)


def _blocks(x):
    n = x.shape[1] // NB
    return [x[:, i * n:(i + 1) * n] for i in range(NB)]


def _left_terms(s, d=None):
    if d is None:
        return {n: s[i] for n, (kind, i, _) in enumerate(TERMS) if kind == "a"}
    ts = {t: [t * x for x in s] for t in NODES if t > 0}
    e = [[d[i] + ts[t][i] if t > 0 else d[i] - ts[-t][i] for i in range(NB)] for t in NODES]
    out = {}
    for n, (kind, i, j) in enumerate(TERMS):
        if kind == "a":
            out[n] = s[i]
        elif kind == "b":
            out[n] = e[i][i]
        else:
            x, y = e[j if kind == "q" else i][i], e[j][j]
            gain = _gains(kind, i, j)[0]
            out[n] = _scaled(x - y if gain > 0 else y - x, abs(gain))
    return out


def _right_terms(w):
    f = [[b.astype(F32) for b in row] for row in w]
    out = []
    for kind, i, j in TERMS:
        if kind in "qr":
            gain = _gains(kind, i, j)[1]
            if kind == "q" and gain == 1.0:
                val = w[i][j]
            else:
                val = _scaled(f[i][j] if kind == "q" else f[i][j] + f[j][i], gain)
        else:
            val = f[i][i]
            for k in range(NB):
                if k != i:
                    val = val - f[i][k] if kind == "a" else val + f[k][i]
        out.append(val.astype(BF16))
    return out


def _block_product(nl, left, right, acc=None):
    acc = [[None] * NB for _ in range(nl)] if acc is None else [list(row) for row in acc]

    def add(row, j, x):
        acc[row][j] = x if acc[row][j] is None else acc[row][j] + x

    for n, (kind, i, j) in enumerate(TERMS):
        if nl == 1:
            if kind in "aq":
                p = _dot(left(TERMS.index(("a", i, i))), right(n))
                if kind == "q":
                    p = _scaled(p, 1.0 / _gains(kind, i, j)[1])
                    add(0, j, p)
                add(0, i, p)
            continue
        p = _dot(left(n), right(n))
        if kind == "a":
            u = p
        elif kind == "b":
            add(0, i, u)
            add(1, i, p - NODES[i] * u)
        else:
            u = u + p
            add(0, j, p)
            add(1, j, -NODES[i if kind == "q" else j] * p)
    return acc


def _long_product(left, right_ref, k0, k1, acc):
    def right(c, n):
        return _rows(right_ref[n, k0 * LANES // 2:k1 * LANES // 2, c * LANES:(c + 1) * LANES])

    return [_block_product(len(old), left, functools.partial(right, c), old)
            for c, old in enumerate(acc)]


def _column_tiles(row_blocks):
    width = row_blocks[0].shape[1] // NB
    return [[[b[:, j * width + c:j * width + c + LANES] for j in range(NB)] for b in row_blocks]
            for c in range(0, width, LANES)]


def _row_blocks(tiles):
    return [jnp.concatenate([t[r][j] for j in range(NB) for t in tiles], axis=1)
            for r in range(len(tiles[0]))]


def _run(*gens, order=()):
    for which in order:
        next(gens[which], None)
    for gen in gens:
        for _ in gen:
            pass


def _make_kernel(S, D, H, E, M, T, F):
    NSEG = S // T
    NG = H // NB
    DB = D // NB
    NDC = DB // DC
    PITCH = DC + 1
    FC = NB * LANES
    NFC = F // FC
    EARLY = NSTRIP // 2
    L = M + T
    scale = float(E) ** -0.5
    assert NSTRIP == NG >= NFC and NSEG > LAG + 2

    def mask_tables(nl):
        r = jax.lax.broadcasted_iota(jnp.int32, (nl * L, nl * L), 0)
        c = jax.lax.broadcasted_iota(jnp.int32, (nl * L, nl * L), 1)
        same = (r < L) == (c < L)
        vis = same & ((jnp.where(r < L, r, r - L) < M) | (c <= r))
        return vis, jnp.where(same, -1e9 * LOG2E, -jnp.inf).astype(F32)

    def kernel(x_hbm, mem_ref, wq_hbm, wk_hbm, wv_hbm, wo_hbm, wg_hbm, wu_hbm, wd_hbm, out_hbm,
               wqkv, wo, wgu, wd, st_qkv, st_word, st_row, st_col, x_v,
               h_s, o_s, hb_s, y_s, z_s, out_s,
               sem_qkv, sem_row, sem_col, sem_x, sem_out):
        def qkv_copy(which, i):
            return pltpu.make_async_copy((wq_hbm, wk_hbm, wv_hbm)[which].at[:, i % NDC],
                                         st_qkv.at[i % NSTAGE], sem_qkv.at[i % NSTAGE])

        def row_copy(src, i):
            return pltpu.make_async_copy(src.at[i], st_row.at[i], sem_row.at[i])

        def gu_copy(which, c):
            slot = (2 * c + which) % NSTRIP
            cols = pl.ds(pl.multiple_of(c * FC, FC), FC)
            return pltpu.make_async_copy((wg_hbm, wu_hbm)[which].at[:, cols],
                                         st_col.at[slot], sem_col.at[slot])

        def convert(src, dst, row0=0, col0=0):
            n = src.shape[0] // NB
            sub = 32 * FC // src.shape[1]

            @pl.loop(0, n // sub)
            def _(r):
                w = [_blocks(src[pl.ds(pl.multiple_of(i * n + r * sub, sub), sub), :])
                     for i in range(NB)]
                rows = pl.ds(pl.multiple_of((row0 + r * sub) // 2, sub // 2), sub // 2)
                for k, val in enumerate(_right_terms(w)):
                    _store_rows(dst.at[k, rows], col0, val)

        def convert_qkv(i):
            for b in range(NB):
                for d in range(DC):
                    st_word[b, pl.ds(d // 2 + d % 2 * DC // 2, H // 2, stride=PITCH), :] = (
                        pltpu.bitcast(st_qkv[i % NSTAGE, b, d * H:(d + 1) * H, :], U32))
            rows = pl.ds(pl.multiple_of((i % NDC) * (DC // 2), DC // 2), DC // 2)
            for g in range(NG):
                w = []
                for b in range(NB):
                    w.append([])
                    for pair in range(g * NB // 2, (g + 1) * NB // 2):
                        x = st_word[b, pl.ds(pair * PITCH, DC // 2), :]
                        y = st_word[b, pl.ds(pair * PITCH + DC // 2, DC // 2), :]
                        w[-1].append(_rows((x & np.uint32(0xFFFF)) | (y << 16)))
                        w[-1].append(_rows((x >> 16) | (y & np.uint32(0xFFFF0000))))
                for k, val in enumerate(_right_terms(w)):
                    _store_rows(wqkv.at[i // NDC, g // 2, k, rows], g % 2 * E, val)

        def convert_wo(g):
            for which in range(2):
                pl.when(g % 2 == which)(gu_copy(which, g // 2).start)
            row_copy(wo_hbm, g).wait()
            convert(st_row.at[g], wo, g * E)

        def convert_gu(c):
            for which in range(2):
                gu_copy(which, c).wait()
                convert(st_col.at[(2 * c + which) % NSTRIP], wgu.at[c], 0, which * LANES)
            pending = c + NSTRIP // 2

            @pl.when(pending < NFC)
            def _():
                for which in range(2):
                    gu_copy(which, pending).start()

            for j in range(2):
                piece = 2 * (pending - NFC) + j
                pl.when((piece >= 0) & (piece < NFC))(
                    row_copy(wd_hbm, jnp.clip(piece, 0, NFC - 1)).start)

        def convert_wd(c):
            row_copy(wd_hbm, c).wait()
            convert(st_row.at[c], wd, c * LANES)

        x_head = pltpu.make_async_copy(x_hbm.at[0:LAG + 2], x_v.at[0:LAG + 2], sem_x.at[0])
        x_rest = pltpu.make_async_copy(x_hbm.at[LAG + 2:NSEG], x_v.at[LAG + 2:NSEG], sem_x.at[1])

        def out_copy(i, lo, hi):
            return pltpu.make_async_copy(x_v.at[lo:hi], out_hbm.at[lo:hi], sem_out.at[i])

        def x_seg(seg):
            return x_v[seg].astype(F32)

        def set_rows(*blocks):
            for j, (mem, tok) in enumerate(blocks):
                h_s[j, :M, :] = mem
                h_s[j, M:, :] = tok

        def attention(nl, residual, before_out=None):
            vis, fill = mask_tables(nl)
            h = _left_terms(*[_blocks(h_s[j]) for j in range(nl)])

            def proj(j, g):
                cols = slice(g % 2 * E, (g % 2 + 1) * E)
                c = _block_product(nl, h.__getitem__,
                                   lambda n: _rows(wqkv[j, g // 2, n, :, cols]))
                heads = [jnp.concatenate([row[h] for row in c], axis=0) for h in range(NB)]
                return heads if j == 0 else [x.astype(BF16) for x in heads]

            def proj_all(g):
                k = proj(1, g)
                return proj(0, g), k, proj(2, g)

            def attend(s, v):
                s = jnp.where(vis, s * (scale * LOG2E), fill)
                p = jnp.exp2(s - jnp.max(s, axis=-1, keepdims=True))
                tot = jnp.sum(p, axis=-1, keepdims=True)
                inv = pl.reciprocal(tot, approx=True)
                inv = inv * (2.0 - tot * inv)
                return _dot(p, v) * inv

            def out_proj(g0, g1, acc):
                if acc is None:
                    acc = _column_tiles([jnp.concatenate([jnp.zeros((M, D), F32), x], axis=0)
                                         for x in residual()])
                return _long_product(
                    lambda n: jnp.concatenate([o_s[n, g] for g in range(g0, g1)], axis=1),
                    wo, g0, g1, acc)

            q, k, v = proj_all(0)
            acc, done = None, 0
            for g in range(NG):
                scores = [_dot_nt(q[h], k[h]) for h in range(NB)]
                for at, upto in (OUT_SPLIT if before_out is None else ()):
                    if at == g:
                        acc, done = out_proj(done, upto, acc), upto
                if g + 1 < NG:
                    nxt = proj_all(g + 1)
                else:
                    yield
                o = [attend(scores[h], v[h]) for h in range(NB)]
                parts = [[x[j * L:(j + 1) * L] for x in o] for j in range(nl)]
                for n, a in _left_terms(*parts).items():
                    o_s[n, g] = a
                q, k, v = nxt
                yield
            if before_out is not None:
                before_out()
                for _, upto in OUT_SPLIT:
                    acc, done = out_proj(done, upto, acc), upto
            acc = out_proj(done, NG, acc)
            yield
            for j, y in enumerate(_row_blocks(acc)):
                y_s[j] = y

        def set_glu_rows(*blocks):
            for j, b in enumerate(blocks):
                hb_s[j, 0:b.shape[0], :] = _ln(b, 0.5)

        def glu(nl, rows, residual, finish, before_down=lambda c: None):
            hb = _left_terms(*[_blocks(hb_s[j, 0:rows, :]) for j in range(nl)])
            hb = {n: a.astype(BF16) for n, a in hb.items()}

            acts = []

            def gate_up(c):
                g, u = (_block_product(nl, hb.__getitem__,
                                       lambda n: _rows(wgu[c, n, :, j * LANES:(j + 1) * LANES]))
                        for j in range(2))
                act = [[jnp.tanh(x) * y + y for x, y in zip(gr, ur)] for gr, ur in zip(g, u)]
                acts.append(_left_terms(*act))

            def down(c0, c1, acc):
                before_down(c0)
                acc = _column_tiles(residual()) if acc is None else acc
                return _long_product(
                    lambda n: jnp.concatenate([acts[c][n] for c in range(c0, c1)], axis=1),
                    wd, c0, c1, acc)

            acc, done = None, 0
            for c in range(NFC):
                gate_up(c)
                for at, upto in DOWN_SPLIT:
                    if at == c:
                        acc, done = down(done, upto, acc), upto
                yield
            finish(_row_blocks(down(done, NFC, acc)))

        x_head.start()
        for i in range(NSTAGE):
            qkv_copy(0, i).start()

        @pl.loop(0, 3 * NDC)
        def _(i):
            for which in range(3):
                pl.when(i // NDC == which)(qkv_copy(which, i).wait)
            convert_qkv(i)
            for which in range(3):
                pl.when((i + NSTAGE) // NDC == which)(qkv_copy(which, i + NSTAGE).start)
            piece = i + NSTAGE - 3 * NDC
            pl.when(piece >= 0)(row_copy(wo_hbm, jnp.maximum(piece, 0)).start)

        for g in range(NSTAGE, NG):
            row_copy(wo_hbm, g).start()
        x_head.wait()
        mem0 = mem_ref[...].astype(F32)
        set_rows((mem0, _ln(x_seg(0))))

        @pl.loop(0, LAG)
        def _(t):
            def convert_arrived():
                pl.loop(0, jnp.where(t == 0, NG, 0))(convert_wo)
                pl.loop(jnp.maximum(t - 1, 0) * EARLY,
                        jnp.where(t + 1 < LAG, t * EARLY, NFC))(convert_gu)

            _run(attention(1, lambda: [x_seg(t)], convert_arrived))
            z_s[t] = y_s[0, M:, :]
            set_rows((y_s[0, :M, :], _ln(x_seg(t + 1))))

        set_glu_rows(z_s[0])

        def head_down(c):
            cut = DOWN_SPLIT[1][1]
            if c in (0, cut):
                pl.loop(c, NFC if c else cut)(convert_wd)

        def head_finish(z):
            z_s[0], = z

        _run(glu(1, T, lambda: [z_s[0]], head_finish, head_down))
        x_rest.start()

        def tokens():
            return [y_s[0, M:, :], y_s[1, M:, :]]

        def step_rows(t):
            set_rows((y_s[0, :M, :], _ln(x_seg(jnp.minimum(t, NSEG - 1)))),
                     (y_s[1, :M, :], _ln(z_s[(t - LAG) % RING])))

        def glu_finish(t):
            def finish(z):
                z_s[t % RING], out_s[...] = z
            return finish

        y_s[1] = jnp.concatenate([mem0, z_s[1]], axis=0)
        out_s[...] = z_s[0]
        step_rows(LAG)
        set_glu_rows(*tokens())

        def emit(seg):
            x_v[seg] = out_s[...].astype(x_v.dtype)

        def second_step():
            x_rest.wait()
            z_s[1] = out_s[...]
            step_rows(LAG + 1)

        @pl.loop(LAG, NSEG)
        def _(t):
            pl.when(t == LAG + 1)(second_step)
            emit(jnp.maximum(t - 2 - LAG, 0))
            previous = tokens()

            def attention_then_next_rows():
                yield from attention(2, lambda: [x_seg(t), z_s[(t - LAG) % RING]])
                step_rows(t + 1)
                set_glu_rows(*tokens())

            _run(glu(2, T, lambda: previous, glu_finish(t - 1)), attention_then_next_rows(),
                 order=(1,) * NG + (0, 1, 0, 0, 1, 1))

        ready = NSEG - 1 - LAG
        emit(NSEG - 2 - LAG)
        out_copy(0, 0, ready).start()
        set_rows((y_s[1, :M, :], _ln(z_s[(NSEG - LAG) % RING])))
        _run(glu(2, T, tokens, glu_finish(NSEG - 1)))
        emit(NSEG - 1 - LAG)

        @pl.loop(NSEG - LAG, NSEG)
        def _(t):
            _run(attention(1, lambda: [z_s[t % RING]]))
            set_rows((y_s[0, :M, :], _ln(z_s[jnp.minimum(t + 1, NSEG - 1) % RING])))
            z_s[t % RING] = y_s[0, M:, :]

        def last_rows():
            y = jnp.concatenate([z_s[t % RING] for t in range(NSEG - LAG, NSEG)], axis=0)
            return y[:LAG * T // 2], y[LAG * T // 2:]

        def last_finish(z):
            z = jnp.concatenate(z, axis=0).astype(x_v.dtype)
            for j in range(LAG):
                x_v[NSEG - LAG + j] = z[j * T:(j + 1) * T]

        set_glu_rows(*last_rows())
        _run(glu(2, LAG * T // 2, last_rows, last_finish))
        out_copy(1, ready, NSEG).start()
        out_copy(0, 0, ready).wait()
        out_copy(1, ready, NSEG).wait()

    dma = pltpu.SemaphoreType.DMA
    nt = len(TERMS)
    scratch = [
        pltpu.VMEM((3, NG // 2, nt, DB // 2, 2 * E), U32),
        pltpu.VMEM((nt, NG * E // 2, DB), U32),
        pltpu.VMEM((NFC, nt, DB // 2, 2 * LANES), U32),
        pltpu.VMEM((nt, NFC * LANES // 2, DB), U32),
        pltpu.VMEM((NSTAGE, NB, DC * H, E), BF16),
        pltpu.VMEM((NB, (PITCH + 7) * H // 2, E), U32),
        pltpu.VMEM((NG, FC, D), BF16),
        pltpu.VMEM((NSTRIP, D, FC), BF16),
        pltpu.VMEM((NSEG, T, D), BF16),
        pltpu.VMEM((2, L, D), F32),
        pltpu.VMEM((nt, NG, L, E), F32),
        pltpu.VMEM((2, LAG * T // 2, D), F32),
        pltpu.VMEM((2, L, D), F32),
        pltpu.VMEM((RING, T, D), F32),
        pltpu.VMEM((T, D), F32),
        dma((NSTAGE,)), dma((NG,)), dma((NSTRIP,)), dma((2,)), dma((2,)),
    ]
    return kernel, scratch


@functools.partial(jax.jit, static_argnames=("A_seg_len",))
def pallas_interleave_layers__memory_aug_recurrent_mem_tr__glu_gated_glu__prompt_kernel(
    A_x: jax.Array,
    A_mem0: jax.Array,
    A_Wq: jax.Array,
    A_Wk: jax.Array,
    A_Wv: jax.Array,
    A_Wo: jax.Array,
    A_seg_len: int,
    B_x: jax.Array,
    B_w_gate: jax.Array,
    B_w_up: jax.Array,
    B_w_down: jax.Array,
):
    del B_x
    B, S, D = A_x.shape
    _, H, E = A_Wq.shape
    M = A_mem0.shape[1]
    F = B_w_gate.shape[1]
    T = int(A_seg_len)
    FC = NB * LANES
    assert (B, D, H, E, M, T, F) == (1, 1024, 32, LANES, 8, 32, 3584) and S % T == 0
    kernel, scratch = _make_kernel(S, D, H, E, M, T, F)
    qkv_shape = (NB, D // (NB * DC), DC * H, E)
    hbm = pl.BlockSpec(memory_space=pl.ANY)
    out = pl.pallas_call(
        kernel,
        out_shape=jax.ShapeDtypeStruct((S // T, T, D), A_x.dtype),
        in_specs=[hbm, pl.BlockSpec(memory_space=pltpu.VMEM)] + [hbm] * 7,
        out_specs=hbm,
        scratch_shapes=scratch,
        compiler_params=pltpu.CompilerParams(
            vmem_limit_bytes=127 * 1024 * 1024),
    )(A_x.reshape(S // T, T, D), A_mem0.reshape(M, D),
      A_Wq.reshape(qkv_shape), A_Wk.reshape(qkv_shape), A_Wv.reshape(qkv_shape),
      A_Wo.reshape(H * E // FC, FC, D), B_w_gate, B_w_up, B_w_down.reshape(F // FC, FC, D))
    return out.reshape(B, S, D)
```

```python
import functools

import jax
import jax.numpy as jnp
import numpy as np
import jax.experimental.pallas as pl
import jax.experimental.pallas.tpu as pltpu

F32 = jnp.float32
BF16 = jnp.bfloat16
U32 = jnp.uint32
EPS = 1e-5
LOG2E = 1.4426950408889634
LANES = 128
NB = 4
LAG = 3
RING = 4
DC = 32
NSTAGE = 4
NSTRIP = 8
OUT_SPLIT = ((3, 2), (5, 4), (7, 6))
DOWN_SPLIT = ((2, 1), (4, 3), (6, 5))

NODES = (0.5, -0.5, 1.5, -1.5)
TERMS = [term for i in range(NB) for term in (
    [("a", i, i)] + [("q", i, j) for j in range(NB) if j != i]
    + [("r", i, j) for j in range(i + 1, NB)] + [("b", i, i)])]


def _gains(kind, i, j):
    gain = 1.0 / (NODES[j] - NODES[i]) if kind == "q" else 1.0 / (NODES[i] - NODES[j])
    right = abs(gain) if kind == "r" or np.frexp(abs(gain))[0] == 0.5 else 1.0
    return gain / right, right


def _scaled(x, gain):
    return x if gain == 1.0 else x * gain


def _centred(x):
    c = x - jnp.mean(x, axis=-1, keepdims=True)
    return c, jnp.mean(c * c, axis=-1, keepdims=True)


def _ln(x):
    c, v = _centred(x)
    return c * jax.lax.rsqrt(v + EPS)


def _rows(words):
    return pltpu.bitcast(words, BF16)


def _store_rows(words_ref, col, rows):
    words_ref.bitcast(BF16)[:, col:col + rows.shape[1]] = rows


def _dot(a, b):
    return jax.lax.dot_general(a, b, (((1,), (0,)), ((), ())), preferred_element_type=F32)


def _dot_nt(a, b):
    return jax.lax.dot_general(a, b, (((1,), (1,)), ((), ())), preferred_element_type=F32)


def _blocks(x):
    n = x.shape[1] // NB
    return [x[:, i * n:(i + 1) * n] for i in range(NB)]


def _left_terms(s, d=None):
    if d is None:
        return {n: s[i] for n, (kind, i, _) in enumerate(TERMS) if kind == "a"}
    ts = {t: [t * x for x in s] for t in NODES if t > 0}
    e = [[d[i] + ts[t][i] if t > 0 else d[i] - ts[-t][i] for i in range(NB)] for t in NODES]
    out = {}
    for n, (kind, i, j) in enumerate(TERMS):
        if kind == "a":
            out[n] = s[i]
        elif kind == "b":
            out[n] = e[i][i]
        else:
            x, y = e[j if kind == "q" else i][i], e[j][j]
            gain = _gains(kind, i, j)[0]
            out[n] = _scaled(x - y if gain > 0 else y - x, abs(gain))
    return out


def _right_terms(w):
    f = [[b.astype(F32) for b in row] for row in w]
    out = []
    for kind, i, j in TERMS:
        if kind in "qr":
            gain = _gains(kind, i, j)[1]
            if kind == "q" and gain == 1.0:
                val = w[i][j]
            else:
                val = _scaled(f[i][j] if kind == "q" else f[i][j] + f[j][i], gain)
        else:
            val = f[i][i]
            for k in range(NB):
                if k != i:
                    val = val - f[i][k] if kind == "a" else val + f[k][i]
        out.append(val.astype(BF16))
    return out


def _block_product(nl, left, right, acc=None):
    acc = [[None] * NB for _ in range(nl)] if acc is None else [list(row) for row in acc]

    def add(row, j, x):
        acc[row][j] = x if acc[row][j] is None else acc[row][j] + x

    for n, (kind, i, j) in enumerate(TERMS):
        if nl == 1:
            if kind in "aq":
                p = _dot(left(TERMS.index(("a", i, i))), right(n))
                if kind == "q":
                    p = _scaled(p, 1.0 / _gains(kind, i, j)[1])
                    add(0, j, p)
                add(0, i, p)
            continue
        p = _dot(left(n), right(n))
        if kind == "a":
            u = p
        elif kind == "b":
            add(0, i, u)
            add(1, i, p - NODES[i] * u)
        else:
            u = u + p
            add(0, j, p)
            add(1, j, -NODES[i if kind == "q" else j] * p)
    return acc


def _long_product(left, right_ref, k0, k1, acc):
    def right(c, n):
        return _rows(right_ref[n, k0 * LANES // 2:k1 * LANES // 2, c * LANES:(c + 1) * LANES])

    return [_block_product(len(old), left, functools.partial(right, c), old)
            for c, old in enumerate(acc)]


def _column_tiles(row_blocks):
    width = row_blocks[0].shape[1] // NB
    return [[[b[:, j * width + c:j * width + c + LANES] for j in range(NB)] for b in row_blocks]
            for c in range(0, width, LANES)]


def _row_blocks(tiles):
    return [jnp.concatenate([t[r][j] for j in range(NB) for t in tiles], axis=1)
            for r in range(len(tiles[0]))]


def _run(*gens, order=()):
    for which in order:
        next(gens[which], None)
    for gen in gens:
        for _ in gen:
            pass


def _make_kernel(S, D, H, E, M, T, F):
    NSEG = S // T
    NG = H // NB
    DB = D // NB
    NDC = DB // DC
    PITCH = DC + 1
    FC = NB * LANES
    NFC = F // FC
    EARLY = NSTRIP // 2
    L = M + T
    scale = float(E) ** -0.5
    assert NSTRIP == NG >= NFC and NSEG > LAG + 2

    def mask_tables(nl):
        r = jax.lax.broadcasted_iota(jnp.int32, (nl * L, nl * L), 0)
        c = jax.lax.broadcasted_iota(jnp.int32, (nl * L, nl * L), 1)
        same = (r < L) == (c < L)
        vis = same & ((jnp.where(r < L, r, r - L) < M) | (c <= r))
        return vis, jnp.where(same, -1e9 * LOG2E, -jnp.inf).astype(F32)

    def kernel(x_hbm, mem_ref, wq_hbm, wk_hbm, wv_hbm, wo_hbm, wg_hbm, wu_hbm, wd_hbm, out_hbm,
               wqkv, wo, wgu, wd, st_qkv, st_word, st_row, st_col, x_v,
               h_s, o_s, hb_s, y_s, z_s, out_s,
               sem_qkv, sem_row, sem_col, sem_x, sem_out):
        def qkv_copy(which, i):
            return pltpu.make_async_copy((wq_hbm, wk_hbm, wv_hbm)[which].at[:, i % NDC],
                                         st_qkv.at[i % NSTAGE], sem_qkv.at[i % NSTAGE])

        def row_copy(src, i):
            return pltpu.make_async_copy(src.at[i], st_row.at[i], sem_row.at[i])

        def gu_copy(which, c):
            slot = (2 * c + which) % NSTRIP
            cols = pl.ds(pl.multiple_of(c * FC, FC), FC)
            return pltpu.make_async_copy((wg_hbm, wu_hbm)[which].at[:, cols],
                                         st_col.at[slot], sem_col.at[slot])

        def convert(src, dst, row0=0, col0=0):
            n = src.shape[0] // NB
            sub = 32 * FC // src.shape[1]

            @pl.loop(0, n // sub)
            def _(r):
                w = [_blocks(src[pl.ds(pl.multiple_of(i * n + r * sub, sub), sub), :])
                     for i in range(NB)]
                rows = pl.ds(pl.multiple_of((row0 + r * sub) // 2, sub // 2), sub // 2)
                for k, val in enumerate(_right_terms(w)):
                    _store_rows(dst.at[k, rows], col0, val)

        def convert_qkv(i):
            for b in range(NB):
                for d in range(DC):
                    st_word[b, pl.ds(d // 2 + d % 2 * DC // 2, H // 2, stride=PITCH), :] = (
                        pltpu.bitcast(st_qkv[i % NSTAGE, b, d * H:(d + 1) * H, :], U32))
            rows = pl.ds(pl.multiple_of((i % NDC) * (DC // 2), DC // 2), DC // 2)
            for g in range(NG):
                w = []
                for b in range(NB):
                    w.append([])
                    for pair in range(g * NB // 2, (g + 1) * NB // 2):
                        x = st_word[b, pl.ds(pair * PITCH, DC // 2), :]
                        y = st_word[b, pl.ds(pair * PITCH + DC // 2, DC // 2), :]
                        w[-1].append(_rows((x & np.uint32(0xFFFF)) | (y << 16)))
                        w[-1].append(_rows((x >> 16) | (y & np.uint32(0xFFFF0000))))
                for k, val in enumerate(_right_terms(w)):
                    _store_rows(wqkv.at[i // NDC, g // 2, k, rows], g % 2 * E, val)

        def convert_wo(g):
            for which in range(2):
                pl.when(g % 2 == which)(gu_copy(which, g // 2).start)
            row_copy(wo_hbm, g).wait()
            convert(st_row.at[g], wo, g * E)

        def convert_gu(c):
            for which in range(2):
                gu_copy(which, c).wait()
                convert(st_col.at[(2 * c + which) % NSTRIP], wgu.at[c], 0, which * LANES)
            pending = c + NSTRIP // 2

            @pl.when(pending < NFC)
            def _():
                for which in range(2):
                    gu_copy(which, pending).start()

            for j in range(2):
                piece = 2 * (pending - NFC) + j
                pl.when((piece >= 0) & (piece < NFC))(
                    row_copy(wd_hbm, jnp.clip(piece, 0, NFC - 1)).start)

        def convert_wd(c):
            row_copy(wd_hbm, c).wait()
            convert(st_row.at[c], wd, c * LANES)

        x_head = pltpu.make_async_copy(x_hbm.at[0:LAG + 2], x_v.at[0:LAG + 2], sem_x.at[0])
        x_rest = pltpu.make_async_copy(x_hbm.at[LAG + 2:NSEG], x_v.at[LAG + 2:NSEG], sem_x.at[1])

        def out_copy(i, lo, hi):
            return pltpu.make_async_copy(x_v.at[lo:hi], out_hbm.at[lo:hi], sem_out.at[i])

        def x_seg(seg):
            return x_v[seg].astype(F32)

        def set_rows(*blocks):
            for j, (mem, tok) in enumerate(blocks):
                h_s[j, :M, :] = mem
                h_s[j, M:, :] = tok

        def attention(nl, residual, before_out=None):
            vis, fill = mask_tables(nl)
            h = _left_terms(*[_blocks(h_s[j]) for j in range(nl)])

            def proj(j, g):
                cols = slice(g % 2 * E, (g % 2 + 1) * E)
                c = _block_product(nl, h.__getitem__,
                                   lambda n: _rows(wqkv[j, g // 2, n, :, cols]))
                heads = [jnp.concatenate([row[h] for row in c], axis=0) for h in range(NB)]
                return heads if j == 0 else [x.astype(BF16) for x in heads]

            def proj_all(g):
                k = proj(1, g)
                return proj(0, g), k, proj(2, g)

            def attend(s, v):
                s = jnp.where(vis, s * (scale * LOG2E), fill)
                p = jnp.exp2(s - jnp.max(s, axis=-1, keepdims=True))
                tot = jnp.sum(p, axis=-1, keepdims=True)
                inv = pl.reciprocal(tot, approx=True)
                inv = inv * (2.0 - tot * inv)
                return _dot(p, v) * inv

            def out_proj(g0, g1, acc):
                if acc is None:
                    acc = _column_tiles([jnp.concatenate([jnp.zeros((M, D), F32), x], axis=0)
                                         for x in residual()])
                return _long_product(
                    lambda n: jnp.concatenate([o_s[n, g] for g in range(g0, g1)], axis=1),
                    wo, g0, g1, acc)

            q, k, v = proj_all(0)
            acc, done = None, 0
            for g in range(NG):
                scores = [_dot_nt(q[h], k[h]) for h in range(NB)]
                for at, upto in (OUT_SPLIT if before_out is None else ()):
                    if at == g:
                        acc, done = out_proj(done, upto, acc), upto
                if g + 1 < NG:
                    nxt = proj_all(g + 1)
                else:
                    yield
                o = [attend(scores[h], v[h]) for h in range(NB)]
                parts = [[x[j * L:(j + 1) * L] for x in o] for j in range(nl)]
                for n, a in _left_terms(*parts).items():
                    o_s[n, g] = a
                q, k, v = nxt
                yield
            if before_out is not None:
                before_out()
                for _, upto in OUT_SPLIT:
                    acc, done = out_proj(done, upto, acc), upto
            acc = out_proj(done, NG, acc)
            yield
            for j, y in enumerate(_row_blocks(acc)):
                y_s[j] = y

        def set_glu_rows(*blocks):
            for j, b in enumerate(blocks):
                c, v = _centred(b)
                unit = jax.lax.rsqrt(v + 1e-30)
                size = jax.lax.rsqrt(v + EPS) * ((v + 1e-30) * unit)
                hb_s[j, 0:b.shape[0], 0:D] = c * (0.5 * unit)
                hb_s[j, 0:b.shape[0], D:] = jnp.broadcast_to(size, (b.shape[0], LANES))

        def glu(nl, rows, residual, finish, before_down=lambda c: None):
            hb = _left_terms(*[_blocks(hb_s[j, 0:rows, 0:D]) for j in range(nl)])
            hb = {n: a.astype(BF16) for n, a in hb.items()}

            size = [hb_s[j, 0:rows, D:] for j in range(nl)]
            acts = []

            def gate_up(c):
                g, u = (_block_product(nl, hb.__getitem__,
                                       lambda n: _rows(wgu[c, n, :, j * LANES:(j + 1) * LANES]))
                        for j in range(2))
                act = [[jnp.tanh(x * size[j]) * y + y for x, y in zip(g[j], u[j])] for j in range(nl)]
                acts.append(_left_terms(*act))

            def down(c0, c1, acc):
                before_down(c0)
                acc = [[[None] * NB] * nl] * (DB // LANES) if acc is None else acc
                return _long_product(
                    lambda n: jnp.concatenate([acts[c][n] for c in range(c0, c1)], axis=1),
                    wd, c0, c1, acc)

            acc, done = None, 0
            for c in range(NFC):
                gate_up(c)
                for at, upto in DOWN_SPLIT:
                    if at == c:
                        acc, done = down(done, upto, acc), upto
                yield
            finish([y + x * jnp.tile(w, (1, D // LANES)) for y, x, w in zip(
                residual(), _row_blocks(down(done, NFC, acc)), size)])

        x_head.start()
        for i in range(NSTAGE):
            qkv_copy(0, i).start()

        @pl.loop(0, 3 * NDC)
        def _(i):
            for which in range(3):
                pl.when(i // NDC == which)(qkv_copy(which, i).wait)
            convert_qkv(i)
            for which in range(3):
                pl.when((i + NSTAGE) // NDC == which)(qkv_copy(which, i + NSTAGE).start)
            piece = i + NSTAGE - 3 * NDC
            pl.when(piece >= 0)(row_copy(wo_hbm, jnp.maximum(piece, 0)).start)

        for g in range(NSTAGE, NG):
            row_copy(wo_hbm, g).start()
        x_head.wait()
        mem0 = mem_ref[...].astype(F32)
        set_rows((mem0, _ln(x_seg(0))))

        @pl.loop(0, LAG)
        def _(t):
            def convert_arrived():
                pl.loop(0, jnp.where(t == 0, NG, 0))(convert_wo)
                pl.loop(jnp.maximum(t - 1, 0) * EARLY,
                        jnp.where(t + 1 < LAG, t * EARLY, NFC))(convert_gu)

            _run(attention(1, lambda: [x_seg(t)], convert_arrived))
            z_s[t] = y_s[0, M:, :]
            set_rows((y_s[0, :M, :], _ln(x_seg(t + 1))))

        set_glu_rows(z_s[0])

        def head_down(c):
            cut = DOWN_SPLIT[1][1]
            if c in (0, cut):
                pl.loop(c, NFC if c else cut)(convert_wd)

        def head_finish(z):
            z_s[0], = z

        _run(glu(1, T, lambda: [z_s[0]], head_finish, head_down))
        x_rest.start()

        def tokens():
            return [y_s[0, M:, :], y_s[1, M:, :]]

        def step_rows(t):
            set_rows((y_s[0, :M, :], _ln(x_seg(jnp.minimum(t, NSEG - 1)))),
                     (y_s[1, :M, :], _ln(z_s[(t - LAG) % RING])))

        def glu_finish(t):
            def finish(z):
                z_s[t % RING], out_s[...] = z
            return finish

        y_s[1] = jnp.concatenate([mem0, z_s[1]], axis=0)
        out_s[...] = z_s[0]
        step_rows(LAG)
        set_glu_rows(*tokens())

        def emit(seg):
            x_v[seg] = out_s[...].astype(x_v.dtype)

        def second_step():
            x_rest.wait()
            z_s[1] = out_s[...]
            step_rows(LAG + 1)

        @pl.loop(LAG, NSEG)
        def _(t):
            pl.when(t == LAG + 1)(second_step)
            emit(jnp.maximum(t - 2 - LAG, 0))
            previous = tokens()

            def attention_then_next_rows():
                yield from attention(2, lambda: [x_seg(t), z_s[(t - LAG) % RING]])
                step_rows(t + 1)
                set_glu_rows(*tokens())

            _run(glu(2, T, lambda: previous, glu_finish(t - 1)), attention_then_next_rows(),
                 order=(1,) * NG + (0, 1, 0, 1, 1))

        ready = NSEG - 1 - LAG
        emit(NSEG - 2 - LAG)
        out_copy(0, 0, ready).start()
        set_rows((y_s[1, :M, :], _ln(z_s[(NSEG - LAG) % RING])))
        _run(glu(2, T, tokens, glu_finish(NSEG - 1)))
        emit(NSEG - 1 - LAG)

        @pl.loop(NSEG - LAG, NSEG)
        def _(t):
            _run(attention(1, lambda: [z_s[t % RING]]))
            set_rows((y_s[0, :M, :], _ln(z_s[jnp.minimum(t + 1, NSEG - 1) % RING])))
            z_s[t % RING] = y_s[0, M:, :]

        def last_rows():
            y = jnp.concatenate([z_s[t % RING] for t in range(NSEG - LAG, NSEG)], axis=0)
            return y[:LAG * T // 2], y[LAG * T // 2:]

        def last_finish(z):
            z = jnp.concatenate(z, axis=0).astype(x_v.dtype)
            for j in range(LAG):
                x_v[NSEG - LAG + j] = z[j * T:(j + 1) * T]

        set_glu_rows(*last_rows())
        _run(glu(2, LAG * T // 2, last_rows, last_finish))
        out_copy(1, ready, NSEG).start()
        out_copy(0, 0, ready).wait()
        out_copy(1, ready, NSEG).wait()

    dma = pltpu.SemaphoreType.DMA
    nt = len(TERMS)
    scratch = [
        pltpu.VMEM((3, NG // 2, nt, DB // 2, 2 * E), U32),
        pltpu.VMEM((nt, NG * E // 2, DB), U32),
        pltpu.VMEM((NFC, nt, DB // 2, 2 * LANES), U32),
        pltpu.VMEM((nt, NFC * LANES // 2, DB), U32),
        pltpu.VMEM((NSTAGE, NB, DC * H, E), BF16),
        pltpu.VMEM((NB, (PITCH + 7) * H // 2, E), U32),
        pltpu.VMEM((NG, FC, D), BF16),
        pltpu.VMEM((NSTRIP, D, FC), BF16),
        pltpu.VMEM((NSEG, T, D), BF16),
        pltpu.VMEM((2, L, D), F32),
        pltpu.VMEM((nt, NG, L, E), F32),
        pltpu.VMEM((2, LAG * T // 2, D + LANES), F32),
        pltpu.VMEM((2, L, D), F32),
        pltpu.VMEM((RING, T, D), F32),
        pltpu.VMEM((T, D), F32),
        dma((NSTAGE,)), dma((NG,)), dma((NSTRIP,)), dma((2,)), dma((2,)),
    ]
    return kernel, scratch


@functools.partial(jax.jit, static_argnames=("A_seg_len",))
def pallas_interleave_layers__memory_aug_recurrent_mem_tr__glu_gated_glu__prompt_kernel(
    A_x: jax.Array,
    A_mem0: jax.Array,
    A_Wq: jax.Array,
    A_Wk: jax.Array,
    A_Wv: jax.Array,
    A_Wo: jax.Array,
    A_seg_len: int,
    B_x: jax.Array,
    B_w_gate: jax.Array,
    B_w_up: jax.Array,
    B_w_down: jax.Array,
):
    del B_x
    B, S, D = A_x.shape
    _, H, E = A_Wq.shape
    M = A_mem0.shape[1]
    F = B_w_gate.shape[1]
    T = int(A_seg_len)
    FC = NB * LANES
    assert (B, D, H, E, M, T, F) == (1, 1024, 32, LANES, 8, 32, 3584) and S % T == 0
    kernel, scratch = _make_kernel(S, D, H, E, M, T, F)
    qkv_shape = (NB, D // (NB * DC), DC * H, E)
    hbm = pl.BlockSpec(memory_space=pl.ANY)
    out = pl.pallas_call(
        kernel,
        out_shape=jax.ShapeDtypeStruct((S // T, T, D), A_x.dtype),
        in_specs=[hbm, pl.BlockSpec(memory_space=pltpu.VMEM)] + [hbm] * 7,
        out_specs=hbm,
        scratch_shapes=scratch,
        compiler_params=pltpu.CompilerParams(
            vmem_limit_bytes=127 * 1024 * 1024),
    )(A_x.reshape(S // T, T, D), A_mem0.reshape(M, D),
      A_Wq.reshape(qkv_shape), A_Wk.reshape(qkv_shape), A_Wv.reshape(qkv_shape),
      A_Wo.reshape(H * E // FC, FC, D), B_w_gate, B_w_up, B_w_down.reshape(F // FC, FC, D))
    return out.reshape(B, S, D)
```
